```python
import jax
import jax.numpy as jnp

def _softmax(x, axis=-1):
    return jax.nn.softmax(x, axis=axis)
def _gelu(x):
    return jax.nn.gelu(x, approximate=True)
def _silu(x):
    return jax.nn.silu(x)
def _sigmoid(x):
    return jax.nn.sigmoid(x)
def _layernorm(x, axis=-1, eps=1e-5):
    m = jnp.mean(x, axis=axis, keepdims=True)
    v = jnp.var(x, axis=axis, keepdims=True)
    return (x - m) / jnp.sqrt(v + eps)
def _scatter_add(tgt, idx, src, axis=0):
    return tgt.at[idx].add(src)
def _segment_sum(src, seg, n):
    return jax.ops.segment_sum(src, seg, n)
class _Rng:
    def __init__(self, key):
        self._k = key
    def _next(self):
        self._k, sub = jax.random.split(self._k)
        return sub
    def normal(self, shape):
        return jax.random.normal(self._next(), shape, dtype=jnp.bfloat16)
    def randint(self, lo, hi, shape):
        return jax.random.randint(self._next(), shape, lo, hi, dtype=jnp.int32)
    def uniform(self, shape, lo=0.0, hi=1.0):
        return jax.random.uniform(self._next(), shape, jnp.bfloat16, lo, hi)
    def permutation(self, n):
        return jax.random.permutation(self._next(), n)


kernel_name = 'interleave_layers__sliding_local_dilated__softmax_full_mha__prompt'

def setup_inputs():
    _rng = _Rng(jax.random.key(int.from_bytes(__import__("os").urandom(4), "little")))
    _w = (lambda a: (lambda t: t.astype(jnp.bfloat16) if jnp.issubdtype(t.dtype, jnp.floating) else t)(jnp.asarray(a)))
    def _A_setup():
        B, S, D = 1, 2048, 1024
        return {
            "x": _w((lambda *s: _rng.normal(s) * 0.05)(B, S, D)),
            "wqkv": _w((lambda *s: _rng.normal(s) * 0.05)(D, 3 * D)),
            "wo": _w((lambda *s: _rng.normal(s) * 0.05)(D, D)),
        }
    _A_in = _A_setup()

    def _B_setup():
        B, S, D = 1, 2048, 1024
        return {
            "x": _w((lambda *s: _rng.normal(s) * 0.05)(B, S, D)),
            "wqkv": _w((lambda *s: _rng.normal(s) * 0.05)(D, 3 * D)),
            "wo": _w((lambda *s: _rng.normal(s) * 0.05)(D, D)),
        }
    _B_in = _B_setup()

    return {
        "A_x": _A_in["x"],
        "A_wqkv": _A_in["wqkv"],
        "A_wo": _A_in["wo"],
        "B_x": _B_in["x"],
        "B_wqkv": _B_in["wqkv"],
        "B_wo": _B_in["wo"],
    }

def reference(A_x, A_wqkv, A_wo, B_x, B_wqkv, B_wo):
    def _A_ref(x, wqkv, wo):
        B, S, D = x.shape
        H = 32; Dh = D // H
        W, dil = 8, 2
        qkv = (lambda x, *d: x.transpose(*d))((x @ wqkv).reshape(B, S, 3, H, Dh), 2, 0, 3, 1, 4)
        q, k, v = qkv[0], qkv[1], qkv[2]
        scale = Dh ** -0.5
        pos = jnp.arange(S)
        off = jnp.arange(W) * dil
        idx = pos[:, None] - off[None, :]
        mask = idx >= 0
        idx_c = jnp.where(mask, idx, 0).reshape(-1)
        kg = k[:, :, idx_c, :].reshape(B, H, S, W, Dh)
        vg = v[:, :, idx_c, :].reshape(B, H, S, W, Dh)
        logits = jnp.einsum("bhsd,bhswd->bhsw", q, kg) * scale
        logits = jnp.where(mask[None, None, :, :], logits, -1e9)
        attn = _softmax(logits, axis=-1)
        o = jnp.einsum("bhsw,bhswd->bhsd", attn, vg)
        return (lambda x, *d: x.transpose(*d))(o, 0, 2, 1, 3).reshape(B, S, D) @ wo

    def _B_ref(x, wqkv, wo):
        B, S, D = x.shape
        H = 32; Dh = D // H
        qkv = (lambda x, *d: x.transpose(*d))((x @ wqkv).reshape(B, S, 3, H, Dh), 2, 0, 3, 1, 4)
        q, k, v = qkv[0], qkv[1], qkv[2]
        scale = Dh ** -0.5
        scores = jnp.einsum("bhqd,bhkd->bhqk", q, k) * scale
        p = _softmax(scores, axis=-1)
        o = jnp.einsum("bhqk,bhkd->bhqd", p, v)
        return (lambda x, *d: x.transpose(*d))(o, 0, 2, 1, 3).reshape(B, S, D) @ wo

    x = A_x
    x = x + _A_ref(_layernorm(x, axis=-1), A_wqkv, A_wo)
    x = x + _B_ref(_layernorm(x, axis=-1), B_wqkv, B_wo)
    x = x + _A_ref(_layernorm(x, axis=-1), A_wqkv, A_wo)
    x = x + _B_ref(_layernorm(x, axis=-1), B_wqkv, B_wo)
    return x
```

```python
import math

import jax
import numpy as np
import jax.numpy as jnp
from jax import lax
import jax.experimental.pallas as pl
import jax.experimental.pallas.tpu as pltpu

S = 2048
D = 1024
DH = 32
WIN = 8
EPS = 1e-5
LOG2E = math.log2(math.e)
QSCALE = DH ** -0.5 * LOG2E
MASKED = -1e9 * LOG2E

NQ = 512
KC = 128
NC = S // KC
LAG = 2
T0 = 24

BF = jnp.bfloat16
F32 = jnp.float32
U32 = jnp.uint32


def _pack(x):
    return pltpu.bitcast(x, U32)


def _unpack(x):
    return pltpu.bitcast(x, BF)


def _halves(w):
    lo = lax.bitcast_convert_type(w << 16, F32)
    hi = lax.bitcast_convert_type(w & np.uint32(0xFFFF0000), F32)
    return lo, hi


def _ds(i, n):
    if isinstance(i, int):
        return pl.ds(i * n, n)
    return pl.ds(pl.multiple_of(i * n, n), n)


def _dot(a, b):
    return jnp.dot(a, b, preferred_element_type=F32)


def _kernel(x_hbm, aq_hbm, ao_hbm, bq_hbm, bo_hbm, out_hbm,
            x_raw, aq_raw, ao_raw, bq_raw, bo_raw, tmp0, tmp1,
            aq_t0, aq_t1, ao_t, bq_t, bo_t,
            x_t, xn_t, o_t,
            q0, q1, k0, k1, v0, v1, vfirst,
            bq_s, bk_s, bv_s, s0, s1,
            sem_x, sem_aq, sem_w, sem_o):
    aq_t, qbuf, kbuf, vbuf, sbuf, tmp = (aq_t0, aq_t1), (q0, q1), (k0, k1), (v0, v1), (s0, s1), (tmp0, tmp1)

    def x_copy(ct):
        return pltpu.make_async_copy(x_hbm.at[:, _ds(ct, 128)], x_raw.at[ct], sem_x.at[ct])

    def aq_copy(g, t):
        return pltpu.make_async_copy(aq_hbm.at[:, _ds(4 * t + g, 256)], aq_raw.at[:, _ds(4 * t + g, 256)],
                                     sem_aq.at[4 * t + g])

    def w_copy(i):
        src, dst = ((ao_hbm, ao_raw), (bq_hbm, bq_raw), (bo_hbm, bo_raw))[i]
        return pltpu.make_async_copy(src, dst, sem_w.at[i])

    def out_copy(ct):
        return pltpu.make_async_copy(x_raw.at[ct], out_hbm.at[:, _ds(ct, 128)], sem_o.at[ct])

    def load_x(ct):
        scr = tmp[ct % 2]
        scr[...] = _pack(x_raw[ct])
        for c in range(8):
            lo, hi = _halves(scr[pl.ds(c, 128, stride=8), :].T)
            x_t[_ds(ct, 128), _ds(c, 128)] = lo
            x_t[_ds(ct, 128), _ds(8 + c, 128)] = hi

    def store_x(ct, y, scr):
        bits = lax.bitcast_convert_type(y.astype(BF).astype(F32), U32)
        for c in range(8):
            w = (bits[:, c * 128:(c + 1) * 128] >> 16) | bits[:, (8 + c) * 128:(9 + c) * 128]
            scr[pl.ds(c, 128, stride=8), :] = w.T
        x_raw[ct] = _unpack(scr[...])

    def head_major(scr, dp, n):
        lo, hi = _halves(scr[pl.ds(dp, 8 * n, stride=16), :])
        return jnp.concatenate([lo.reshape(n, 8, 128), hi.reshape(n, 8, 128)], axis=1)

    def prep_aq(g, par, t):
        scr = tmp[t % 2]
        wt = _pack(aq_raw[:, _ds(4 * t + g, 256)].T)
        for kt in range(8):
            scr[_ds(kt, 128), :] = wt[:, kt * 128:(kt + 1) * 128]
        for dp in range(16):
            w = _pack(head_major(scr, dp, 8).reshape(128, 128).astype(BF))
            aq_t[par][g // 2, pl.ds(t * 128 + dp * 8, 8), :] = jnp.concatenate(
                [w[kt * 8:(kt + 1) * 8] for kt in range(8)], axis=1)

    def prep_ao(ct, scr):
        scr[pl.ds(0, 512), :] = _pack(ao_raw[:, _ds(ct, 128)])
        w = jnp.concatenate([head_major(scr, dp, 4) for dp in range(16)], axis=1)
        ao_t[_ds(ct, 64), :] = _pack(w.reshape(D, 128).astype(BF).T)

    def prep_plain(raw, dst, ct):
        dst[_ds(ct, 64), :] = _pack(raw[:, _ds(ct, 128)].T)

    def layernorm(x, tile):
        x3 = x.reshape(D // 8, 8, 128)
        mean = jnp.sum(jnp.sum(x3, axis=0), axis=0, keepdims=True) * (1.0 / D)
        xc = x3 - jnp.broadcast_to(mean, (8, 128))
        var = jnp.sum(jnp.sum(xc * xc, axis=0), axis=0, keepdims=True) * (1.0 / D)
        xn = xc * jnp.broadcast_to(lax.rsqrt(var + EPS), (8, 128))
        xn_t[:, _ds(tile, 128)] = _pack(xn.reshape(D, 128).astype(BF))

    def out_proj(w_t, tile, norm):
        x = x_t[:, _ds(tile, 128)] + _dot(_unpack(w_t[...]), _unpack(o_t[:, _ds(tile, 128)]))
        x_t[:, _ds(tile, 128)] = x
        if norm:
            layernorm(x, tile)

    def a_qkv(u, par):
        g, e = u % 4, u // 4
        lane0 = lax.broadcasted_iota(jnp.int32, (256, 128), 1) == 0
        first = None
        for c in range(8):
            y = _dot(_unpack(aq_t[par][g // 2]), _unpack(xn_t[:, _ds(8 * e + c, 128)]))
            q, k, v = y[:256], y[256:512], y[512:]
            qbuf[par][:, _ds(c, 128)] = q
            kbuf[par][:, _ds(7 + c, 128)] = k
            vbuf[par][:, _ds(7 + c, 128)] = v
            if c == 0:
                if isinstance(e, int):
                    first = v if e == 0 else vfirst[g]
                else:
                    first = jnp.where(e == 0, v, vfirst[g])
                vfirst[g] = first
            else:
                kbuf[par][:, _ds(c - 1, 128)] = pltpu.roll(k, 1, 1)
                vbuf[par][:, _ds(c - 1, 128)] = jnp.where(lane0, first, pltpu.roll(v, 1, 1))

    def a_attn(u, par, c):
        g, e = u % 4, u // 4
        win = pl.ds(c * 128, WIN * 128)
        acc = None
        for d in range(DH):
            t = jnp.tile(qbuf[par][_ds(d, 8), _ds(c, 128)], (1, WIN)) * kbuf[par][_ds(d, 8), win]
            acc = t if acc is None else acc + t
        lane0 = lax.broadcasted_iota(jnp.int32, (8, 128), 1) == 0
        logit = []
        for w in range(WIN):
            t = acc[:, w * 128:(w + 1) * 128] * QSCALE
            logit.append(jnp.where(lane0, MASKED, t) if c + w < 7 else t)
        m = logit[0]
        for t in logit[1:]:
            m = jnp.maximum(m, t)
        p = [jnp.exp2(t - m) for t in logit]
        l = p[0]
        for t in p[1:]:
            l = l + t
        r = 1.0 / l
        p = jnp.concatenate([t * r for t in p], axis=1)
        p = jnp.concatenate([p, p], axis=0)
        for dp in range(DH // 2):
            t = p * vbuf[par][_ds(dp, 16), win]
            o = t[:, :128]
            for w in range(1, WIN):
                o = o + t[:, w * 128:(w + 1) * 128]
            o_t[_ds(16 * g + dp, 8), _ds(8 * e + c, 128)] = _pack(o.astype(BF))

    def a_step(u, par, attn=True, prep_next=True):
        a_qkv(u, par)
        if attn:
            for c in range(8):
                a_attn(u - 1, 1 - par, c)
        if prep_next:
            for t in range(3):
                prep_aq((u + 1) % 4, 1 - par, t)
        prep_ao(u, tmp[1])

    def b_qkv(j):
        xn = _unpack(xn_t[:, _ds(j, 256)])
        k = _dot(_unpack(bq_t[_ds(1, 512), :]), xn).astype(BF)
        for g in range(8):
            bk_s[g, _ds(j, 128), :] = _pack(k[g * 128:(g + 1) * 128].T)
        q = _dot(_unpack(bq_t[_ds(0, 512), :]), xn) * QSCALE
        bq_s[:, _ds(j, 256)] = _pack(q.astype(BF))
        v = _dot(_unpack(bq_t[_ds(2, 512), :]), xn)
        bv_s[:, _ds(j, 256)] = _pack(v.astype(BF))

    def b_steps(i, t_lo, t_hi, state, qk_end=None):
        m_old, m_new, m_run, l, acc = state
        ms = {t_lo // NC - 2: m_old, t_lo // NC - 1: m_new}
        hist = []
        for t in range(t_lo, t_hi):
            u, c = divmod(t, NC)
            s = None
            if qk_end is None or t < qk_end:
                n, h = i + u // 4, u % 4
                g, qb = n % 8, n // 8
                q = [_unpack(bq_s[_ds(4 * g + h, 16), _ds(qb, NQ)])]
                if h > 0:
                    q.insert(0, jnp.zeros((DH * h, NQ), BF))
                if h < 3:
                    q.append(jnp.zeros((DH * (3 - h), NQ), BF))
                s = _dot(_unpack(bk_s[g, _ds(c, KC // 2), :]), jnp.concatenate(q, axis=0))
            up, cp = divmod(t - NC - LAG, NC)
            if up >= 0:
                m = ms[up]
                if len(hist) >= 2 and hist[-2][1] is not None:
                    m = jnp.where(hist[-1][0] < 0, hist[-2][1], m)
                z = sbuf[up % 2][_ds(cp, KC), :].reshape(KC // 8, 8, NQ) - m
            if s is not None:
                sbuf[u % 2][_ds(c, KC), :] = s
                mx = jnp.max(s.reshape(KC // 8, 8, NQ), axis=0)
                m_run = mx if c == 0 else jnp.maximum(m_run, mx)
                if c == NC - 1:
                    ms[u] = jnp.broadcast_to(jnp.max(m_run, axis=0, keepdims=True), (8, NQ))
            if up >= 0:
                n, h = i + up // 4, up % 4
                g, qb = n % 8, n // 8
                p = jnp.exp2(z)
                ls = jnp.sum(p, axis=0)
                l = ls if cp == 0 else l + ls
                hist.append((l, None if s is None else s[KC - 8:]))
                a = _dot(_unpack(bv_s[_ds(4 * g + h, 16), _ds(cp, KC)]), p.reshape(KC, NQ).astype(BF))
                acc = a if cp == 0 else acc + a
                if cp == NC - 1:
                    r = 1.0 / jnp.sum(l, axis=0, keepdims=True)
                    o_t[_ds(4 * g + h, 16), _ds(qb, NQ)] = _pack((acc * r).astype(BF))
        zero = jnp.zeros((8, NQ), F32)
        return ms.get(t_hi // NC - 2, zero), ms.get(t_hi // NC - 1, zero), m_run, l, acc

    def b_attn():
        zero = jnp.zeros((8, NQ), F32)
        n_iter = (D // DH) * (S // NQ) // 4
        state = b_steps(0, 0, T0, (zero, zero, zero, zero, jnp.zeros((DH, NQ), F32)))
        state = lax.fori_loop(0, n_iter - 1, lambda i, st: b_steps(i, T0, T0 + 4 * NC, st), state)
        b_steps(n_iter - 1, T0, 5 * NC + LAG, state, qk_end=4 * NC)

    for ct in range(8):
        x_copy(ct).start()
    for g in range(4):
        for t in range(3):
            aq_copy(g, t).start()
        if g == 1:
            w_copy(0).start()
    w_copy(1).start()
    w_copy(2).start()

    for ct in range(8):
        x_copy(ct).wait()
        load_x(ct)
    for tile in range(8):
        layernorm(x_t[:, _ds(tile, 128)], tile)
    for t in range(3):
        aq_copy(0, t).wait()
        prep_aq(0, 0, t)

    def layer_pair(it, carry):
        @pl.when(it == 0)
        def _():
            for t in range(3):
                aq_copy(1, t).wait()
            w_copy(0).wait()

        a_step(0, 0, attn=False)
        for tile in range(8, 16):
            layernorm(x_t[:, _ds(tile, 128)], tile)

        @pl.when(it == 0)
        def _():
            for g in (2, 3):
                for t in range(3):
                    aq_copy(g, t).wait()

        def a_pair(j, c):
            a_step(2 * j + 1, 1)
            a_step(2 * j + 2, 0)
            return c

        lax.fori_loop(0, 3, a_pair, 0)

        @pl.when(it == 0)
        def _():
            w_copy(1).wait()
            w_copy(2).wait()

        a_step(7, 1, prep_next=False)
        for tile in range(8):
            out_proj(ao_t, tile, True)
            a_attn(7, 1, tile)
        for tile in range(8, 16):
            out_proj(ao_t, tile, False)
            for t in range(3):
                prep_plain(bq_raw, bq_t, 3 * (tile - 8) + t)

        b_qkv(0)
        for tile in range(8, 16):
            layernorm(x_t[:, _ds(tile, 128)], tile)
            prep_plain(bo_raw, bo_t, tile - 8)

        def b_body(j, c):
            b_qkv(j)
            return c

        lax.fori_loop(1, 8, b_body, 0)
        b_attn()

        @pl.when(it == 0)
        def _():
            for tile in range(16):
                out_proj(bo_t, tile, tile < 8)

        return carry

    lax.fori_loop(0, 2, layer_pair, 0)

    for ct in range(8):
        y = x_t[_ds(ct, 128), :] + _dot(_unpack(bo_t[_ds(ct, 64), :]), _unpack(o_t[...]))
        store_x(ct, y, tmp[ct % 2])
        out_copy(ct).start()
    for ct in range(8):
        out_copy(ct).wait()


@jax.jit
def pallas_interleave_layers__sliding_local_dilated__softmax_full_mha__prompt_kernel(
    A_x: jax.Array,
    A_wqkv: jax.Array,
    A_wo: jax.Array,
    B_x: jax.Array,
    B_wqkv: jax.Array,
    B_wo: jax.Array,
):
    del B_x
    vmem = pltpu.VMEM
    scratch = [
        vmem((8, S, 128), BF), vmem((D, 3 * D), BF), vmem((D, D), BF), vmem((D, 3 * D), BF), vmem((D, D), BF),
        vmem((S // 2, 128), U32), vmem((S // 2, 128), U32),
        vmem((2, 384, D), U32), vmem((2, 384, D), U32),
        vmem((D // 2, D), U32), vmem((3 * D // 2, D), U32), vmem((D // 2, D), U32),
        vmem((D, S), F32), vmem((D // 2, S), U32), vmem((D // 2, S), U32),
        vmem((256, 8 * 128), F32), vmem((256, 8 * 128), F32),
        vmem((256, 15 * 128), F32), vmem((256, 15 * 128), F32),
        vmem((256, 15 * 128), F32), vmem((256, 15 * 128), F32),
        vmem((4, 256, 128), F32),
        vmem((D // 2, S), U32), vmem((8, S // 2, 128), U32), vmem((D // 2, S), U32),
        vmem((S, NQ), F32), vmem((S, NQ), F32),
        pltpu.SemaphoreType.DMA((8,)), pltpu.SemaphoreType.DMA((12,)),
        pltpu.SemaphoreType.DMA((3,)), pltpu.SemaphoreType.DMA((8,)),
    ]
    out = pl.pallas_call(
        _kernel,
        out_shape=jax.ShapeDtypeStruct((S, D), A_x.dtype),
        in_specs=[pl.BlockSpec(memory_space=pl.ANY)] * 5,
        out_specs=pl.BlockSpec(memory_space=pl.ANY),
        scratch_shapes=scratch,
        compiler_params=pltpu.CompilerParams(vmem_limit_bytes=120 * 1024 * 1024),
        name="interleaved_attention_layers",
    )(A_x.reshape(S, D), A_wqkv, A_wo, B_wqkv, B_wo)
    return out.reshape(A_x.shape)
```

```python
import math

import jax
import numpy as np
import jax.numpy as jnp
from jax import lax
import jax.experimental.pallas as pl
import jax.experimental.pallas.tpu as pltpu

S = 2048
D = 1024
DH = 32
WIN = 8
EPS = 1e-5
LOG2E = math.log2(math.e)
QSCALE = DH ** -0.5 * LOG2E
MASKED = -1e9 * LOG2E

NQ = 512
KC = 128
NC = S // KC
LAG = 2
T0 = 24

BF = jnp.bfloat16
F32 = jnp.float32
U32 = jnp.uint32
WAO, WBQ, WBK, WBV, WBO = range(5)
PH = "all"
def on(p): return PH == "all" or p in PH.split(",")
CFG = {}
LAG = CFG.get("lag", 3)


def _pack(x):
    return pltpu.bitcast(x.astype(BF), U32)


def _unpack(x):
    return pltpu.bitcast(x, BF)


def _halves(w):
    lo = lax.bitcast_convert_type(w << 16, F32)
    hi = lax.bitcast_convert_type(w & np.uint32(0xFFFF0000), F32)
    return lo, hi


def _ds(i, n):
    if isinstance(i, int):
        return pl.ds(i * n, n)
    return pl.ds(pl.multiple_of(i * n, n), n)


def _dot(a, b):
    return jnp.dot(a, b, preferred_element_type=F32)


def _lhs7(a11, a12, a21, a22):
    return (a11 + a22, a21 + a22, a22, a12 - a22, a11 + a12, a11, a21 - a11)


def _rhs7(b11, b12, b21, b22):
    return (b11 + b22, b11, b21 - b11, b21 + b22, b22, b12 - b22, b11 + b12)


def _after(x, token):
    return jnp.where(token < -jnp.inf, jnp.zeros_like(x), x)


def _head_after(x, token):
    if token is None:
        return x
    head = _after(x[:8], jnp.tile(token, (1, x.shape[1] // 128)))
    return head if x.shape[0] == 8 else jnp.concatenate([head, x[8:]], axis=0)


class _Lane:
    def __init__(self):
        self.token = self.link = None

    def follow(self, x):
        return _head_after(x, self.token)

    def follow_all(self, x):
        if self.token is None:
            return x
        return _after(x, jnp.tile(self.token, (x.shape[0] // 8, x.shape[1] // 128)))

    def tie(self, *xs):
        if self.token is None:
            return
        t = None
        for x in xs:
            for r in range(0, x.shape[0], 8):
                for c in range(0, x.shape[1], 128):
                    t = x[r:r + 8, c:c + 128] if t is None else t + x[r:r + 8, c:c + 128]
        self.link = t

    def put(self, vals, ref, idx):
        for v, i in zip(vals, idx):
            ref[i] = _pack(v)


class _Pace:
    def __init__(self):
        self.now, self.marks, self.queue, self.gates = 0, [], [], []

    def spread(self, lo, hi, *jobs):
        lane = _Lane()
        total = sum(sum(costs) for _, _, costs in jobs)
        done = 0
        for fn, args, costs in jobs:
            gen = fn(lane, *args)
            for cost in costs:
                self.queue.append((lo + (hi - lo) * done // total, len(self.queue), lane, gen))
                done += cost
        self.queue.append((hi, len(self.queue), lane, None))
        self.queue.sort(key=lambda e: e[:2])

    def dot(self, lhs, rhs):
        for gate in self.gates:
            lhs = jnp.concatenate([_head_after(lhs[:, :128], gate), lhs[:, 128:]], axis=1)
        self.gates = []
        y = _dot(_unpack(lhs), rhs)
        self.marks = (self.now, y)
        self.now += y.shape[0]
        return y

    def gap(self):
        start, y = self.marks
        while self.queue and self.queue[0][0] < self.now:
            t, _, lane, gen = self.queue.pop(0)
            if gen is None:
                if lane.link is not None:
                    self.gates.append(lane.link)
                continue
            r = max(t - start, 0) // 8 * 8
            lane.token = y[r:r + 8] if lane.link is None else y[r:r + 8] + lane.link
            lane.link = None
            next(gen)


def _run(job):
    fn, args, _ = job
    for _ in fn(_Lane(), *args):
        pass


def _job(costs):
    def wrap(fn):
        return lambda *a: (fn, a, costs(*a) if callable(costs) else costs)
    return wrap


def _mm7(wv, lhs, rhs, emit):
    def m(i):
        return wv.dot(lhs(i), rhs(i))
    c11 = c22 = m(0)
    wv.gap()
    c21 = m(1)
    c22 = c22 - c21
    wv.gap()
    t = m(2)
    emit(1, 0, c21 + t)
    c11 = c11 + t
    wv.gap()
    c11 = c11 + m(3)
    wv.gap()
    c12 = m(4)
    emit(0, 0, c11 - c12)
    wv.gap()
    t = m(5)
    emit(0, 1, c12 + t)
    c22 = c22 + t
    wv.gap()
    emit(1, 1, c22 + m(6))
    wv.gap()


def _kernel(x_hbm, aq_hbm, ao_hbm, bq_hbm, bo_hbm, out_hbm,
            x_raw, aq_raw, w_raw, tmp, wt,
            aq0, aq1, aq2, aq3, wb,
            x_t, xs, o_t,
            qb, kb, vb, vfirst,
            bq_s, bk_s, bv_s, s0, s1,
            sem_x, sem_aq, sem_w, sem_o):
    aq_w, sbuf = (aq0, aq1, aq2, aq3), (s0, s1)

    def x_copy(ct):
        return pltpu.make_async_copy(x_hbm.at[:, _ds(ct, 128)], x_raw.at[ct], sem_x.at[ct])

    def aq_copy(g, t):
        return pltpu.make_async_copy(aq_hbm.at[:, _ds(4 * t + g, 256)], aq_raw.at[:, _ds(4 * t + g, 256)],
                                     sem_aq.at[4 * t + g])

    def w_copy(i):
        src, lo = ((ao_hbm, WAO), (bq_hbm, WBQ), (bo_hbm, WBO))[i]
        return pltpu.make_async_copy(src, w_raw.at[:, pl.ds(lo * D, src.shape[1])], sem_w.at[i])

    def out_copy(ct):
        return pltpu.make_async_copy(x_raw.at[ct], out_hbm.at[:, _ds(ct, 128)], sem_o.at[ct])

    def load_x(ct):
        tmp[pl.ds(0, S // 2), :] = _pack(x_raw[ct])
        for c in range(8):
            lo, hi = _halves(tmp[pl.ds(c, 128, stride=8), :].T)
            x_t[c, _ds(ct, 128), :] = lo
            x_t[8 + c, _ds(ct, 128), :] = hi

    @_job([1] * 8)
    def store_x1(ln, ct):
        for c in range(8):
            lo = lax.bitcast_convert_type(x_t[c, _ds(ct, 128), :].astype(BF).astype(F32), U32)
            hi = lax.bitcast_convert_type(x_t[8 + c, _ds(ct, 128), :].astype(BF).astype(F32), U32)
            tmp[pl.ds(ct // 4 * D + c, 128, stride=8), :] = ln.follow((lo >> 16) | hi).T
            yield

    @_job([1] * 32)
    def store_x2(ln, ct):
        for r in range(32):
            w = tmp[pl.ds(ct // 4 * D + r * 32, 32), :]
            if ln.token is not None:
                w = _after(w, jnp.tile(ln.token, (4, 1)))
            x_raw[ct, _ds(r, 64), :] = _unpack(w)
            if r == 31:
                out_copy(ct).start()
            yield

    def head_major(ln, base, dp):
        return jnp.concatenate(_halves(ln.follow(tmp[pl.ds(base + dp, 8, stride=16), :])), axis=0)

    @_job([1] * 24)
    def prep_aq1(ln, g):
        for n in range(3):
            for kt in range(8):
                w = _pack(aq_raw[_ds(kt, 128), _ds(4 * ((n + 1) % 3) + g, 256)])
                tmp[pl.ds(n * D + kt * 128, 128), :] = _pack(_unpack(ln.follow(w)).T)
                yield

    @_job([30] * 96)
    def prep_aq2(ln, g):
        for n in range(3):
            for dp in range(8):
                for k in range(4):
                    a = [head_major(ln, n * D + (k + 4 * kh) * 128, dp + 8 * h) for h in range(2) for kh in range(2)]
                    ln.put(_lhs7(*a), aq_w[g],
                           [(pl.ds(i * 192 + n * 64 + dp * 8, 8), _ds(k, 128)) for i in range(7)])
                    yield

    @_job([16] * 128)
    def permute_ao(ln):
        tmp[...] = jnp.concatenate([_pack(w_raw[:, _ds(8 * WAO + ct, 128)]) for ct in range(8)], axis=0)
        for ct in range(8):
            for r in range(16):
                w = jnp.concatenate([head_major(ln, ct * 512 + r // 4 * 128, 4 * (r % 4) + dp) for dp in range(4)], axis=0)
                ln.put([w], wt, [(pl.ds(512 + r * 32, 32), _ds(ct, 128))])
                yield

    @_job([1] * 32)
    def prep_w1(ln, j):
        for ct in range(8):
            for k in range(4):
                if j == WAO:
                    w = wt[_ds(4 + k, 128), _ds(ct, 128)]
                else:
                    w = _pack(w_raw[_ds(k, 256), _ds(8 * j + ct, 128)])
                wt[_ds(ct, 64), _ds(k, 256)] = _pack(_unpack(ln.follow(w)).T)
                yield

    @_job([24] * 128)
    def prep_w2(ln, j):
        for r in range(32):
            for k in range(4):
                a = [_unpack(ln.follow(wt[_ds(32 * h + r, 8), _ds(4 * kh + k, 128)])).astype(F32)
                     for h in range(2) for kh in range(2)]
                ln.put(_lhs7(*a), wb,
                       [(_ds(32 * (7 * j + i) + r, 8), _ds(k, 128)) for i in range(7)])
                yield

    @_job([40] * 16 + [30] * 32)
    def layernorm(ln, p):
        stat = []
        for k in range(2):
            acc = [None, None]
            for r in range(8):
                for n in range(2):
                    x = x_t[2 * p + n, _ds(r, 128), :].reshape(16, 8, 128)
                    if k:
                        x = x - ln.follow(stat[0][n])
                        x = x * x
                    t = x[0] if r == 0 else ln.follow(acc[n]) + x[0]
                    acc[n] = t + jnp.sum(x[1:], axis=0)
                yield
            stat.append([jnp.broadcast_to(jnp.sum(t, axis=0, keepdims=True) * (1.0 / D), (8, 128)) for t in acc])
        rstd = [jnp.tile(lax.rsqrt(v + EPS), (2, 1)) for v in stat[1]]
        for r in range(32):
            m = [jnp.tile(ln.follow(t), (2, 1)) for t in stat[0]]
            b = _rhs7(*[(x_t[2 * p + n, pl.ds(h * 512 + r * 16, 16), :] - m[n]) * rstd[n]
                        for h in range(2) for n in range(2)])
            for i in range(7):
                xs[_ds(32 * p + r, 8), _ds(i, 128)] = _pack(b[i])
            yield

    def o_operands(p):
        return [t.astype(BF) for t in _rhs7(*[o_t[2 * p + n, _ds(h, 512), :] for h in range(2) for n in range(2)])]

    def out_proj(pc, j, p):
        def emit(mh, nh, y):
            x_t[2 * p + nh, _ds(mh, 512), :] += y
        rhs = o_operands(p)
        _mm7(pc, lambda i: wb[_ds(7 * j + i, 256), :], lambda i: rhs[i], emit)

    def a_qkv(wv, g, e):
        lane0 = lax.broadcasted_iota(jnp.int32, (128, 128), 1) == 0
        first = {}
        par = g % 2

        def emit(p, mh, nh, y):
            c, rows = 2 * p + nh, _ds(mh, 128)
            k, v, q = y[:128], y[128:256], y[256:]
            kb[par, rows, _ds(7 + c, 128)] = k
            vb[par, rows, _ds(7 + c, 128)] = v
            qb[par, rows, _ds(c, 128)] = q
            if c == 0:
                if e == 0:
                    vfirst[g, rows, :] = v
                first[mh] = v if e == 0 else vfirst[g, rows, :]
            else:
                kb[par, rows, _ds(c - 1, 128)] = pltpu.roll(k, 1, 1)
                vb[par, rows, _ds(c - 1, 128)] = jnp.where(lane0, first[mh], pltpu.roll(v, 1, 1))

        for p in range(4):
            _mm7(wv, lambda i: aq_w[g][_ds(i, 192), :], lambda i: _unpack(xs[_ds(4 * e + p, 256), _ds(i, 128)]), lambda mh, nh, y: emit(p, mh, nh, y))

    nq, nd = CFG.get("nq", 4), CFG.get("nd", 4)

    @_job(lambda g, e, tiles: ([8 * nq] * (DH // nq - 1) + [CFG.get('sm', 30)] * 4 + [8 * nd] * (DH // nd)) * len(tiles))
    def a_attn(ln, g, e, tiles):
        par = g % 2
        lane0 = lax.broadcasted_iota(jnp.int32, (8, 128), 1) == 0
        for c in tiles:
            win = pl.ds(c * 128, WIN * 128)
            acc = None
            for r in range(DH // nq):
                t = jnp.tile(qb[par, _ds(r, 8 * nq), _ds(c, 128)], (1, WIN)) * kb[par, _ds(r, 8 * nq), win]
                for d in range(nq):
                    acc = t[:8] if acc is None else acc + t[8 * d:8 * d + 8]
                acc = ln.follow_all(acc)
                yield
            logit = []
            for w in range(WIN):
                t = acc[:, w * 128:(w + 1) * 128] * QSCALE
                logit.append(jnp.where(lane0, MASKED, t) if c + w < 7 else t)
            m = logit[0]
            for t in logit[1:]:
                m = jnp.maximum(m, t)
            m = ln.follow(m)
            yield
            p = [jnp.exp2(t - m) for t in logit]
            l = p[0]
            for t in p[1:]:
                l = l + t
            l = ln.follow(l)
            yield
            r = ln.follow(1.0 / l)
            yield
            p = [t * r for t in p]
            for h in range(DH // nd):
                t = jnp.tile(jnp.concatenate([ln.follow(p[0])] + p[1:], axis=1), (nd, 1)) * vb[par, _ds(h, 8 * nd), win]
                o = t[:, :128]
                for w in range(1, WIN):
                    o = o + t[:, w * 128:(w + 1) * 128]
                o_t[8 * e + c, _ds(g * (DH // nd) + h, 8 * nd), :] = o
                yield

    def a_layer(first):
        for u in range(8):
            if not on(f"a{u}"):
                continue
            pc = _Pace()
            if u:
                jobs = [a_attn((u - 1) % 4, (u - 1) // 4, range(8))]
            else:
                jobs = [layernorm(p) for p in range(4 if first else 7, 8)]
            if first and u < 3:
                for t in range(3):
                    aq_copy(u + 1, t).wait()
                pc.spread(0, CFG.get("tr", 5000), prep_aq1(u + 1))
                jobs.append(prep_aq2(u + 1))
            elif first:
                j = (WBQ, WBK, WBV, WAO, WBO)[u - 3]
                if u in (3, 5, 7):
                    w_copy({3: 1, 5: 0, 7: 2}[u]).wait()
                if u == 5:
                    jobs.append(permute_ao())
                pc.spread(0, CFG.get("tr", 5000), prep_w1(j))
                jobs.append(prep_w2(j))
            pc.spread(0, 10200, *jobs)
            a_qkv(pc, u % 4, u // 4)
        for p in range(8):
            if not on(f"ao{p // 4 + 1}"):
                continue
            pc = _Pace()
            jobs = [layernorm(p - 1)] if p else []
            if p < 6:
                jobs.append(a_attn(3, 1, range(p + 2 if p else 0, p + 3)))
            pc.spread(0, 3500 if p != 5 else 3000, *jobs)
            out_proj(pc, WAO, p)

    def b_qkv(wv, p):
        kt = {}

        def emit_k(mh, nh, y):
            kt[mh, nh] = y.astype(BF)
            if nh == 1:
                k = jnp.concatenate([kt[mh, 0], kt[mh, 1]], axis=1)
                for g in range(4):
                    bk_s[4 * mh + g, _ds(p, 128), :] = _pack(k[g * 128:(g + 1) * 128].T)

        def emit_q(mh, nh, y):
            bq_s[_ds(mh, 256), _ds(2 * p + nh, 128)] = _pack(y * QSCALE)

        def emit_v(mh, nh, y):
            bv_s[_ds(mh, 256), _ds(2 * p + nh, 128)] = _pack(y)

        for j, emit in ((WBK, emit_k), (WBQ, emit_q), (WBV, emit_v)):
            _mm7(wv, lambda i: wb[_ds(7 * j + i, 256), :], lambda i: _unpack(xs[_ds(p, 256), _ds(i, 128)]), emit)

    def b_steps(i, t_lo, t_hi, state, qk_end=None):
        m_old, m_new, m_run, l, acc = state
        ms = {t_lo // NC - 2: m_old, t_lo // NC - 1: m_new}
        nsub, off, stride = CFG.get("nsub", 4), CFG.get("off", -8), CFG.get("stride", 24)
        marks = {}
        later = []

        def mark(t, row):
            t, row = t + row // KC, row % KC
            return marks[t][row:row + 8, :128] if t in marks else None

        def pace(x, t, row):
            tok = mark(t, row)
            return x if tok is None else _after(x, jnp.tile(tok, (x.shape[0] // 8, x.shape[1] // 128)))

        for t in range(t_lo, t_hi):
            u, c = divmod(t, NC)
            s = None
            if qk_end is None or t < qk_end:
                n, h = i + u // 4, u % 4
                g, blk = n % 8, n // 8
                q = [_unpack(bq_s[_ds(4 * g + h, 16), _ds(blk, NQ)])]
                if h > 0:
                    q.insert(0, jnp.zeros((DH * h, NQ), BF))
                if h < 3:
                    q.append(jnp.zeros((DH * (3 - h), NQ), BF))
                s = marks[t] = _dot(_unpack(bk_s[g, _ds(c, KC // 2), :]), jnp.concatenate(q, axis=0))
            for f in later:
                f(t)
            later = []
            up, cp = divmod(t - NC - LAG, NC)
            if up >= 0:
                n, h = i + up // 4, up % 4
                g, blk = n % 8, n // 8
                rows = KC // nsub
                p = []
                for j in range(nsub):
                    m = pace(ms[up], t - 1, off + stride * j)
                    z = sbuf[up % 2][pl.ds((cp + 1) * KC - (j + 1) * rows, rows), :].reshape(rows // 8, 8, NQ)
                    e = jnp.exp2(z - m)
                    fresh = cp == 0 and j == 0
                    l = e[0] if fresh else (pace(l, t - 1, off + stride * j) if CFG.get("pl", 0) else l) + e[0]
                    l = l + jnp.sum(e[1:], axis=0)
                    p.insert(0, e.reshape(rows, NQ))
                a = _dot(_unpack(bv_s[_ds(4 * g + h, 16), _ds(cp, KC)]), jnp.concatenate(p, axis=0).astype(BF))
                acc = a if cp == 0 else acc + a
                if cp == NC - 1:
                    def finish(t, l=l, acc=acc, row=4 * g + h, blk=blk):
                        l = pace(jnp.broadcast_to(jnp.sum(l, axis=0, keepdims=True), (8, NQ)), t - 1, CFG.get("f1", 48))
                        o = acc * jnp.tile(pace(1.0 / l, t - 1, CFG.get("f2", 112)), (DH // 8, 1))
                        for n in range(NQ // 128):
                            o_t[blk * (NQ // 128) + n, _ds(row, DH), :] = o[:, n * 128:(n + 1) * 128]
                    finish(t + 1)
            if s is not None:
                sbuf[u % 2][_ds(c, KC), :] = s
                mx = jnp.max(s.reshape(KC // 8, 8, NQ), axis=0)
                m_run = mx if c == 0 else jnp.maximum(m_run, mx)
                if c == NC - 1:
                    ms[u] = jnp.broadcast_to(jnp.max(m_run, axis=0, keepdims=True), (8, NQ))
        zero = jnp.zeros((8, NQ), F32)
        return ms.get(t_hi // NC - 2, zero), ms.get(t_hi // NC - 1, zero), m_run, l, acc

    def b_layer():
        if on("bq1"):
            pc = _Pace()
            pc.spread(0, 3000, layernorm(7))
            b_qkv(pc, 0)

        def body(p, c):
            b_qkv(_Pace(), p)
            return c

        if on("bq2"):
            lax.fori_loop(1, 8, body, 0)
        if on("battn"):
            zero = jnp.zeros((8, NQ), F32)
            n_iter = (D // DH) * (S // NQ) // 4
            state = b_steps(0, 0, T0, (zero, zero, zero, zero, jnp.zeros((DH, NQ), F32)))
            state = lax.fori_loop(0, n_iter - 1, lambda i, st: b_steps(i, T0, T0 + 4 * NC, st), state)
            b_steps(n_iter - 1, T0, 5 * NC + LAG, state, qk_end=4 * NC)

    if on("start"):
      with jax.named_scope("P0_start"):
        order = [x_copy(ct) for ct in range(8)] + [aq_copy(0, t) for t in (1, 2, 0)]
        for cp in order[:3]:
            cp.start()
        for ct in range(8):
            order[ct].wait()
            order[ct + 3].start()
            load_x(ct)
        for p in range(4):
            _run(layernorm(p))
        for cp in order[8:]:
            cp.wait()
        for g in range(1, 4):
            for t in range(3):
                aq_copy(g, t).start()
        _run(prep_aq1(0))
        _run(prep_aq2(0))
        for i in (1, 0, 2):
            w_copy(i).start()

    with jax.named_scope("P1_a"):
        a_layer(CFG.get('first', True))
    with jax.named_scope("P2_b"):
        b_layer()
    if on("bo"):
      with jax.named_scope("P3_bo"):
        for p in range(8):
            pc = _Pace()
            if p:
                pc.spread(0, 3500, layernorm(p - 1))
            out_proj(pc, WBO, p)
    if PH == "all":
        with jax.named_scope("P4_a"):
            a_layer(False)
        with jax.named_scope("P5_b"):
            b_layer()

    if on("final"):
      with jax.named_scope("P6_final"):
        rhs = [o_operands(p) for p in range(8)]
        for r in range(4):
            pc = _Pace()
            if r:
                pc.spread(0, 3000, store_x1(r - 1), store_x1(r + 3))
                pc.spread(3500, 6500, store_x2(r - 1), store_x2(r + 3))
            for p in range(8):
                def emit(mh, nh, y):
                    x_t[2 * p + nh, _ds(4 * mh + r, 128), :] += y
                _mm7(pc, lambda i: wb[_ds(4 * (7 * WBO + i) + r, 64), :], lambda i: rhs[p][i], emit)
        for job in (store_x1(7), store_x1(3), store_x2(7), store_x2(3)):
            _run(job)
        for ct in range(8):
            out_copy(ct).wait()
    else:
        def keep(i, c):
            for r_ in (x_t, o_t, qb, kb, vb):
                s0[pl.ds(0, 8), pl.ds(0, 128)] += r_[i, pl.ds(0, 8), pl.ds(0, 128)]
            for r_ in (bk_s,):
                tmp[pl.ds(0, 8), :] |= r_[i, pl.ds(0, 8), pl.ds(0, 128)]
            for r_ in (bq_s, bv_s, xs, wb, aq0, aq1, aq2, aq3):
                tmp[pl.ds(0, 8), :] |= r_[_ds(i, 8), pl.ds(0, 128)]
            return c
        lax.fori_loop(0, 2, keep, 0)
        x_raw[0, pl.ds(0, 16), :] = _unpack(tmp[pl.ds(0, 8), :] | lax.bitcast_convert_type(s0[pl.ds(0, 8), pl.ds(0, 128)], U32))
        out_copy(0).start(); out_copy(0).wait()


@jax.jit
def pallas_interleave_layers__sliding_local_dilated__softmax_full_mha__prompt_kernel(
    A_x: jax.Array,
    A_wqkv: jax.Array,
    A_wo: jax.Array,
    B_x: jax.Array,
    B_wqkv: jax.Array,
    B_wo: jax.Array,
):
    del B_x
    vmem = pltpu.VMEM
    scratch = [
        vmem((8, S, 128), BF), vmem((D, 3 * D), BF), vmem((D, 5 * D), BF), vmem((4 * D, 128), U32), vmem((D, D), U32),
        *[vmem((7 * 192, D // 2), U32)] * 4, vmem((5 * 7 * 256, D // 2), U32),
        vmem((16, D, 128), F32), vmem((8 * 256, 7 * 128), U32), vmem((16, D, 128), F32),
        vmem((2, 256, 8 * 128), F32), vmem((2, 256, 15 * 128), F32), vmem((2, 256, 15 * 128), F32),
        vmem((4, 256, 128), F32),
        vmem((D // 2, S), U32), vmem((8, S // 2, 128), U32), vmem((D // 2, S), U32),
        vmem((S, NQ), F32), vmem((S, NQ), F32),
        pltpu.SemaphoreType.DMA((8,)), pltpu.SemaphoreType.DMA((12,)),
        pltpu.SemaphoreType.DMA((3,)), pltpu.SemaphoreType.DMA((8,)),
    ]
    out = pl.pallas_call(
        _kernel,
        out_shape=jax.ShapeDtypeStruct((S, D), A_x.dtype),
        in_specs=[pl.BlockSpec(memory_space=pl.ANY)] * 5,
        out_specs=pl.BlockSpec(memory_space=pl.ANY),
        scratch_shapes=scratch,
        compiler_params=pltpu.CompilerParams(vmem_limit_bytes=124 * 1024 * 1024),
        name="interleaved_attention_layers",
    )(A_x.reshape(S, D), A_wqkv, A_wo, B_wqkv, B_wo)
    return out.reshape(A_x.shape)
```

```python
import math

import jax
import jax.numpy as jnp
import numpy as np
from jax import lax
import jax.experimental.pallas as pl
import jax.experimental.pallas.tpu as pltpu

S = 2048
D = 1024
DH = 32
WIN = 8
EPS = 1e-5
LOG2E = math.log2(math.e)
QSCALE = DH ** -0.5 * LOG2E
MASKED = -1e9 * LOG2E

NQ = 512
KC = 128
NC = S // KC
LAG = 3
T0 = 24

BF = jnp.bfloat16
F32 = jnp.float32
U32 = jnp.uint32
WAO, WBQ, WBK, WBV, WBO = range(5)
PH = "all"
def on(p): return PH == "all" or p in PH.split(",")
CFG = {}


def _pack(x):
    return pltpu.bitcast(x.astype(BF), U32)


def _unpack(x):
    return pltpu.bitcast(x, BF)


def _halves(w):
    lo = lax.bitcast_convert_type(w << 16, F32)
    hi = lax.bitcast_convert_type(w & np.uint32(0xFFFF0000), F32)
    return lo, hi


def _ds(i, n):
    if isinstance(i, int):
        return pl.ds(i * n, n)
    return pl.ds(pl.multiple_of(i * n, n), n)


def _dot(a, b):
    return jnp.dot(a, b, preferred_element_type=F32)


def _after(x, token):
    if token is None:
        return x
    token = jnp.tile(token, (x.shape[0] // 8, x.shape[1] // 128))
    return jnp.where(token < -jnp.inf, jnp.zeros_like(x), x)


class _Lane:
    token = None

    def __call__(self, x):
        return _after(x, self.token)

    def head(self, x):
        return x if self.token is None else jnp.concatenate([self(x[:8]), x[8:]], axis=0)


class _Pace:
    def __init__(self):
        self.now, self.queue = 0, []

    def spread(self, lo, hi, *jobs):
        lane = _Lane()
        total = sum(sum(costs) for _, _, costs in jobs)
        done = 0
        for fn, args, costs in jobs:
            gen = fn(lane, *args)
            for cost in costs:
                self.queue.append((lo + (hi - lo) * done // total, len(self.queue), lane, gen))
                done += cost
        self.queue.sort(key=lambda e: e[:2])

    def matmul(self, lhs, rhs):
        y = None
        for k in range(2):
            part = _dot(_unpack(lhs(k)), _unpack(rhs(k)))
            start, self.now = self.now, self.now + part.shape[0]
            while self.queue and self.queue[0][0] < self.now:
                t, _, lane, gen = self.queue.pop(0)
                row = (t - start) // 8 * 8
                lane.token = part[row:row + 8]
                next(gen)
            y = part if y is None else y + part
        return y


def _run(job):
    fn, args, _ = job
    for _ in fn(_Lane(), *args):
        pass


def _job(costs):
    def wrap(fn):
        return lambda *a: (fn, a, costs(*a) if callable(costs) else costs)
    return wrap


def _kernel(x_hbm, aq_hbm, ao_hbm, bq_hbm, bo_hbm, out_hbm,
            x_raw, aq_raw, w_raw, tmp, xtmp, ao_perm,
            aq_t, w_t, x_t, xn_t, o_t,
            qb, kb, vb, vfirst,
            bq_s, bk_s, bv_s, s0, s1,
            sem_x, sem_aq, sem_w, sem_o):
    sbuf = (s0, s1)

    def x_copy(h, j):
        return pltpu.make_async_copy(x_hbm.at[:, h, :, _ds(j, 256)], x_raw.at[h, :, :, _ds(j, 256)],
                                     sem_x.at[4 * h + j])

    def aq_copy(g, t):
        return pltpu.make_async_copy(aq_hbm.at[:, _ds(4 * t + g, 256)], aq_raw.at[:, _ds(4 * t + g, 256)],
                                     sem_aq.at[4 * t + g])

    def w_copy(i):
        src, lo = ((ao_hbm, WAO), (bq_hbm, WBQ), (bo_hbm, WBO))[i]
        return pltpu.make_async_copy(src, w_raw.at[:, pl.ds(lo * D, src.shape[1])], sem_w.at[i])

    def out_copy(h, ct):
        return pltpu.make_async_copy(x_raw.at[h, :, :, _ds(ct, 128)], out_hbm.at[:, h, :, _ds(ct, 128)],
                                     sem_o.at[8 * h + ct])

    def dma(starts, waits):
        for cp in starts:
            cp.start()
        for cp in waits:
            cp.wait()

    @_job([1] * 5)
    def load_x(ln, h, ct):
        w = _pack(x_raw[h, :, :, _ds(ct, 128)].reshape(S // 2, 128))
        xtmp[_ds(ct, 512), :] = ln(w)
        yield
        for c in range(4):
            lo, hi = _halves(ln.head(xtmp[pl.ds(ct * 512 + c, 128, stride=4), :]).T)
            x_t[4 * h + c, _ds(ct, 128), :] = lo
            x_t[8 + 4 * h + c, _ds(ct, 128), :] = hi
            yield

    @_job([1])
    def store_x1(ln, ct, c):
        lo = lax.bitcast_convert_type(x_t[c, _ds(ct, 128), :].astype(BF).astype(F32), U32)
        hi = lax.bitcast_convert_type(x_t[8 + c, _ds(ct, 128), :].astype(BF).astype(F32), U32)
        (xtmp, tmp)[c // 4][pl.ds(ct * 512 + c % 4, 128, stride=4), :] = ln.head((lo >> 16) | hi).T
        yield

    @_job([1] * 8)
    def store_x2(ln, ct, h):
        for r in range(8):
            w = ln((xtmp, tmp)[h][pl.ds(ct * 512 + r * 64, 64), :])
            x_raw[h, _ds(r, 16), :, _ds(ct, 128)] = _unpack(w).reshape(16, 8, 128)
            if r == 7:
                out_copy(h, ct).start()
            yield

    def head_major(ln, base, dp, n):
        lo, hi = _halves(ln(tmp[pl.ds(base + dp, 8 * n, stride=16), :]))
        return jnp.concatenate([lo.reshape(n, 8, 128), hi.reshape(n, 8, 128)], axis=1)

    @_job([1] * 8)
    def prep_aq1(ln, g, n):
        for kt in range(8):
            w = _pack(aq_raw[_ds(kt, 128), _ds(4 * ((n + 1) % 3) + g, 256)])
            tmp[pl.ds(n * D + kt * 128, 128), :] = _pack(_unpack(ln.head(w)).T)
            yield

    @_job([40] * 16)
    def prep_aq2(ln, g, n):
        for dp in range(16):
            w = head_major(ln, n * D, dp, 8)
            aq_t[_ds(16 * (3 * g + n) + dp, 8), :] = _pack(jnp.concatenate([w[kt] for kt in range(8)], axis=1))
            yield

    @_job([40] * 72)
    def permute_ao(ln):
        for g in range(4):
            for half in range(2):
                w = [_pack(w_raw[_ds(g, 256), _ds(8 * WAO + 4 * half + ct, 128)]) for ct in range(4)]
                tmp[_ds(2 * g + half, 512), :] = ln(jnp.concatenate(w, axis=0))
                yield
            for dp in range(16):
                w = head_major(ln, g * D, dp, 8)
                ao_perm[_ds(16 * g + dp, 8), :] = _pack(jnp.concatenate([w[ct] for ct in range(8)], axis=1))
                yield

    @_job([1] * 32)
    def prep_w(ln, j):
        for ct in range(8):
            for k in range(4):
                if j == WAO:
                    w = ao_perm[_ds(k, 128), _ds(ct, 128)]
                else:
                    w = _pack(w_raw[_ds(k, 256), _ds(8 * j + ct, 128)])
                w_t[_ds(8 * j + ct, 64), _ds(k, 256)] = _pack(_unpack(ln.head(w)).T)
                yield

    @_job([40] * 10 + [30] * 8)
    def layernorm(ln, tile):
        stat = []
        for k in range(2):
            for r in range(4):
                x = x_t[tile, _ds(r, 256), :].reshape(16, 16, 128)
                if k:
                    x = x - ln(stat[0])
                    x = x * x
                acc = ln(jnp.sum(x, axis=0) if r == 0 else acc + jnp.sum(x, axis=0))
                yield
            t = jnp.broadcast_to(jnp.sum(acc, axis=0, keepdims=True) * (1.0 / D), (16, 128))
            stat.append(ln(lax.rsqrt(t + EPS) if k else t))
            yield
        for r in range(8):
            x = (x_t[tile, _ds(r, 128), :].reshape(8, 16, 128) - ln(stat[0])) * stat[1]
            xn_t[_ds(r, 64), _ds(tile, 128)] = _pack(x.reshape(128, 128))
            yield

    def project(pc, w_ref, row, words, src, tile):
        return pc.matmul(lambda k: w_ref[_ds(row, words), _ds(k, 512)], lambda k: src[_ds(k, 256), _ds(tile, 128)])

    def out_proj(pc, j, tile):
        for r in range(4):
            x_t[tile, _ds(r, 256), :] += project(pc, w_t, 4 * j + r, 128, o_t, tile)

    def a_qkv(pc, g, e, c):
        par = g % 2
        k = project(pc, aq_t, 3 * g, 128, xn_t, 8 * e + c)
        kb[par, :, _ds(7 + c, 128)] = k
        if c:
            kb[par, :, _ds(c - 1, 128)] = pltpu.roll(k, 1, 1)
        v = project(pc, aq_t, 3 * g + 1, 128, xn_t, 8 * e + c)
        vb[par, :, _ds(7 + c, 128)] = v
        if c:
            lane0 = lax.broadcasted_iota(jnp.int32, (256, 128), 1) == 0
            vb[par, :, _ds(c - 1, 128)] = jnp.where(lane0, vfirst[g], pltpu.roll(v, 1, 1))
        elif e == 0:
            vfirst[g] = v
        qb[par, :, _ds(c, 128)] = project(pc, aq_t, 3 * g + 2, 128, xn_t, 8 * e + c)

    nq, nd = CFG.get("nq", 4), CFG.get("nd", 4)

    @_job([8 * nq] * (DH // nq - 1) + [30] * 4 + [8 * nd] * (DH // nd))
    def a_attn(ln, g, e, c):
        par = g % 2
        win = pl.ds(c * 128, WIN * 128)
        for r in range(DH // nq):
            t = jnp.tile(qb[par, _ds(r, 8 * nq), _ds(c, 128)], (1, WIN)) * kb[par, _ds(r, 8 * nq), win]
            t = jnp.sum(t.reshape(nq, 8, WIN * 128), axis=0)
            acc = ln(t if r == 0 else acc + t)
            yield
        lane0 = lax.broadcasted_iota(jnp.int32, (8, 128), 1) == 0
        logit = []
        for w in range(WIN):
            t = acc[:, w * 128:(w + 1) * 128] * QSCALE
            logit.append(jnp.where(lane0, MASKED, t) if c + w < 7 else t)
        m = logit[0]
        for t in logit[1:]:
            m = jnp.maximum(m, t)
        m = ln(m)
        yield
        p = [jnp.exp2(t - m) for t in logit]
        l = ln(sum(p[1:], p[0]))
        yield
        r = ln(1.0 / l)
        yield
        p = [t * r for t in p]
        for h in range(DH // nd):
            t = jnp.tile(jnp.concatenate([ln(p[0])] + p[1:], axis=1), (nd, 1)) * vb[par, _ds(h, 8 * nd), win]
            o = sum([t[:, w * 128:(w + 1) * 128] for w in range(1, WIN)], t[:, :128])
            o_t[_ds(g * (DH // nd) + h, 4 * nd), _ds(8 * e + c, 128)] = _pack(o)
            yield

    def a_layer(first):
        def slab(g):
            return [aq_copy(g, t) for t in range(3)]

        for u in range(8):
            if not on(f"a{u}"):
                continue
            pc = _Pace()
            jobs = [a_attn((u - 1) % 4, (u - 1) // 4, c) for c in range(8)] if u else []
            if not first:
                if u == 0:
                    pc.spread(0, 2000, layernorm(15))
            elif u == 0:
                for c in (0, 1, 2, 4, 5, 6):
                    pc.spread(1536 * c, 1536 * c + 1200, layernorm(c + 1))
                pc.spread(3072, 4900, *[load_x(1, ct) for ct in range(8)])
                pc.spread(5150, 5900, layernorm(4))
                pc.spread(6144, 8500, *[prep_aq1(1, n) for n in range(3)])
                pc.spread(8800, 12000, *[prep_aq2(1, n) for n in range(3)])
            elif u < 3:
                if u == 1:
                    dma([w_copy(i) for i in range(3)], slab(2) + slab(3))
                pc.spread(0, 6000, *[prep_aq1(u + 1, n) for n in range(3)])
                jobs += [layernorm(5 + 3 * u + n) for n in range(3)] + [prep_aq2(u + 1, n) for n in range(3)]
            else:
                if u == 3:
                    dma([], [w_copy(i) for i in range(3)])
                    jobs += [layernorm(14), layernorm(15)]
                if u == 4:
                    jobs.append(permute_ao())
                pc.spread(0, 11500, prep_w((WBQ, WBK, WAO, WBV, WBO)[u - 3]))
            if jobs:
                pc.spread(0, 12000, *jobs)
            for c in range(8):
                if first and u == 0 and c == 2:
                    dma([], [x_copy(1, j) for j in range(4)])
                if first and u == 0 and c == 4:
                    dma(slab(2) + slab(3), slab(1))
                a_qkv(pc, u % 4, u // 4, c)
        for tile in range(16):
            if not on(f"ao{tile // 8 + 1}"):
                continue
            pc = _Pace()
            pc.spread(0, 2000, *([layernorm(tile - 1)] if tile else []), *([a_attn(3, 1, tile)] if tile < 8 else []))
            out_proj(pc, WAO, tile)

    def b_qkv(pc, p):
        for r in range(4):
            k = jnp.concatenate([project(pc, w_t, 4 * WBK + r, 128, xn_t, 2 * p + n).astype(BF) for n in range(2)], axis=1)
            for g in range(2):
                bk_s[_ds(p, 128), _ds(2 * r + g, 128)] = _pack(k[g * 128:(g + 1) * 128].T)
        for n in range(2):
            for r in range(4):
                bq_s[_ds(r, 128), _ds(2 * p + n, 128)] = _pack(project(pc, w_t, 4 * WBQ + r, 128, xn_t, 2 * p + n) * QSCALE)
            for r in range(4):
                bv_s[_ds(r, 128), _ds(2 * p + n, 128)] = _pack(project(pc, w_t, 4 * WBV + r, 128, xn_t, 2 * p + n))

    def b_steps(i, t_lo, t_hi, state, qk_end=None):
        m_old, m_new, m_run, l, acc = state
        ms = {t_lo // NC - 2: m_old, t_lo // NC - 1: m_new}
        scores = {}

        def pace(x, t, row):
            t, row = t + row // KC, row % KC
            return _after(x, scores[t][row:row + 8, :128]) if t in scores else x

        def where(u):
            n = i + u // 4
            return n % 8, (u + 3) % 4, n // 8

        for t in range(t_lo, t_hi):
            u, c = divmod(t, NC)
            if qk_end is None or t < qk_end:
                g, h, blk = where(u)
                q = [_unpack(bq_s[_ds(4 * g + h, 16), _ds(blk, NQ)])]
                if h > 0:
                    q.insert(0, jnp.zeros((DH * h, NQ), BF))
                if h < 3:
                    q.append(jnp.zeros((DH * (3 - h), NQ), BF))
                scores[t] = _dot(_unpack(bk_s[_ds(c, KC // 2), _ds(g, 128)]), jnp.concatenate(q, axis=0))
            up, cp = divmod(t - NC - LAG, NC)
            if up >= 0:
                g, h, blk = where(up)
                p = []
                for j in range(4):
                    z = sbuf[up % 2][_ds(4 * cp + 3 - j, KC // 4), :].reshape(KC // 32, 8, NQ)
                    e = jnp.exp2(z - pace(ms[up], t - 1, 24 * j - 8))
                    l = jnp.sum(e, axis=0) if cp == 0 and j == 0 else l + jnp.sum(e, axis=0)
                    p.insert(0, e.reshape(KC // 4, NQ))
                a = _dot(_unpack(bv_s[_ds(4 * g + h, 16), _ds(cp, KC)]), jnp.concatenate(p, axis=0).astype(BF))
                acc = a if cp == 0 else acc + a
                if cp == NC - 1:
                    total = pace(jnp.broadcast_to(jnp.sum(l, axis=0, keepdims=True), (8, NQ)), t, 48)
                    o = acc * jnp.tile(pace(1.0 / total, t, 112), (DH // 8, 1))
                    o_t[_ds(4 * g + h, 16), _ds(blk, NQ)] = _pack(o)
            if t in scores:
                sbuf[u % 2][_ds(c, KC), :] = scores[t]
                mx = jnp.max(scores[t].reshape(KC // 8, 8, NQ), axis=0)
                m_run = mx if c == 0 else jnp.maximum(m_run, mx)
                if c == NC - 1:
                    ms[u] = jnp.broadcast_to(jnp.max(m_run, axis=0, keepdims=True), (8, NQ))
        zero = jnp.zeros((8, NQ), F32)
        return ms.get(t_hi // NC - 2, zero), ms.get(t_hi // NC - 1, zero), m_run, l, acc

    def b_layer():
        if on("bq1"):
            pc = _Pace()
            pc.spread(0, 2000, layernorm(15))
            b_qkv(pc, 0)
        if on("bq2"):
            lax.fori_loop(1, 8, lambda p, c: b_qkv(_Pace(), p), None)
        if on("battn"):
            zero = jnp.zeros((8, NQ), F32)
            n_iter = (D // DH) * (S // NQ) // 4
            U = CFG.get("U", 1)
            state = b_steps(0, 0, T0, (zero, zero, zero, zero, jnp.zeros((DH, NQ), F32)))
            state = lax.fori_loop(0, (n_iter - 1) // U, lambda i, st: b_steps(U * i, T0, T0 + 4 * U * NC, st), state)
            done = (n_iter - 1) // U * U
            b_steps(done, T0, (4 * (n_iter - done) + 1) * NC + LAG, state, qk_end=4 * (n_iter - done) * NC)

    if on("start"):
      with jax.named_scope("P0_start"):
        dma([x_copy(0, 0), x_copy(0, 1)], [])
        nxt = [x_copy(0, 2), x_copy(0, 3), aq_copy(0, 1), aq_copy(0, 2)]
        for j in range(4):
            dma([nxt[j]], [x_copy(0, j)])
            _run(load_x(0, 2 * j))
            _run(load_x(0, 2 * j + 1))
        dma([aq_copy(0, 0)], [aq_copy(0, 1)])
        _run(layernorm(0))
        _run(prep_aq1(0, 0))
        dma([x_copy(1, 0)], [aq_copy(0, 2)])
        _run(prep_aq1(0, 1))
        _run(prep_aq2(0, 0))
        dma([x_copy(1, 1)], [aq_copy(0, 0)])
        dma([x_copy(1, 2), x_copy(1, 3)] + [aq_copy(1, t) for t in range(3)], [])
        _run(prep_aq1(0, 2))
        _run(prep_aq2(0, 1))
        _run(prep_aq2(0, 2))

    with jax.named_scope("P1_a"):
        a_layer(CFG.get("first", True))
    with jax.named_scope("P2_b"):
        b_layer()
    if on("bo"):
      with jax.named_scope("P3_bo"):
        for tile in range(16):
            pc = _Pace()
            if tile:
                pc.spread(0, 2000, layernorm(tile - 1))
            out_proj(pc, WBO, tile)
    if PH == "all":
        with jax.named_scope("P4_a"):
            a_layer(False)
        with jax.named_scope("P5_b"):
            b_layer()

    if on("final"):
      with jax.named_scope("P6_final"):
        for r in range(4):
            for c in range(8):
                pc = _Pace()
                r1, c1 = divmod(8 * r + c - 1, 8)
                if r1 >= 0:
                    pc.spread(0, 300, store_x1(2 * r1, c1), store_x1(2 * r1 + 1, c1))
                r2, c2 = divmod(8 * r + c - 2, 8)
                if r2 >= 0 and c2 % 4 == 3:
                    pc.spread(0, 1000, store_x2(2 * r2, c2 // 4), store_x2(2 * r2 + 1, c2 // 4))
                for tile in (c, 8 + c):
                    x_t[tile, _ds(r, 256), :] += project(pc, w_t, 4 * WBO + r, 128, o_t, tile)
        for job in (store_x1(6, 7), store_x1(7, 7), store_x2(6, 1), store_x2(7, 1)):
            _run(job)
        dma([], [out_copy(h, ct) for h in range(2) for ct in range(8)])
    else:
        def keep(i, c):
            for r_ in (x_t, qb, kb, vb):
                s0[pl.ds(0, 8), pl.ds(0, 128)] += r_[i, pl.ds(0, 8), pl.ds(0, 128)]
            for r_ in (bq_s, bv_s, bk_s, xn_t, o_t, w_t, aq_t, ao_perm):
                tmp[pl.ds(0, 8), :] |= r_[_ds(i, 8), pl.ds(0, 128)]
            return c
        lax.fori_loop(0, 2, keep, 0)
        x_raw[0, pl.ds(0, 2), :, pl.ds(0, 128)] = _unpack(tmp[pl.ds(0, 8), :] | lax.bitcast_convert_type(s0[pl.ds(0, 8), pl.ds(0, 128)], U32)).reshape(2, 8, 128)
        out_copy(0, 0).start(); out_copy(0, 0).wait()


@jax.jit
def pallas_interleave_layers__sliding_local_dilated__softmax_full_mha__prompt_kernel(
    A_x: jax.Array,
    A_wqkv: jax.Array,
    A_wo: jax.Array,
    B_x: jax.Array,
    B_wqkv: jax.Array,
    B_wo: jax.Array,
):
    del B_x
    vmem = pltpu.VMEM
    scratch = [
        vmem((2, 128, 8, D), BF), vmem((D, 3 * D), BF), vmem((D, 5 * D), BF),
        vmem((4 * D, 128), U32), vmem((4 * D, 128), U32), vmem((D // 2, D), U32),
        vmem((3 * D // 2, D), U32), vmem((5 * D // 2, D), U32),
        vmem((16, D, 128), F32), vmem((D // 2, S), U32), vmem((D // 2, S), U32),
        vmem((2, 256, 8 * 128), F32), vmem((2, 256, 15 * 128), F32), vmem((2, 256, 15 * 128), F32),
        vmem((4, 256, 128), F32),
        vmem((D // 2, S), U32), vmem((S // 2, D), U32), vmem((D // 2, S), U32),
        vmem((S, NQ), F32), vmem((S, NQ), F32),
        pltpu.SemaphoreType.DMA((8,)), pltpu.SemaphoreType.DMA((12,)),
        pltpu.SemaphoreType.DMA((3,)), pltpu.SemaphoreType.DMA((16,)),
    ]
    out = pl.pallas_call(
        _kernel,
        out_shape=jax.ShapeDtypeStruct((128, 2, 8, D), A_x.dtype),
        in_specs=[pl.BlockSpec(memory_space=pl.ANY)] * 5,
        out_specs=pl.BlockSpec(memory_space=pl.ANY),
        scratch_shapes=scratch,
        compiler_params=pltpu.CompilerParams(vmem_limit_bytes=124 * 1024 * 1024),
        name="interleaved_attention_layers",
    )(A_x.reshape(128, 2, 8, D), A_wqkv, A_wo, B_wqkv, B_wo)
    return out.reshape(A_x.shape)
```

```python
import math

import jax
import jax.numpy as jnp
import numpy as np
from jax import lax
import jax.experimental.pallas as pl
import jax.experimental.pallas.tpu as pltpu

S = 2048
D = 1024
DH = 32
WIN = 8
EPS = 1e-5
LOG2E = math.log2(math.e)
QSCALE = DH ** -0.5 * LOG2E
MASKED = -1e9 * LOG2E

NQ = 512
KC = 128
NC = S // KC
LAG = 3
T0 = 24

BF = jnp.bfloat16
F32 = jnp.float32
U32 = jnp.uint32
WAO, WBQ, WBK, WBV, WBO = range(5)
PH = "all"
def on(p): return PH == "all" or p in PH.split(",")
CFG = {}


def _pack(x):
    return pltpu.bitcast(x.astype(BF), U32)


def _unpack(x):
    return pltpu.bitcast(x, BF)


def _halves(w):
    lo = lax.bitcast_convert_type(w << 16, F32)
    hi = lax.bitcast_convert_type(w & np.uint32(0xFFFF0000), F32)
    return lo, hi


def _ds(i, n):
    if isinstance(i, int):
        return pl.ds(i * n, n)
    return pl.ds(pl.multiple_of(i * n, n), n)


def _dot(a, b):
    return jnp.dot(a, b, preferred_element_type=F32)


def _after(x, token):
    if token is None:
        return x
    token = jnp.tile(token, (x.shape[0] // 8, x.shape[1] // 128))
    return jnp.where(token < -jnp.inf, jnp.zeros_like(x), x)


class _Lane:
    token = None

    def __call__(self, x):
        return _after(x, self.token)

    def head(self, x):
        return x if self.token is None else jnp.concatenate([self(x[:8]), x[8:]], axis=0)


class _Pace:
    def __init__(self):
        self.now, self.queue = 0, []

    def spread(self, lo, hi, *jobs):
        lane = _Lane()
        total = sum(sum(costs) for _, _, costs in jobs)
        done = 0
        for fn, args, costs in jobs:
            gen = fn(lane, *args)
            for cost in costs:
                self.queue.append((lo + (hi - lo) * done // total, len(self.queue), lane, gen))
                done += cost
        self.queue.sort(key=lambda e: e[:2])

    def matmul(self, lhs, rhs):
        y = None
        for k in range(2):
            part = _dot(_unpack(lhs(k)), _unpack(rhs(k)))
            start, self.now = self.now, self.now + part.shape[0]
            while self.queue and self.queue[0][0] < self.now:
                t, _, lane, gen = self.queue.pop(0)
                row = (t - start) // 8 * 8
                lane.token = part[row:row + 8]
                next(gen)
            y = part if y is None else y + part
        return y


def _run(job):
    fn, args, _ = job
    for _ in fn(_Lane(), *args):
        pass


def _job(costs):
    def wrap(fn):
        return lambda *a: (fn, a, costs(*a) if callable(costs) else costs)
    return wrap


def _kernel(x_hbm, aq_hbm, ao_hbm, bq_hbm, bo_hbm, out_hbm,
            x_raw, aq_raw, w_raw, tmp, xtmp, ao_perm,
            aq_t, w_t, x_t, xn_t, o_t,
            qb, kb, vb, vfirst,
            bq_s, bk_s, bv_s, s0, s1, qs, ks, vs, qf, kf,
            sem_x, sem_aq, sem_w, sem_o):
    sbuf = (s0, s1)

    def x_copy(j):
        h, rows = ((0, pl.ds(0, 56)), (0, pl.ds(56, 72)), (1, pl.ds(0, 128)))[j]
        return pltpu.make_async_copy(x_hbm.at[rows, h], x_raw.at[h, rows], sem_x.at[j])

    def aq_copy(g, t):
        return pltpu.make_async_copy(aq_hbm.at[:, _ds(4 * t + g, 256)], aq_raw.at[:, _ds(4 * t + g, 256)],
                                     sem_aq.at[4 * t + g])

    def w_copy(i):
        src, lo = ((ao_hbm, WAO), (bq_hbm, WBQ), (bo_hbm, WBO))[i]
        return pltpu.make_async_copy(src, w_raw.at[:, pl.ds(lo * D, src.shape[1])], sem_w.at[i])

    def out_copy(h, ct):
        return pltpu.make_async_copy(x_raw.at[h, :, :, _ds(ct, 128)], out_hbm.at[:, h, :, _ds(ct, 128)],
                                     sem_o.at[8 * h + ct])

    def weights(n):
        groups = ((0,), (1,), (2, 3), (), ())[n]
        return [aq_copy(g, t) for g in groups for t in range(3)] + [w_copy(i) for i in range(3) if n == 3]

    def dma(starts, waits):
        for cp in starts:
            cp.start()
        for cp in waits:
            cp.wait()

    @_job([1] * 5)
    def load_x(ln, h, ct):
        w = _pack(x_raw[h, :, :, _ds(ct, 128)].reshape(S // 2, 128))
        xtmp[_ds(ct, 512), :] = ln(w)
        yield
        for c in range(4):
            lo, hi = _halves(ln.head(xtmp[pl.ds(ct * 512 + c, 128, stride=4), :]).T)
            x_t[4 * h + c, _ds(ct, 128), :] = lo
            x_t[8 + 4 * h + c, _ds(ct, 128), :] = hi
            yield

    @_job([1])
    def store_x1(ln, ct, c):
        lo = lax.bitcast_convert_type(x_t[c, _ds(ct, 128), :].astype(BF).astype(F32), U32)
        hi = lax.bitcast_convert_type(x_t[8 + c, _ds(ct, 128), :].astype(BF).astype(F32), U32)
        (xtmp, tmp)[c // 4][pl.ds(ct * 512 + c % 4, 128, stride=4), :] = ln.head((lo >> 16) | hi).T
        yield

    @_job([1] * 8)
    def store_x2(ln, ct, h):
        for r in range(8):
            w = ln((xtmp, tmp)[h][pl.ds(ct * 512 + r * 64, 64), :])
            x_raw[h, _ds(r, 16), :, _ds(ct, 128)] = _unpack(w).reshape(16, 8, 128)
            if r == 7:
                out_copy(h, ct).start()
            yield

    def head_major(ln, base, dp, n):
        lo, hi = _halves(ln(tmp[pl.ds(base + dp, 8 * n, stride=16), :]))
        return jnp.concatenate([lo.reshape(n, 8, 128), hi.reshape(n, 8, 128)], axis=1)

    @_job([1] * 8)
    def prep_aq1(ln, g, n):
        for kt in range(8):
            w = _pack(aq_raw[_ds(kt, 128), _ds(4 * ((n + 1) % 3) + g, 256)])
            tmp[pl.ds(n * D + kt * 128, 128), :] = _pack(_unpack(ln.head(w)).T)
            yield

    @_job([40] * 16)
    def prep_aq2(ln, g, n):
        for dp in range(16):
            w = head_major(ln, n * D, dp, 8)
            aq_t[_ds(16 * (3 * g + n) + dp, 8), :] = _pack(jnp.concatenate([w[kt] for kt in range(8)], axis=1))
            yield

    @_job([60] * 4 + [40] * 16)
    def permute_ao(ln, g):
        for n in range(4):
            w = [_pack(w_raw[_ds(g, 256), _ds(8 * WAO + 2 * n + ct, 128)]) for ct in range(2)]
            tmp[_ds(4 * g + n, 256), :] = ln(jnp.concatenate(w, axis=0))
            yield
        for dp in range(16):
            w = head_major(ln, g * D, dp, 8)
            ao_perm[_ds(16 * g + dp, 8), :] = _pack(jnp.concatenate([w[ct] for ct in range(8)], axis=1))
            yield

    @_job([1] * 32)
    def prep_w(ln, j):
        for ct in range(8):
            for k in range(4):
                if j == WAO:
                    w = ao_perm[_ds(k, 128), _ds(ct, 128)]
                else:
                    w = _pack(w_raw[_ds(k, 256), _ds(8 * j + ct, 128)])
                w_t[_ds(8 * j + ct, 64), _ds(k, 256)] = _pack(_unpack(ln.head(w)).T)
                yield

    @_job([40] * 10 + [30] * 8)
    def layernorm(ln, tile):
        stat = []
        for k in range(2):
            for r in range(4):
                x = x_t[tile, _ds(r, 256), :].reshape(16, 16, 128)
                if k:
                    x = x - ln(stat[0])
                    x = x * x
                acc = ln(jnp.sum(x, axis=0) if r == 0 else acc + jnp.sum(x, axis=0))
                yield
            t = jnp.broadcast_to(jnp.sum(acc, axis=0, keepdims=True) * (1.0 / D), (16, 128))
            stat.append(ln(lax.rsqrt(t + EPS) if k else t))
            yield
        for r in range(8):
            x = (x_t[tile, _ds(r, 128), :].reshape(8, 16, 128) - ln(stat[0])) * stat[1]
            xn_t[_ds(r, 64), _ds(tile, 128)] = _pack(x.reshape(128, 128))
            yield

    def project(pc, w_ref, row, words, src, tile):
        return pc.matmul(lambda k: w_ref[_ds(row, words), _ds(k, 512)], lambda k: src[_ds(k, 256), _ds(tile, 128)])

    def out_proj(pc, j, tile):
        for r in range(4):
            x_t[tile, _ds(r, 256), :] += project(pc, w_t, 4 * j + r, 128, o_t, tile)

    def a_qkv(pc, g, e, c):
        par = g % 2
        k = project(pc, aq_t, 3 * g, 128, xn_t, 8 * e + c)
        kb[par, :, _ds(7 + c, 128)] = k
        if c:
            kb[par, :, _ds(c - 1, 128)] = pltpu.roll(k, 1, 1)
        v = project(pc, aq_t, 3 * g + 1, 128, xn_t, 8 * e + c)
        vb[par, :, _ds(7 + c, 128)] = v
        if c:
            lane0 = lax.broadcasted_iota(jnp.int32, (256, 128), 1) == 0
            vb[par, :, _ds(c - 1, 128)] = jnp.where(lane0, vfirst[g], pltpu.roll(v, 1, 1))
        elif e == 0:
            vfirst[g] = v
        qb[par, :, _ds(c, 128)] = project(pc, aq_t, 3 * g + 2, 128, xn_t, 8 * e + c)

    nq, nd = CFG.get("nq", 4), CFG.get("nd", 4)

    @_job([8 * nq] * (DH // nq - 1) + [30] * 4 + [8 * nd] * (DH // nd))
    def a_attn(ln, g, e, c):
        par = g % 2
        win = pl.ds(c * 128, WIN * 128)
        for r in range(DH // nq):
            t = jnp.tile(qb[par, _ds(r, 8 * nq), _ds(c, 128)], (1, WIN)) * kb[par, _ds(r, 8 * nq), win]
            t = jnp.sum(t.reshape(nq, 8, WIN * 128), axis=0)
            acc = ln(t if r == 0 else acc + t)
            yield
        lane0 = lax.broadcasted_iota(jnp.int32, (8, 128), 1) == 0
        logit = []
        for w in range(WIN):
            t = acc[:, w * 128:(w + 1) * 128] * QSCALE
            logit.append(jnp.where(lane0, MASKED, t) if c + w < 7 else t)
        m = logit[0]
        for t in logit[1:]:
            m = jnp.maximum(m, t)
        m = ln(m)
        yield
        p = [jnp.exp2(t - m) for t in logit]
        l = ln(sum(p[1:], p[0]))
        yield
        r = ln(1.0 / l)
        yield
        p = [t * r for t in p]
        for h in range(DH // nd):
            t = jnp.tile(jnp.concatenate([ln(p[0])] + p[1:], axis=1), (nd, 1)) * vb[par, _ds(h, 8 * nd), win]
            o = sum([t[:, w * 128:(w + 1) * 128] for w in range(1, WIN)], t[:, :128])
            o_t[_ds(g * (DH // nd) + h, 4 * nd), _ds(8 * e + c, 128)] = _pack(o)
            yield

    def a_layer(first):
        for u in range(8):
            if not on(f"a{u}"):
                continue
            pc = _Pace()
            jobs = [a_attn((u - 1) % 4, (u - 1) // 4, c) for c in range(8)] if u else []
            if not first:
                if u == 0:
                    pc.spread(0, 2000, layernorm(15))
            elif u == 0:
                for lo, tile in ((300, 1), (1536, 2), (2300, 3), (5200, 4), (6144, 5), (6900, 6), (7680, 7)):
                    pc.spread(lo, lo + (700 if tile < 7 else 1800), layernorm(tile))
                pc.spread(3072, 5000, *[load_x(1, ct) for ct in range(8)])
                pc.spread(7680, 9500, *[prep_aq1(1, n) for n in range(3)])
                pc.spread(9700, 12200, *[prep_aq2(1, n) for n in range(3)])
            elif u < 3:
                pc.spread(4608, 8500, *[prep_aq1(u + 1, n) for n in range(3)])
                jobs += [layernorm(5 + 3 * u + n) for n in range(3)] + [prep_aq2(u + 1, n) for n in range(3)]
            else:
                if u == 3:
                    jobs += [layernorm(14), layernorm(15)]
                if u in (4, 5):
                    jobs += [permute_ao(2 * u - 8), permute_ao(2 * u - 7)]
                pc.spread(1536, 11500, prep_w((WBQ, WBK, WBV, WAO, WBO)[u - 3]))
            if jobs:
                pc.spread(0, 12000, *jobs)
            for c in range(8):
                if first and (u, c) in ((0, 2), (0, 5), (1, 3), (3, 1)):
                    n = ((0, 2), (0, 5), (1, 3), (3, 1)).index((u, c))
                    dma([], weights(n) if n else [x_copy(2)])
                    dma(weights(n + 1), [])
                a_qkv(pc, u % 4, u // 4, c)
        for tile in range(16):
            if not on(f"ao{tile // 8 + 1}"):
                continue
            pc = _Pace()
            pc.spread(0, 2000, *([layernorm(tile - 1)] if tile else []), *([a_attn(3, 1, tile)] if tile < 8 else []))
            out_proj(pc, WAO, tile)

    def b_qkv(pc, p):
        for r in range(4):
            k = jnp.concatenate([project(pc, w_t, 4 * WBK + r, 128, xn_t, 2 * p + n).astype(BF) for n in range(2)], axis=1)
            for g in range(2):
                bk_s[_ds(p, 128), _ds(2 * r + g, 128)] = _pack(k[g * 128:(g + 1) * 128].T)
        for n in range(2):
            for r in range(4):
                bq_s[_ds(r, 128), _ds(2 * p + n, 128)] = _pack(project(pc, w_t, 4 * WBQ + r, 128, xn_t, 2 * p + n) * QSCALE)
            for r in range(4):
                bv_s[_ds(r, 128), _ds(2 * p + n, 128)] = _pack(project(pc, w_t, 4 * WBV + r, 128, xn_t, 2 * p + n))

    NV = CFG.get("nv", 6)
    VCHUNK = CFG.get("vc", [NC * b // NV for b in range(NV)])
    NT = NQ // 128

    def stage_k(hold, head, par, c):
        k = bk_s[_ds(c, KC // 2), _ds(head // 4, 128)]
        k = jnp.concatenate([hold(k[:8]), k[8:]], axis=0)
        ks[par, _ds(c, KC // 2), :] = pltpu.roll(k, (128 - DH * (head % 4)) % 128, 1)

    def spread_k(hold, par, b, r):
        k = _unpack(hold(ks[par, pl.ds((VCHUNK[b] + 1) * KC // 2 - 8, 8), :])).astype(F32)
        kf[par, _ds(4 * b + r, 128), :] = jnp.concatenate(
            [jnp.broadcast_to(k[:, d:d + 1], (16, 128)) for d in range(8 * r, 8 * r + 8)], axis=0)

    def stage_v(hold, head, par, r):
        vs[par, :, _ds(r, 512)] = hold(bv_s[_ds(head, DH // 2), _ds(r, 512)])

    def spread_q(hold, head, blk, r):
        q = hold(bq_s[_ds(2 * head + r // 4, 8), _ds(blk, NQ)])
        if r % 4 == 0:
            qs[blk % 2, _ds(r // 4, 8), :] = q
        q = _unpack(q).astype(F32)
        for d in range(4 * r, 4 * r + 4):
            qf[blk % 2, _ds(d, 8), :] = jnp.broadcast_to(q[d % 16:d % 16 + 1], (8, NQ))

    @_job([1] * (NC + 4 * NV + 8))
    def stage_first(ln):
        for c in range(NC):
            stage_k(ln, 0, 0, c)
            yield
        for n in range(4 * NV):
            spread_k(ln, 0, n // 4, n % 4)
            yield
        for r in range(8):
            spread_q(ln, 0, 0, r)
            yield

    def b_steps(head0, t_lo, t_hi, state, qk_end=None):
        m_old, m_new, m_run, l, acc = state
        ms = {t_lo // NC - 2: m_old, t_lo // NC - 1: m_new}
        marks = {}

        def pace(x, t, frac):
            t, frac = t + math.floor(frac), frac - math.floor(frac)
            if t not in marks:
                return x
            row = int(frac * marks[t].shape[0]) // CFG.get("gr", 8) * CFG.get("gr", 8)
            return _after(x, marks[t][row:row + 8])

        for t in range(t_lo, t_hi):
            u, c = divmod(t, NC)
            par = u // 4 % 2
            if qk_end is None or t < qk_end:
                words = KC // 2 - (8 if c in VCHUNK else 0)
                q = jnp.concatenate([_unpack(qs[u % 2]), jnp.zeros((128 - DH, NQ), BF)], axis=0)
                s = _dot(_unpack(ks[par, pl.ds(c * KC // 2, words), :]), q)
                marks[t] = s[:, :128]
            up, cp = divmod(t - NC - LAG, NC)
            if up >= 0:
                ns = CFG.get("ns", 4)
                p = []
                for j in range(ns):
                    z = sbuf[up % 2][_ds(ns * cp + ns - 1 - j, KC // ns), :].reshape(-1, 8, NQ)
                    e = jnp.exp2(z - pace(ms[up], t - 1, CFG.get("st", 1.0) * j / ns + CFG.get("off", -0.32)))
                    l = jnp.sum(e, axis=0) if cp == 0 and j == 0 else l + jnp.sum(e, axis=0)
                    p.insert(0, e.reshape(KC // ns, NQ))
                a = _dot(_unpack(vs[up // 4 % 2, :, _ds(cp, KC)]), jnp.concatenate(p, axis=0).astype(BF))
                acc = a if cp == 0 else acc + a
                if t in marks:
                    marks[t] = jnp.concatenate([marks[t], a[:, :128]], axis=0)
                if cp == NC - 1:
                    total = pace(jnp.broadcast_to(jnp.sum(l, axis=0, keepdims=True), (8, NQ)), t, 0.3)
                    o = acc * jnp.tile(pace(1.0 / total, t, 0.7), (DH // 8, 1))
                    o_t[_ds(head0 + up // 4, DH // 2), _ds(up % 4, NQ)] = _pack(o)
            if t in marks:
                sbuf[u % 2][pl.ds(c * KC, 2 * words), :] = s
                mx = jnp.max(s.reshape(-1, 8, NQ), axis=0)
                m_run = mx if c == 0 else jnp.maximum(m_run, mx)
                nd, nt = CFG.get("aa", 4), CFG.get("nt", 1)
                per_unit = NV * NT // nt * DH // nd
                for n in range(per_unit * c // NC, per_unit * (c + 1) // NC):
                    (b, j), r = divmod(n * nd // DH, NT // nt), n % (DH // nd)
                    kd = jnp.tile(kf[par, _ds(b * (DH // nd) + r, 16 * nd), :], (1, nt)).reshape(nd, 2, 8, nt * 128)
                    term = jnp.sum(kd * qf[u % 2, _ds(r, 8 * nd), _ds(j, nt * 128)].reshape(nd, 1, 8, nt * 128), axis=0)
                    term = term.reshape(16, nt * 128)
                    sv = pace(term if r == 0 else sv + term, t, (n + 1) * NC / per_unit - c - CFG.get("ld", 0.6))
                    if r == DH // nd - 1:
                        sbuf[u % 2][pl.ds((VCHUNK[b] + 1) * KC - 16, 16), _ds(j, nt * 128)] = sv
                        w = nt * 128
                        m_run = jnp.concatenate(
                            [jnp.maximum(m_run[:, k * w:(k + 1) * w], jnp.maximum(sv[:8], sv[8:])) if k == j
                             else m_run[:, k * w:(k + 1) * w] for k in range(NT // nt)], axis=1)
                if c == NC - 1:
                    ms[u] = jnp.broadcast_to(jnp.max(m_run, axis=0, keepdims=True), (8, NQ))
                if (qk_end is None or t + NC < qk_end) and c % 2 == 0:
                    spread_q(lambda x: pace(x, t, -0.5), head0 + (u + 1) // 4, (u + 1) % 4, c // 2)
                if u % 4 == 0 and c % 4 == 3:
                    stage_v(lambda x: pace(x, t, -0.5), head0 + u // 4, par, c // 4)
                if qk_end is None or t + 4 * NC < qk_end:
                    n = (t % (4 * NC) - T0 - 3) * 4 // 5
                    if u % 4 == 0:
                        stage_k(lambda x: pace(x, t, -1.0), head0 + u // 4 + 1, 1 - par, c)
                    elif 0 <= n < 4 * NV and n != (t % (4 * NC) - T0 - 4) * 4 // 5:
                        spread_k(lambda x: pace(x, t, -1.0), 1 - par, n // 4, n % 4)
        zero = jnp.zeros((8, NQ), F32)
        return ms.get(t_hi // NC - 2, zero), ms.get(t_hi // NC - 1, zero), m_run, l, acc

    def b_layer():
        if on("bq1"):
            pc = _Pace()
            pc.spread(0, 2000, layernorm(15))
            b_qkv(pc, 0)
        if on("bq2"):
            lax.fori_loop(1, 7, lambda p, c: b_qkv(_Pace(), p), None)
            pc = _Pace()
            pc.spread(4400, 11800, stage_first())
            b_qkv(pc, 7)
        if on("battn"):
            zero = jnp.zeros((8, NQ), F32)
            heads = D // DH
            state = b_steps(0, 0, T0, (zero, zero, zero, zero, jnp.zeros((DH, NQ), F32)))
            state = lax.fori_loop(0, heads // 2 - 1, lambda i, st: b_steps(2 * i, T0, T0 + 8 * NC, st), state)
            if CFG.get("epi", 1):
                b_steps(heads - 2, T0, 9 * NC + LAG, state, qk_end=8 * NC)

    if on("start"):
      with jax.named_scope("P0_start"):
        dma([x_copy(0), x_copy(1)], [x_copy(0)])
        dma(weights(0), [x_copy(1)])
        for ct in range(8):
            _run(load_x(0, ct))
        _run(layernorm(0))
        dma([], weights(0))
        dma([x_copy(2)], [])
      for n in range(3):
        _run(prep_aq1(0, n))
      for n in range(3):
        _run(prep_aq2(0, n))

    a_layer(CFG.get("first", True))
    with jax.named_scope("P2_b"):
        b_layer()
    if on("bo"):
      with jax.named_scope("P3_bo"):
        for tile in range(16):
            pc = _Pace()
            if tile:
                pc.spread(0, 2000, layernorm(tile - 1))
            out_proj(pc, WBO, tile)
    if PH == "all":
        with jax.named_scope("P4_a"):
            a_layer(False)
        with jax.named_scope("P5_b"):
            b_layer()

    if on("final"):
      with jax.named_scope("P6_final"):
        for r in range(4):
            for c in range(8):
                pc = _Pace()
                r1, c1 = divmod(8 * r + c - 1, 8)
                if r1 >= 0:
                    pc.spread(0, 300, store_x1(2 * r1, c1), store_x1(2 * r1 + 1, c1))
                r2, c2 = divmod(8 * r + c - 2, 8)
                if r2 >= 0 and c2 % 4 == 3:
                    pc.spread(0, 1000, store_x2(2 * r2, c2 // 4), store_x2(2 * r2 + 1, c2 // 4))
                for tile in (c, 8 + c):
                    x_t[tile, _ds(r, 256), :] += project(pc, w_t, 4 * WBO + r, 128, o_t, tile)
        for job in (store_x1(6, 7), store_x1(7, 7), store_x2(6, 1), store_x2(7, 1)):
            _run(job)
        dma([], [out_copy(h, ct) for h in range(2) for ct in range(8)])
    else:
        def keep(i, c):
            for r_ in (x_t, qb, kb, vb, qf, kf):
                s0[pl.ds(0, 8), pl.ds(0, 128)] += r_[i, pl.ds(0, 8), pl.ds(0, 128)]
            for r_ in (bq_s, bv_s, bk_s, xn_t, o_t, w_t, aq_t, ao_perm):
                tmp[pl.ds(0, 8), :] |= r_[_ds(i, 8), pl.ds(0, 128)]
            return c
        lax.fori_loop(0, 2, keep, 0)
        x_raw[0, pl.ds(0, 2), :, pl.ds(0, 128)] = _unpack(tmp[pl.ds(0, 8), :] | lax.bitcast_convert_type(s0[pl.ds(0, 8), pl.ds(0, 128)], U32)).reshape(2, 8, 128)
        out_copy(0, 0).start(); out_copy(0, 0).wait()


@jax.jit
def pallas_interleave_layers__sliding_local_dilated__softmax_full_mha__prompt_kernel(
    A_x: jax.Array,
    A_wqkv: jax.Array,
    A_wo: jax.Array,
    B_x: jax.Array,
    B_wqkv: jax.Array,
    B_wo: jax.Array,
):
    del B_x
    vmem = pltpu.VMEM
    scratch = [
        vmem((2, 128, 8, D), BF), vmem((D, 3 * D), BF), vmem((D, 5 * D), BF),
        vmem((4 * D, 128), U32), vmem((4 * D, 128), U32), vmem((D // 2, D), U32),
        vmem((3 * D // 2, D), U32), vmem((5 * D // 2, D), U32),
        vmem((16, D, 128), F32), vmem((D // 2, S), U32), vmem((D // 2, S), U32),
        vmem((2, 256, 8 * 128), F32), vmem((2, 256, 15 * 128), F32), vmem((2, 256, 15 * 128), F32),
        vmem((4, 256, 128), F32),
        vmem((D // 2, S), U32), vmem((S // 2, D), U32), vmem((D // 2, S), U32),
        vmem((S, NQ), F32), vmem((S, NQ), F32),
        vmem((2, DH // 2, NQ), U32), vmem((2, S // 2, 128), U32), vmem((2, DH // 2, S), U32),
        vmem((2, 8 * DH, NQ), F32), vmem((2, 8 * DH * 16, 128), F32),
        pltpu.SemaphoreType.DMA((3,)), pltpu.SemaphoreType.DMA((12,)),
        pltpu.SemaphoreType.DMA((3,)), pltpu.SemaphoreType.DMA((16,)),
    ]
    out = pl.pallas_call(
        _kernel,
        out_shape=jax.ShapeDtypeStruct((128, 2, 8, D), A_x.dtype),
        in_specs=[pl.BlockSpec(memory_space=pl.ANY)] * 5,
        out_specs=pl.BlockSpec(memory_space=pl.ANY),
        scratch_shapes=scratch,
        compiler_params=pltpu.CompilerParams(vmem_limit_bytes=124 * 1024 * 1024),
        name="interleaved_attention_layers",
    )(A_x.reshape(128, 2, 8, D), A_wqkv, A_wo, B_wqkv, B_wo)
    return out.reshape(A_x.shape)
```

```python
import math

import jax
import jax.numpy as jnp
import numpy as np
from jax import lax
import jax.experimental.pallas as pl
import jax.experimental.pallas.tpu as pltpu

S = 2048
D = 1024
DH = 32
WIN = 8
EPS = 1e-5
LOG2E = math.log2(math.e)
QSCALE = DH ** -0.5 * LOG2E
MASKED = -1e9 * LOG2E

NQ = 512
KC = 128
NC = S // KC
LAG = 3
T0 = 24

BF = jnp.bfloat16
F32 = jnp.float32
U32 = jnp.uint32
WAO, WBQ, WBK, WBV, WBO = range(5)
PH = "all"
def on(p): return PH == "all" or p in PH.split(",")
CFG = {}


def _pack(x):
    return pltpu.bitcast(x.astype(BF), U32)


def _unpack(x):
    return pltpu.bitcast(x, BF)


def _halves(w):
    lo = lax.bitcast_convert_type(w << 16, F32)
    hi = lax.bitcast_convert_type(w & np.uint32(0xFFFF0000), F32)
    return lo, hi


def _ds(i, n):
    if isinstance(i, int):
        return pl.ds(i * n, n)
    return pl.ds(pl.multiple_of(i * n, n), n)


def _dot(a, b):
    return jnp.dot(a, b, preferred_element_type=F32)


def _after(x, token):
    if token is None:
        return x
    token = jnp.tile(token, (x.shape[0] // 8, x.shape[1] // 128))
    return jnp.where(token < -jnp.inf, jnp.zeros_like(x), x)


class _Lane:
    token = None

    def __call__(self, x):
        return _after(x, self.token)

    def head(self, x):
        return x if self.token is None else jnp.concatenate([self(x[:8]), x[8:]], axis=0)


class _Pace:
    def __init__(self):
        self.now, self.queue, self.results = 0, [], []

    def spread(self, lo, hi, *jobs):
        lane = _Lane()
        total = sum(sum(costs) for _, _, costs in jobs)
        done = 0
        for fn, args, costs in jobs:
            gen = fn(lane, *args)
            for cost in costs:
                self.queue.append((lo + (hi - lo) * done // total, len(self.queue), lane, gen))
                done += cost
        self.queue.sort(key=lambda e: e[:2])

    def mark(self, time):
        for start, y in reversed(self.results):
            if start <= time:
                row = (time - start) // 8 * 8
                return y[row:row + 8, :128]
        return None

    def tick(self, y):
        self.results.append((self.now, y))
        self.now += y.shape[0]
        while self.queue and self.queue[0][0] < self.now:
            time, _, lane, gen = self.queue.pop(0)
            lane.token = self.mark(time)
            next(gen)
        return y

    def matmul(self, lhs, rhs):
        lo, hi = [self.tick(_dot(_unpack(lhs(k)), _unpack(rhs(k)))) for k in range(2)]
        return lo + hi


def _run(job):
    fn, args, _ = job
    for _ in fn(_Lane(), *args):
        pass


def _job(costs):
    def wrap(fn):
        return lambda *a: (fn, a, costs(*a) if callable(costs) else costs)
    return wrap


def _kernel(x_hbm, aq_hbm, ao_hbm, bq_hbm, bo_hbm, out_hbm,
            x_raw, aq_raw, w_raw, tmp, xtmp, ao_perm,
            aq_t, w_t, x_t, xn_t, o_t,
            qb, kb, vb, vfirst,
            bq_s, bk_s, bv_s, s0, s1, qs, ks, vs, qf, kf,
            sem_x, sem_aq, sem_w, sem_o):
    sbuf = (s0, s1)

    def x_copy(j):
        h, rows = ((0, pl.ds(0, 56)), (0, pl.ds(56, 72)), (1, pl.ds(0, 128)))[j]
        return pltpu.make_async_copy(x_hbm.at[rows, h], x_raw.at[h, rows], sem_x.at[j])

    def aq_copy(g, t):
        return pltpu.make_async_copy(aq_hbm.at[:, _ds(4 * t + g, 256)], aq_raw.at[:, _ds(4 * t + g, 256)],
                                     sem_aq.at[4 * t + g])

    def w_copy(i):
        src, lo = ((ao_hbm, WAO), (bq_hbm, WBQ), (bo_hbm, WBO))[i]
        return pltpu.make_async_copy(src, w_raw.at[:, pl.ds(lo * D, src.shape[1])], sem_w.at[i])

    def out_copy(h, ct):
        return pltpu.make_async_copy(x_raw.at[h, :, :, _ds(ct, 128)], out_hbm.at[:, h, :, _ds(ct, 128)],
                                     sem_o.at[8 * h + ct])

    def weights(n):
        groups, blocks = (((0,), ()), ((1,), ()), ((2, 3), (0,)), ((), (1, 2)))[n]
        return [aq_copy(g, t) for g in groups for t in range(3)] + [w_copy(i) for i in blocks]

    def dma(starts, waits):
        for cp in starts:
            cp.start()
        for cp in waits:
            cp.wait()

    @_job([1] * 5)
    def load_x(ln, h, ct):
        w = _pack(x_raw[h, :, :, _ds(ct, 128)].reshape(S // 2, 128))
        xtmp[_ds(ct, 512), :] = ln(w)
        yield
        for c in range(4):
            lo, hi = _halves(ln.head(xtmp[pl.ds(ct * 512 + c, 128, stride=4), :]).T)
            x_t[4 * h + c, _ds(ct, 128), :] = lo
            x_t[8 + 4 * h + c, _ds(ct, 128), :] = hi
            yield

    @_job([1])
    def store_x1(ln, ct, c):
        lo = lax.bitcast_convert_type(x_t[c, _ds(ct, 128), :].astype(BF).astype(F32), U32)
        hi = lax.bitcast_convert_type(x_t[8 + c, _ds(ct, 128), :].astype(BF).astype(F32), U32)
        (xtmp, tmp)[c // 4][pl.ds(ct * 512 + c % 4, 128, stride=4), :] = ln.head((lo >> 16) | hi).T
        yield

    @_job([1] * 8)
    def store_x2(ln, ct, h):
        for r in range(8):
            w = ln((xtmp, tmp)[h][pl.ds(ct * 512 + r * 64, 64), :])
            x_raw[h, _ds(r, 16), :, _ds(ct, 128)] = _unpack(w).reshape(16, 8, 128)
            if r == 7:
                out_copy(h, ct).start()
            yield

    def head_major(ln, scr, base, dp, n):
        lo, hi = _halves(ln(scr[pl.ds(base + dp, 8 * n, stride=16), :]))
        return jnp.concatenate([lo.reshape(n, 8, 128), hi.reshape(n, 8, 128)], axis=1)

    @_job([1] * 8)
    def prep_aq1(ln, g, n):
        for kt in range(8):
            w = _pack(aq_raw[_ds(kt, 128), _ds(4 * ((n + 1) % 3) + g, 256)])
            tmp[pl.ds(n * D + kt * 128, 128), :] = _pack(_unpack(ln.head(w)).T)
            yield

    @_job([40] * 16)
    def prep_aq2(ln, g, n):
        for dp in range(16):
            w = head_major(ln, tmp, n * D, dp, 8)
            aq_t[_ds(16 * (3 * g + n) + dp, 8), :] = _pack(jnp.concatenate([w[kt] for kt in range(8)], axis=1))
            yield

    @_job([60] * 4 + [40] * 16)
    def permute_ao(ln, g):
        for n in range(4):
            w = [_pack(w_raw[_ds(g, 256), _ds(8 * WAO + 2 * n + ct, 128)]) for ct in range(2)]
            xtmp[_ds(4 * g + n, 256), :] = ln(jnp.concatenate(w, axis=0))
            yield
        for dp in range(16):
            w = head_major(ln, xtmp, g * D, dp, 8)
            ao_perm[_ds(16 * g + dp, 8), :] = _pack(jnp.concatenate([w[ct] for ct in range(8)], axis=1))
            yield

    @_job(lambda j, tiles: [1] * (4 * len(tiles)))
    def prep_w(ln, j, tiles):
        for ct in tiles:
            for k in range(4):
                if j == WAO:
                    w = ao_perm[_ds(k, 128), _ds(ct, 128)]
                else:
                    w = _pack(w_raw[_ds(k, 256), _ds(8 * j + ct, 128)])
                w_t[_ds(8 * j + ct, 64), _ds(k, 256)] = _pack(_unpack(ln.head(w)).T)
                yield

    @_job([40] * 10 + [30] * 8)
    def layernorm(ln, tile):
        stat = []
        for k in range(2):
            for r in range(4):
                x = x_t[tile, _ds(r, 256), :].reshape(16, 16, 128)
                if k:
                    x = x - ln(stat[0])
                    x = x * x
                acc = ln(jnp.sum(x, axis=0) if r == 0 else acc + jnp.sum(x, axis=0))
                yield
            t = jnp.broadcast_to(jnp.sum(acc, axis=0, keepdims=True) * (1.0 / D), (16, 128))
            stat.append(ln(lax.rsqrt(t + EPS) if k else t))
            yield
        for r in range(8):
            x = (x_t[tile, _ds(r, 128), :].reshape(8, 16, 128) - ln(stat[0])) * stat[1]
            xn_t[_ds(r, 64), _ds(tile, 128)] = _pack(x.reshape(128, 128))
            yield

    def project(pc, w_ref, row, words, src, tile):
        return pc.matmul(lambda k: w_ref[_ds(row, words), _ds(k, 512)], lambda k: src[_ds(k, 256), _ds(tile, 128)])

    def out_proj(pc, j, tile):
        for r in range(4):
            x_t[tile, _ds(r, 256), :] += project(pc, w_t, 4 * j + r, 128, o_t, tile)

    def a_qkv(pc, g, e, c):
        par = g % 2
        k = project(pc, aq_t, 3 * g, 128, xn_t, 8 * e + c)
        kb[par, :, _ds(7 + c, 128)] = k
        if c:
            kb[par, :, _ds(c - 1, 128)] = pltpu.roll(k, 1, 1)
        v = project(pc, aq_t, 3 * g + 1, 128, xn_t, 8 * e + c)
        vb[par, :, _ds(7 + c, 128)] = v
        if c:
            lane0 = lax.broadcasted_iota(jnp.int32, (256, 128), 1) == 0
            vb[par, :, _ds(c - 1, 128)] = jnp.where(lane0, vfirst[g], pltpu.roll(v, 1, 1))
        elif e == 0:
            vfirst[g] = v
        qb[par, :, _ds(c, 128)] = project(pc, aq_t, 3 * g + 2, 128, xn_t, 8 * e + c)

    nq, nd = CFG.get("nq", 4), CFG.get("nd", 4)

    @_job([8 * nq] * (DH // nq - 1) + [30] * 4 + [8 * nd] * (DH // nd))
    def a_attn(ln, g, e, c):
        par = g % 2
        win = pl.ds(c * 128, WIN * 128)
        for r in range(DH // nq):
            t = jnp.tile(qb[par, _ds(r, 8 * nq), _ds(c, 128)], (1, WIN)) * kb[par, _ds(r, 8 * nq), win]
            t = jnp.sum(t.reshape(nq, 8, WIN * 128), axis=0)
            acc = ln(t if r == 0 else acc + t)
            yield
        lane0 = lax.broadcasted_iota(jnp.int32, (8, 128), 1) == 0
        logit = []
        for w in range(WIN):
            t = acc[:, w * 128:(w + 1) * 128] * QSCALE
            logit.append(jnp.where(lane0, MASKED, t) if c + w < 7 else t)
        m = logit[0]
        for t in logit[1:]:
            m = jnp.maximum(m, t)
        m = ln(m)
        yield
        p = [jnp.exp2(t - m) for t in logit]
        l = ln(sum(p[1:], p[0]))
        yield
        r = ln(1.0 / l)
        yield
        p = [t * r for t in p]
        for h in range(DH // nd):
            t = jnp.tile(jnp.concatenate([ln(p[0])] + p[1:], axis=1), (nd, 1)) * vb[par, _ds(h, 8 * nd), win]
            o = sum([t[:, w * 128:(w + 1) * 128] for w in range(1, WIN)], t[:, :128])
            o_t[_ds(g * (DH // nd) + h, 4 * nd), _ds(8 * e + c, 128)] = _pack(o)
            yield

    def a_layer(first):
        for u in range(8):
            if not on(f"a{u}"):
                continue
            pc = _Pace()
            jobs = [a_attn((u - 1) % 4, (u - 1) // 4, c) for c in range(8)] if u else []
            if not first:
                if u == 0:
                    pc.spread(0, 2000, layernorm(15))
            elif u == 0:
                for lo, tile in ((300, 1), (1536, 2), (2300, 3), (5200, 4), (6144, 5), (6900, 6), (7680, 7)):
                    pc.spread(lo, lo + (700 if tile < 7 else 1800), layernorm(tile))
                pc.spread(3072, 5000, *[load_x(1, ct) for ct in range(8)])
                pc.spread(7680, 9500, *[prep_aq1(1, n) for n in range(3)])
                pc.spread(9700, 12200, *[prep_aq2(1, n) for n in range(3)])
            elif u < 3:
                pc.spread(6144 if u == 1 else 0, 8800, *[prep_aq1(u + 1, n) for n in range(3)])
                jobs += [layernorm(t) for t in range(8, 12)] if u == 1 else [permute_ao(g) for g in range(4)]
                jobs += [prep_aq2(u + 1, n) for n in range(3)]
            elif u == 3:
                jobs += [layernorm(t) for t in range(12, 16)]
                pc.spread(0, 6000, prep_w(WAO, range(8)))
            if jobs:
                pc.spread(0, 12000, *jobs)
            for c in range(8):
                if first and (u, c) in ((0, 2), (0, 5), (1, 4)):
                    n = ((0, 2), (0, 5), (1, 4)).index((u, c))
                    dma([], weights(n) if n else [x_copy(2)])
                    dma(weights(n + 1), [])
                a_qkv(pc, u % 4, u // 4, c)
        if first:
            dma([], weights(3))
        for tile in range(16):
            if not on(f"ao{tile // 8 + 1}"):
                continue
            pc = _Pace()
            pc.spread(0, 2000, *([layernorm(tile - 1)] if tile else []), *([a_attn(3, 1, tile)] if tile < 8 else []))
            if first and tile >= 4:
                pc.spread(0, 1800, prep_w((WBK, WBQ, WBV)[tile // 4 - 1], (tile % 4 * 2, tile % 4 * 2 + 1)))
            out_proj(pc, WAO, tile)

    def b_qkv(pc, p):
        for r in range(4):
            k = jnp.concatenate([project(pc, w_t, 4 * WBK + r, 128, xn_t, 2 * p + n).astype(BF) for n in range(2)], axis=1)
            for g in range(2):
                bk_s[_ds(p, 128), _ds(2 * r + g, 128)] = _pack(k[g * 128:(g + 1) * 128].T)
        for n in range(2):
            for r in range(4):
                bq_s[_ds(r, 128), _ds(2 * p + n, 128)] = _pack(project(pc, w_t, 4 * WBQ + r, 128, xn_t, 2 * p + n) * QSCALE)
            for r in range(4):
                bv_s[_ds(r, 128), _ds(2 * p + n, 128)] = _pack(project(pc, w_t, 4 * WBV + r, 128, xn_t, 2 * p + n))

    NV = CFG.get("nv", 6)
    VCHUNK = CFG.get("vc", [NC * b // NV for b in range(NV)])
    NT = NQ // 128

    def stage_k(hold, head, par, c):
        k = bk_s[_ds(c, KC // 2), _ds(head // 4, 128)]
        k = jnp.concatenate([hold(k[:8]), k[8:]], axis=0)
        ks[par, _ds(c, KC // 2), :] = pltpu.roll(k, (128 - DH * (head % 4)) % 128, 1)

    def spread_k(hold, par, b, r):
        k = _unpack(hold(ks[par, pl.ds((VCHUNK[b] + 1) * KC // 2 - 8, 8), :])).astype(F32)
        kf[par, _ds(4 * b + r, 128), :] = jnp.concatenate(
            [jnp.broadcast_to(k[:, d:d + 1], (16, 128)) for d in range(8 * r, 8 * r + 8)], axis=0)

    def stage_v(hold, head, par, r):
        vs[par, :, _ds(r, 512)] = hold(bv_s[_ds(head, DH // 2), _ds(r, 512)])

    def spread_q(hold, head, blk, r):
        q = hold(bq_s[_ds(2 * head + r // 4, 8), _ds(blk, NQ)])
        if r % 4 == 0:
            qs[blk % 2, _ds(r // 4, 8), :] = q
        q = _unpack(q).astype(F32)
        for d in range(4 * r, 4 * r + 4):
            qf[blk % 2, _ds(d, 8), :] = jnp.broadcast_to(q[d % 16:d % 16 + 1], (8, NQ))

    @_job([1] * (NC + 4 * NV + 8))
    def stage_first(ln):
        for c in range(NC):
            stage_k(ln, 0, 0, c)
            yield
        for n in range(4 * NV):
            spread_k(ln, 0, n // 4, n % 4)
            yield
        for r in range(8):
            spread_q(ln, 0, 0, r)
            yield

    @_job([1] * NT)
    def reduce_max(ln, m, ms, u):
        out = []
        for j in range(NT):
            top = jnp.max(m[:, j * 128:(j + 1) * 128], axis=0, keepdims=True)
            out.append(ln(jnp.broadcast_to(top, (8, 128))))
            ms[u] = jnp.concatenate(out, axis=1)
            yield

    @_job([1] * (2 * NT))
    def normalise(ln, l, acc, head, blk):
        for j in range(NT):
            total = jnp.sum(l[:, j * 128:(j + 1) * 128], axis=0, keepdims=True)
            total = ln(jnp.broadcast_to(total, (8, 128)))
            yield
            o = acc[:, j * 128:(j + 1) * 128] * jnp.tile(ln(1.0 / total), (DH // 8, 1))
            o_t[_ds(head, DH // 2), _ds(blk * NT + j, 128)] = _pack(o)
            yield

    def b_steps(head0, t_lo, t_hi, state, qk_end=None, filler=None):
        m_old, m_new, m_run, l, acc = state
        ms = {t_lo // NC - 2: m_old, t_lo // NC - 1: m_new}
        pc = _Pace()

        def hold(time):
            return lambda x: _after(x, pc.mark(time))

        for t in range(t_lo, t_hi):
            u, c = divmod(t, NC)
            par = u // 4 % 2
            live = qk_end is None or t < qk_end
            start = pc.now
            if live:
                words = KC // 2 - (8 if c in VCHUNK else 0)
                q = jnp.concatenate([_unpack(qs[u % 2]), jnp.zeros((128 - DH, NQ), BF)], axis=0)
                s = pc.tick(_dot(_unpack(ks[par, pl.ds(c * KC // 2, words), :]), q))
            else:
                filler(pc, t - qk_end)
            up, cp = divmod(t - NC - LAG, NC)
            if up >= 0:
                p = []
                for j in range(4):
                    z = sbuf[up % 2][_ds(4 * cp + 3 - j, KC // 4), :].reshape(-1, 8, NQ)
                    e = jnp.exp2(z - hold(pc.now - CFG.get("eo", (310, 280, 234, 204))[j])(ms[up]))
                    l = jnp.sum(e, axis=0) if cp == 0 and j == 0 else l + jnp.sum(e, axis=0)
                    p.insert(0, e.reshape(KC // 4, NQ))
                a = pc.tick(_dot(_unpack(vs[up // 4 % 2, :, _ds(cp, KC)]), jnp.concatenate(p, axis=0).astype(BF)))
                acc = a if cp == 0 else acc + a
                if cp == NC - 1:
                    job = normalise(l, acc, head0 + up // 4, up % 4)
                    _run(job) if t == t_hi - 1 else pc.spread(pc.now, pc.now + CFG.get("fo", 250), job)
            if not live:
                continue
            sbuf[u % 2][pl.ds(c * KC, 2 * words), :] = s
            mx = jnp.max(s.reshape(-1, 8, NQ), axis=0)
            m_run = mx if c == 0 else jnp.maximum(m_run, mx)
            nd, nt = CFG.get("aa", 4), CFG.get("nt", 1)
            w = nt * 128
            pieces = NV * NT // nt * DH // nd // NC
            for n in range(pieces):
                bj, r = divmod(c * pieces + n, DH // nd)
                b, j = divmod(bj, NT // nt)
                kd = jnp.tile(kf[par, _ds(b * (DH // nd) + r, 16 * nd), :], (1, nt)).reshape(nd, 2, 8, w)
                term = jnp.sum(kd * qf[u % 2, _ds(r, 8 * nd), _ds(j, w)].reshape(nd, 1, 8, w), axis=0).reshape(16, w)
                sv = hold(start + (pc.now - start) * (n + 1) // pieces - CFG.get("ld", 95))(term if r == 0 else sv + term)
                if r == DH // nd - 1:
                    sbuf[u % 2][pl.ds((VCHUNK[b] + 1) * KC - 16, 16), _ds(j, w)] = sv
                    m_run = jnp.concatenate(
                        [jnp.maximum(m_run[:, k * w:(k + 1) * w], jnp.maximum(sv[:8], sv[8:])) if k == j
                         else m_run[:, k * w:(k + 1) * w] for k in range(NT // nt)], axis=1)
            if c == NC - 1:
                pc.spread(pc.now + 30, pc.now + CFG.get("fm", 210), reduce_max(m_run, ms, u))
            sq = CFG.get("sq", (5, 6, 7, 8, 9, 10, 11, 12))
            if (qk_end is None or t + NC < qk_end) and c in sq:
                spread_q(hold(start - CFG.get("qo", 80)), head0 + (u + 1) // 4, (u + 1) % 4, sq.index(c))
            if u % 4 == 0 and c % 4 == 3:
                stage_v(hold(start - 80), head0 + u // 4, par, c // 4)
            if qk_end is None or t + 4 * NC < qk_end:
                n = (t % (4 * NC) - T0 - 3) * 4 // 5
                if u % 4 == 0:
                    stage_k(hold(start - 154), head0 + u // 4 + 1, 1 - par, c)
                elif 0 <= n < 4 * NV and n != (t % (4 * NC) - T0 - 4) * 4 // 5:
                    spread_k(hold(start - 154), 1 - par, n // 4, n % 4)
        assert not pc.queue
        zero = jnp.zeros((8, NQ), F32)
        return ms.get(t_hi // NC - 2, zero), ms.get(t_hi // NC - 1, zero), m_run, l, acc

    def early_out_proj(pc, n):
        if n < 16:
            x_t[0, _ds(n, 64), :] += project(pc, w_t, 16 * WBO + n, 32, o_t, 0)

    def b_layer(first):
        if on("bq1"):
            pc = _Pace()
            pc.spread(0, 2000, layernorm(15))
            if first:
                pc.spread(4500, 11500, prep_w(WBO, range(8)))
            b_qkv(pc, 0)
        if on("bq2"):
            lax.fori_loop(1, 7, lambda p, c: b_qkv(_Pace(), p), None)
            pc = _Pace()
            pc.spread(4400, 11800, stage_first())
            b_qkv(pc, 7)
        if on("battn"):
            zero = jnp.zeros((8, NQ), F32)
            heads = D // DH
            state = b_steps(0, 0, T0, (zero, zero, zero, zero, jnp.zeros((DH, NQ), F32)))
            state = lax.fori_loop(0, heads // 2 - 1, lambda i, st: b_steps(2 * i, T0, T0 + 8 * NC, st), state)
            if CFG.get("epi", 1):
                b_steps(heads - 2, T0, 9 * NC + LAG, state, 8 * NC, early_out_proj)

    if on("start"):
      with jax.named_scope("P0_start"):
        dma([x_copy(0), x_copy(1)], [x_copy(0)])
        dma(weights(0), [x_copy(1)])
        for ct in range(8):
            _run(load_x(0, ct))
        _run(layernorm(0))
        dma([], weights(0))
        dma([x_copy(2)], [])
      for n in range(3):
        _run(prep_aq1(0, n))
      for n in range(3):
        _run(prep_aq2(0, n))

    a_layer(CFG.get("first", True))
    with jax.named_scope("P2_b"):
        b_layer(True)
    if on("bo"):
      with jax.named_scope("P3_bo"):
        for tile in range(1, 16):
            pc = _Pace()
            pc.spread(0, 2000, layernorm(tile - 1))
            out_proj(pc, WBO, tile)
    if PH == "all":
        with jax.named_scope("P4_a"):
            a_layer(False)
        with jax.named_scope("P5_b"):
            b_layer(False)

    if on("final"):
      with jax.named_scope("P6_final"):
        for r in range(4):
            for c in range(8):
                pc = _Pace()
                r1, c1 = divmod(8 * r + c - 1, 8)
                if r1 >= 0:
                    pc.spread(0, 300, store_x1(2 * r1, c1), store_x1(2 * r1 + 1, c1))
                r2, c2 = divmod(8 * r + c - 2, 8)
                if r2 >= 0 and c2 % 4 == 3:
                    pc.spread(0, 1000, store_x2(2 * r2, c2 // 4), store_x2(2 * r2 + 1, c2 // 4))
                for tile in (c, 8 + c) if c else (8,):
                    x_t[tile, _ds(r, 256), :] += project(pc, w_t, 4 * WBO + r, 128, o_t, tile)
        for job in (store_x1(6, 7), store_x1(7, 7), store_x2(6, 1), store_x2(7, 1)):
            _run(job)
        dma([], [out_copy(h, ct) for h in range(2) for ct in range(8)])
    else:
        def keep(i, c):
            for r_ in (x_t, qb, kb, vb, qf, kf):
                s0[pl.ds(0, 8), pl.ds(0, 128)] += r_[i, pl.ds(0, 8), pl.ds(0, 128)]
            for r_ in (bq_s, bv_s, bk_s, xn_t, o_t, w_t, aq_t, ao_perm):
                tmp[pl.ds(0, 8), :] |= r_[_ds(i, 8), pl.ds(0, 128)]
            return c
        lax.fori_loop(0, 2, keep, 0)
        x_raw[0, pl.ds(0, 2), :, pl.ds(0, 128)] = _unpack(tmp[pl.ds(0, 8), :] | lax.bitcast_convert_type(s0[pl.ds(0, 8), pl.ds(0, 128)], U32)).reshape(2, 8, 128)
        out_copy(0, 0).start(); out_copy(0, 0).wait()


@jax.jit
def pallas_interleave_layers__sliding_local_dilated__softmax_full_mha__prompt_kernel(
    A_x: jax.Array,
    A_wqkv: jax.Array,
    A_wo: jax.Array,
    B_x: jax.Array,
    B_wqkv: jax.Array,
    B_wo: jax.Array,
):
    del B_x
    vmem = pltpu.VMEM
    scratch = [
        vmem((2, 128, 8, D), BF), vmem((D, 3 * D), BF), vmem((D, 5 * D), BF),
        vmem((4 * D, 128), U32), vmem((4 * D, 128), U32), vmem((D // 2, D), U32),
        vmem((3 * D // 2, D), U32), vmem((5 * D // 2, D), U32),
        vmem((16, D, 128), F32), vmem((D // 2, S), U32), vmem((D // 2, S), U32),
        vmem((2, 256, 8 * 128), F32), vmem((2, 256, 15 * 128), F32), vmem((2, 256, 15 * 128), F32),
        vmem((4, 256, 128), F32),
        vmem((D // 2, S), U32), vmem((S // 2, D), U32), vmem((D // 2, S), U32),
        vmem((S, NQ), F32), vmem((S, NQ), F32),
        vmem((2, DH // 2, NQ), U32), vmem((2, S // 2, 128), U32), vmem((2, DH // 2, S), U32),
        vmem((2, 8 * DH, NQ), F32), vmem((2, 8 * DH * 16, 128), F32),
        pltpu.SemaphoreType.DMA((3,)), pltpu.SemaphoreType.DMA((12,)),
        pltpu.SemaphoreType.DMA((3,)), pltpu.SemaphoreType.DMA((16,)),
    ]
    out = pl.pallas_call(
        _kernel,
        out_shape=jax.ShapeDtypeStruct((128, 2, 8, D), A_x.dtype),
        in_specs=[pl.BlockSpec(memory_space=pl.ANY)] * 5,
        out_specs=pl.BlockSpec(memory_space=pl.ANY),
        scratch_shapes=scratch,
        compiler_params=pltpu.CompilerParams(vmem_limit_bytes=124 * 1024 * 1024),
        name="interleaved_attention_layers",
    )(A_x.reshape(128, 2, 8, D), A_wqkv, A_wo, B_wqkv, B_wo)
    return out.reshape(A_x.shape)
```

```python
import math

import jax
import jax.numpy as jnp
import numpy as np
from jax import lax
import jax.experimental.pallas as pl
import jax.experimental.pallas.tpu as pltpu

S = 2048
D = 1024
DH = 32
WIN = 8
EPS = 1e-5
LOG2E = math.log2(math.e)
QSCALE = DH ** -0.5 * LOG2E
MASKED = -1e9 * LOG2E

NQ = 512
NT = NQ // 128
KC = 128
NC = S // KC
LAG = 3
T0 = 24
VCHUNK = (0, 3, 6, 9, 12)
NV = len(VCHUNK)

BF = jnp.bfloat16
F32 = jnp.float32
U32 = jnp.uint32
WAO, WBQ, WBK, WBV, WBO = range(5)


def _pack(x):
    return pltpu.bitcast(x.astype(BF), U32)


def _unpack(x):
    return pltpu.bitcast(x, BF)


def _halves(w):
    lo = lax.bitcast_convert_type(w << 16, F32)
    hi = lax.bitcast_convert_type(w & np.uint32(0xFFFF0000), F32)
    return lo, hi


def _ds(i, n):
    if isinstance(i, int):
        return pl.ds(i * n, n)
    return pl.ds(pl.multiple_of(i * n, n), n)


def _dot(a, b):
    return jnp.dot(a, b, preferred_element_type=F32)


def _after(x, token):
    if token is None:
        return x
    if x.shape != token.shape:
        token = jnp.tile(token, (x.shape[0] // 8, x.shape[1] // 128))
    return lax.select(token < -jnp.inf, jnp.zeros_like(x), x)


class _Hold:
    def __init__(self, token=None):
        self.token = token

    def __call__(self, x):
        return _after(x, self.token)

    def head(self, x):
        return x if self.token is None else jnp.concatenate([self(x[:8]), x[8:]], axis=0)


class _Pace:
    def __init__(self):
        self.now, self.queue, self.results = 0, [], []

    def spread(self, lo, hi, *jobs):
        hold = _Hold()
        total = sum(sum(costs) for _, _, costs in jobs)
        done = 0
        for fn, args, costs in jobs:
            gen = fn(hold, *args)
            for cost in costs:
                self.queue.append((lo + (hi - lo) * done // total, hold, gen))
                done += cost
        self.queue.sort(key=lambda piece: piece[0])

    def at(self, time):
        for start, y in reversed(self.results):
            if start <= time:
                row = (time - start) // 8 * 8
                return _Hold(y[row:row + 8, :128])
        return _Hold()

    def tick(self, y):
        self.results.append((self.now, y))
        self.now += y.shape[0]
        while self.queue and self.queue[0][0] < self.now:
            time, hold, gen = self.queue.pop(0)
            hold.token = self.at(time).token
            next(gen)
        return y

    def close(self):
        assert not self.queue


def _job(costs):
    def wrap(fn):
        return lambda *args: (fn, args, costs(*args) if callable(costs) else costs)
    return wrap


def _run(*jobs):
    for fn, args, _ in jobs:
        for _ in fn(_Hold(), *args):
            pass


def _kernel(x_hbm, aq_hbm, ao_hbm, bq_hbm, bo_hbm, out_hbm,
            x_raw, aq_raw, w_raw, tmp0, tmp1, ao_perm, aq_t, w_t,
            x_t, xn_t, o_t,
            qa, ka, va, v_first,
            q_all, k_all, v_all, q_blk, k_head, v_head, q_rep, k_rep, s0, s1,
            sem_in, sem_out):
    tmp, scores = (tmp0, tmp1), (s0, s1)

    def inputs(n):
        def x(h):
            return x_hbm.at[:, h], x_raw.at[h]

        def aq(col, width):
            return aq_hbm.at[:, pl.ds(col, width)], aq_raw.at[:, pl.ds(col, width)]

        def w(src, j):
            return src, w_raw.at[:, pl.ds(j * D, src.shape[1])]

        batch = ([x(0)], [aq(D, 256)], [aq(2 * D, 256), aq(0, 256)], [x(1)],
                 [aq(t * D + 256, 256) for t in range(3)],
                 [aq(t * D + 512, 512) for t in range(3)] + [w(ao_hbm, WAO)],
                 [w(bq_hbm, WBQ), w(bo_hbm, WBO)])[n]
        return [pltpu.make_async_copy(src, dst, sem_in.at[n]) for src, dst in batch]

    def start(n):
        for copy in inputs(n):
            copy.start()

    def wait(n):
        for copy in inputs(n):
            copy.wait()

    def out_copy(h, r):
        return pltpu.make_async_copy(x_raw.at[h, :, :, _ds(r, 256)], out_hbm.at[:, h, :, _ds(r, 256)], sem_out)

    @_job([1] * 5)
    def load_x(hold, h, ct):
        tmp0[_ds(ct, 512), :] = hold(_pack(x_raw[h, :, :, _ds(ct, 128)].reshape(S // 2, 128)))
        yield
        for c in range(4):
            lo, hi = _halves(hold.head(tmp0[pl.ds(ct * 512 + c, 128, stride=4), :]).T)
            x_t[4 * h + c, _ds(ct, 128), :] = lo
            x_t[8 + 4 * h + c, _ds(ct, 128), :] = hi
            yield

    @_job([1])
    def gather_out(hold, ct, c):
        lo = lax.bitcast_convert_type(x_t[c, _ds(ct, 128), :].astype(BF).astype(F32), U32)
        hi = lax.bitcast_convert_type(x_t[8 + c, _ds(ct, 128), :].astype(BF).astype(F32), U32)
        tmp[c // 4][pl.ds(ct * 512 + c % 4, 128, stride=4), :] = hold.head((lo >> 16) | hi).T
        yield

    @_job([1] * 8)
    def write_out(hold, ct, h):
        for r in range(8):
            w = hold(tmp[h][pl.ds(ct * 512 + r * 64, 64), :])
            x_raw[h, _ds(r, 16), :, _ds(ct, 128)] = _unpack(w).reshape(16, 8, 128)
            if r == 7 and ct % 2:
                out_copy(h, ct // 2).start()
            yield

    def head_major(hold, src, base, dp):
        lo, hi = _halves(hold(src[pl.ds(base + dp, 64, stride=16), :]))
        w = jnp.concatenate([lo.reshape(8, 8, 128), hi.reshape(8, 8, 128)], axis=1)
        return jnp.concatenate([w[n] for n in range(8)], axis=1)

    @_job([1] * 8)
    def transpose_aq(hold, g, n):
        for kt in range(8):
            w = _pack(aq_raw[_ds(kt, 128), _ds(4 * ((n + 1) % 3) + g, 256)])
            tmp1[pl.ds(n * D + kt * 128, 128), :] = _pack(_unpack(hold.head(w)).T)
            yield

    @_job([40] * 16)
    def permute_aq(hold, g, n):
        for dp in range(16):
            aq_t[_ds(16 * (3 * g + n) + dp, 8), :] = _pack(head_major(hold, tmp1, n * D, dp))
            yield

    @_job([60] * 4 + [40] * 16)
    def permute_ao(hold, g):
        for n in range(4):
            w = [_pack(w_raw[_ds(g, 256), _ds(8 * WAO + 2 * n + ct, 128)]) for ct in range(2)]
            tmp0[_ds(4 * g + n, 256), :] = hold(jnp.concatenate(w, axis=0))
            yield
        for dp in range(16):
            ao_perm[_ds(16 * g + dp, 8), :] = _pack(head_major(hold, tmp0, g * D, dp))
            yield

    @_job(lambda j, tiles: [1] * (4 * len(tiles)))
    def transpose_w(hold, j, tiles):
        for ct in tiles:
            for k in range(4):
                if j == WAO:
                    w = ao_perm[_ds(k, 128), _ds(ct, 128)]
                else:
                    w = _pack(w_raw[_ds(k, 256), _ds(8 * j + ct, 128)])
                w_t[_ds(8 * j + ct, 64), _ds(k, 256)] = _pack(_unpack(hold.head(w)).T)
                yield

    @_job([40] * 10 + [30] * 8)
    def layernorm(hold, tile):
        stat = []
        for k in range(2):
            for r in range(4):
                x = x_t[tile, _ds(r, 256), :].reshape(16, 16, 128)
                if k:
                    x = x - hold(stat[0])
                    x = x * x
                acc = hold(jnp.sum(x, axis=0) if r == 0 else acc + jnp.sum(x, axis=0))
                yield
            t = jnp.broadcast_to(jnp.sum(acc, axis=0, keepdims=True) * (1.0 / D), (16, 128))
            stat.append(hold(lax.rsqrt(t + EPS) if k else t))
            yield
        for r in range(8):
            x = (x_t[tile, _ds(r, 128), :].reshape(8, 16, 128) - hold(stat[0])) * stat[1]
            xn_t[_ds(r, 64), _ds(tile, 128)] = _pack(x.reshape(128, 128))
            yield

    def project(pace, w_ref, row, words, src, tile):
        lo, hi = [pace.tick(_dot(_unpack(w_ref[_ds(row, words), _ds(k, D // 2)]),
                                 _unpack(src[_ds(k, D // 4), _ds(tile, 128)]))) for k in range(2)]
        return lo + hi

    def out_proj(pace, j, tile):
        for r in range(4):
            x_t[tile, _ds(r, 256), :] += project(pace, w_t, 4 * j + r, 128, o_t, tile)
        pace.close()

    def a_qkv(pace, g, e, c, arrived):
        par = g % 2
        k = project(pace, aq_t, 3 * g, 128, xn_t, 8 * e + c)
        ka[par, :, _ds(7 + c, 128)] = k
        if arrived:
            wait(arrived)
            start(arrived + 1)
        if c:
            ka[par, :, _ds(c - 1, 128)] = pltpu.roll(k, 1, 1)
        v = project(pace, aq_t, 3 * g + 1, 128, xn_t, 8 * e + c)
        va[par, :, _ds(7 + c, 128)] = v
        if c:
            lane0 = lax.broadcasted_iota(jnp.int32, (256, 128), 1) == 0
            va[par, :, _ds(c - 1, 128)] = jnp.where(lane0, v_first[g], pltpu.roll(v, 1, 1))
        elif e == 0:
            v_first[g] = v
        qa[par, :, _ds(c, 128)] = project(pace, aq_t, 3 * g + 2, 128, xn_t, 8 * e + c)

    @_job([32] * 7 + [30] * 4 + [32] * 8)
    def a_attn(hold, g, e, c):
        par = g % 2
        win = pl.ds(c * 128, WIN * 128)
        for r in range(8):
            t = jnp.tile(qa[par, _ds(r, 32), _ds(c, 128)], (1, WIN)) * ka[par, _ds(r, 32), win]
            t = jnp.sum(t.reshape(4, 8, WIN * 128), axis=0)
            acc = hold(t if r == 0 else acc + t)
            yield
        lane0 = lax.broadcasted_iota(jnp.int32, (8, 128), 1) == 0
        logit = []
        for w in range(WIN):
            t = acc[:, w * 128:(w + 1) * 128] * QSCALE
            logit.append(jnp.where(lane0, MASKED, t) if c + w < 7 else t)
        m = logit[0]
        for t in logit[1:]:
            m = jnp.maximum(m, t)
        m = hold(m)
        yield
        p = [jnp.exp2(t - m) for t in logit]
        total = hold(sum(p[1:], p[0]))
        yield
        inv = hold(1.0 / total)
        yield
        p = [t * inv for t in p]
        for r in range(8):
            t = jnp.tile(jnp.concatenate([hold(p[0])] + p[1:], axis=1), (4, 1)) * va[par, _ds(r, 32), win]
            o = sum([t[:, w * 128:(w + 1) * 128] for w in range(1, WIN)], t[:, :128])
            o_t[_ds(8 * g + r, 16), _ds(8 * e + c, 128)] = _pack(o)
            yield

    def a_layer(first):
        for u in range(8):
            pace = _Pace()
            jobs = [a_attn((u - 1) % 4, (u - 1) // 4, c) for c in range(8)] if u else []
            if not first:
                if u == 0:
                    pace.spread(0, 2000, layernorm(15))
            elif u == 0:
                for lo, hi, tile in ((600, 1300, 1), (1536, 2400, 2), (2500, 3400, 3), (5300, 5950, 4),
                                     (6144, 7000, 5), (7100, 8000, 6), (8192, 9800, 7)):
                    pace.spread(lo, hi, layernorm(tile))
                pace.spread(3584, 5100, *[load_x(1, ct) for ct in range(8)])
                pace.spread(8192, 9700, *[transpose_aq(1, n) for n in range(3)])
                pace.spread(9900, 12200, *[permute_aq(1, n) for n in range(3)])
            elif u < 3:
                pace.spread(6656 if u == 1 else 0, 9000, *[transpose_aq(u + 1, n) for n in range(3)])
                jobs += [layernorm(t) for t in range(8, 12)] if u == 1 else [permute_ao(g) for g in range(4)]
                jobs += [permute_aq(u + 1, n) for n in range(3)]
            elif u == 3:
                wait(6)
                jobs += [layernorm(t) for t in range(12, 16)]
                pace.spread(0, 1700, transpose_w(WAO, range(8)))
            if jobs:
                pace.spread(0, 12000, *jobs)
            for c in range(8):
                a_qkv(pace, u % 4, u // 4, c, first and {(0, 2): 3, (0, 5): 4, (1, 4): 5}.get((u, c)))
            pace.close()
        for tile in range(16):
            pace = _Pace()
            pace.spread(0, 2000, *([layernorm(tile - 1)] if tile else []), *([a_attn(3, 1, tile)] if tile < 8 else []))
            if first and tile >= 4:
                pace.spread(0, 1800, transpose_w((WBK, WBQ, WBV)[tile // 4 - 1], (tile % 4 * 2, tile % 4 * 2 + 1)))
            out_proj(pace, WAO, tile)

    def b_qkv(pace, p):
        for r in range(4):
            k = [project(pace, w_t, 4 * WBK + r, 128, xn_t, 2 * p + n).astype(BF) for n in range(2)]
            k = jnp.concatenate(k, axis=1)
            for g in range(2):
                k_all[_ds(p, 128), _ds(2 * r + g, 128)] = _pack(k[g * 128:(g + 1) * 128].T)
        for tile in (2 * p, 2 * p + 1):
            for r in range(4):
                q_all[_ds(r, 128), _ds(tile, 128)] = _pack(project(pace, w_t, 4 * WBQ + r, 128, xn_t, tile) * QSCALE)
            for r in range(4):
                v_all[_ds(r, 128), _ds(tile, 128)] = _pack(project(pace, w_t, 4 * WBV + r, 128, xn_t, tile))
        pace.close()

    def stage_k(hold, head, par, c):
        k = hold.head(k_all[_ds(c, KC // 2), _ds(head // 4, 128)])
        k_head[par, _ds(c, KC // 2), :] = pltpu.roll(k, (128 - DH * (head % 4)) % 128, 1)

    def repeat_k(hold, par, b, r):
        k = _unpack(hold(k_head[par, pl.ds((VCHUNK[b] + 1) * KC // 2 - 8, 8), :])).astype(F32)
        k_rep[par, _ds(4 * b + r, 128), :] = jnp.concatenate(
            [jnp.broadcast_to(k[:, d:d + 1], (16, 128)) for d in range(8 * r, 8 * r + 8)], axis=0)

    def stage_v(hold, head, par, r):
        v_head[par, :, _ds(r, 512)] = hold(v_all[_ds(head, DH // 2), _ds(r, 512)])

    def stage_q(hold, head, blk, r):
        q = hold(q_all[_ds(2 * head + r // 4, 8), _ds(blk, NQ)])
        if r % 4 == 0:
            q_blk[blk % 2, _ds(r // 4, 8), :] = q
        q = _unpack(q).astype(F32)
        for d in range(4 * r, 4 * r + 4):
            q_rep[blk % 2, _ds(d, 8), :] = jnp.broadcast_to(q[d % 16:d % 16 + 1], (8, NQ))

    @_job([1] * (NC + 4 * NV + 8))
    def stage_first(hold):
        for c in range(NC):
            stage_k(hold, 0, 0, c)
            yield
        for n in range(4 * NV):
            repeat_k(hold, 0, n // 4, n % 4)
            yield
        for r in range(8):
            stage_q(hold, 0, 0, r)
            yield

    @_job([1] * NT)
    def reduce_max(hold, m, row_max, u):
        out = []
        for j in range(NT):
            top = jnp.max(m[:, j * 128:(j + 1) * 128], axis=0, keepdims=True)
            out.append(hold(jnp.broadcast_to(top, (8, 128))))
            if j == NT - 1:
                row_max[u] = jnp.concatenate(out, axis=1)
            yield

    @_job([1] * (2 * NT))
    def normalise(hold, l, acc, head, blk):
        for j in range(NT):
            total = jnp.sum(l[:, j * 128:(j + 1) * 128], axis=0, keepdims=True)
            total = hold(jnp.broadcast_to(total, (8, 128)))
            yield
            o = acc[:, j * 128:(j + 1) * 128] * jnp.tile(hold(1.0 / total), (DH // 8, 1))
            o_t[_ds(head, DH // 2), _ds(blk * NT + j, 128)] = _pack(o)
            yield

    def b_steps(head0, t_lo, t_hi, state, end=math.inf):
        m_prev, m_run, l, acc = state
        row_max = {t_lo // NC - 1: m_prev}
        pace = _Pace()
        for t in range(t_lo, t_hi):
            u, c = divmod(t, NC)
            par, begin = u // 4 % 2, pace.now
            if t < end:
                words = KC // 2 - (8 if c in VCHUNK else 0)
                q = jnp.concatenate([_unpack(q_blk[u % 2]), jnp.zeros((128 - DH, NQ), BF)], axis=0)
                s = pace.tick(_dot(_unpack(k_head[par, pl.ds(c * KC // 2, words), :]), q))
            elif t - end < 16:
                x_t[0, _ds(t - end, 64), :] += project(pace, w_t, 16 * WBO + t - end, 32, o_t, 0)
            up, cp = divmod(t - NC - LAG, NC)
            if up >= 0:
                p = []
                for j, lead in enumerate((310, 280, 234, 204)):
                    z = scores[up % 2][_ds(4 * cp + 3 - j, KC // 4), :].reshape(-1, 8, NQ)
                    e = jnp.exp2(z - pace.at(pace.now - lead)(row_max[up]))
                    l = jnp.sum(e, axis=0) if cp == 0 and j == 0 else l + jnp.sum(e, axis=0)
                    p.insert(0, e.reshape(KC // 4, NQ))
                pv = _dot(_unpack(v_head[up // 4 % 2, :, _ds(cp, KC)]), jnp.concatenate(p, axis=0).astype(BF))
                acc = pace.tick(pv) if cp == 0 else acc + pace.tick(pv)
                if cp == NC - 1:
                    job = normalise(l, acc, head0 + up // 4, up % 4)
                    if t == t_hi - 1:
                        _run(job)
                    else:
                        pace.spread(pace.now, pace.now + 250, job)
            if t >= end:
                continue
            scores[u % 2][pl.ds(c * KC, 2 * words), :] = s
            top = jnp.max(s.reshape(-1, 8, NQ), axis=0)
            m_run = top if c == 0 else jnp.maximum(m_run, top)
            for n in range(2 * NV):
                bj, r = divmod(2 * NV * c + n, 8)
                b, j = divmod(bj, NT)
                term = (k_rep[par, _ds(8 * b + r, 64), :].reshape(4, 2, 8, 128)
                        * q_rep[u % 2, _ds(r, 32), _ds(j, 128)].reshape(4, 1, 8, 128))
                term = jnp.sum(term, axis=0).reshape(16, 128)
                hold = pace.at(begin + (pace.now - begin) * (n + 1) // (2 * NV) - 98)
                sv = hold(term if r == 0 else sv + term)
                if r == 7:
                    scores[u % 2][pl.ds((VCHUNK[b] + 1) * KC - 16, 16), _ds(j, 128)] = sv
                    m_run = [m_run[:, i * 128:(i + 1) * 128] for i in range(NT)]
                    m_run[j] = jnp.maximum(m_run[j], jnp.maximum(sv[:8], sv[8:]))
                    m_run = jnp.concatenate(m_run, axis=1)
            if c == NC - 1:
                pace.spread(pace.now + 30, pace.now + 130, reduce_max(m_run, row_max, u))
            if t + NC < end and 5 <= c < 13:
                stage_q(pace.at(begin - 40), head0 + (u + 1) // 4, (u + 1) % 4, c - 5)
            if u % 4 == 0 and c % 4 == 3:
                stage_v(pace.at(begin - 80), head0 + u // 4, par, c // 4)
            if t + 4 * NC < end:
                n = (t % (4 * NC) - T0 - 3) * 4 // 5
                if u % 4 == 0:
                    stage_k(pace.at(begin - 154), head0 + u // 4 + 1, 1 - par, c)
                elif 0 <= n < 4 * NV and n != (t % (4 * NC) - T0 - 4) * 4 // 5:
                    repeat_k(pace.at(begin - 154), 1 - par, n // 4, n % 4)
        pace.close()
        return row_max.get(t_hi // NC - 1), m_run, l, acc

    def b_layer(first):
        pace = _Pace()
        pace.spread(0, 2000, layernorm(15))
        if first:
            pace.spread(4500, 11500, transpose_w(WBO, range(8)))
        b_qkv(pace, 0)
        lax.fori_loop(1, 7, lambda p, _: b_qkv(_Pace(), p), None)
        pace = _Pace()
        pace.spread(4400, 11800, stage_first())
        b_qkv(pace, 7)
        heads = D // DH
        state = b_steps(0, 0, T0, (None,) * 4)
        state = lax.fori_loop(0, heads // 2 - 1, lambda i, st: b_steps(2 * i, T0, T0 + 8 * NC, st), state)
        b_steps(heads - 2, T0, 9 * NC + LAG, state, 8 * NC)

    for n in range(3):
        start(n)
    wait(0)
    _run(*[load_x(0, ct) for ct in range(8)], layernorm(0))
    wait(1)
    start(3)
    _run(transpose_aq(0, 0), permute_aq(0, 0))
    wait(2)
    _run(transpose_aq(0, 1), transpose_aq(0, 2), permute_aq(0, 1), permute_aq(0, 2))

    a_layer(True)
    b_layer(True)
    for tile in range(1, 16):
        pace = _Pace()
        pace.spread(0, 2000, layernorm(tile - 1))
        out_proj(pace, WBO, tile)
    a_layer(False)
    b_layer(False)

    for r in range(4):
        for c in range(8):
            pace = _Pace()
            r1, c1 = divmod(8 * r + c - 1, 8)
            if r1 >= 0:
                pace.spread(0, 300, gather_out(2 * r1, c1), gather_out(2 * r1 + 1, c1))
            r2, c2 = divmod(8 * r + c - 2, 8)
            if r2 >= 0 and c2 % 4 == 3:
                pace.spread(0, 1000, write_out(2 * r2, c2 // 4), write_out(2 * r2 + 1, c2 // 4))
            for tile in (c, 8 + c) if c else (8,):
                x_t[tile, _ds(r, 256), :] += project(pace, w_t, 4 * WBO + r, 128, o_t, tile)
            pace.close()
    _run(gather_out(6, 7), gather_out(7, 7), write_out(6, 1), write_out(7, 1))
    for n in range(8):
        out_copy(n // 4, n % 4).wait()


@jax.jit
def pallas_interleave_layers__sliding_local_dilated__softmax_full_mha__prompt_kernel(
    A_x: jax.Array,
    A_wqkv: jax.Array,
    A_wo: jax.Array,
    B_x: jax.Array,
    B_wqkv: jax.Array,
    B_wo: jax.Array,
):
    del B_x
    vmem = pltpu.VMEM
    scratch = [
        vmem((2, 128, 8, D), BF), vmem((D, 3 * D), BF), vmem((D, 5 * D), BF),
        vmem((4 * D + 32, 128), U32), vmem((4 * D + 32, 128), U32), vmem((D // 2, D), U32),
        vmem((3 * D // 2, D), U32), vmem((5 * D // 2, D), U32),
        vmem((16, D, 128), F32), vmem((D // 2, S), U32), vmem((D // 2, S), U32),
        vmem((2, 256, 8 * 128), F32), vmem((2, 256, 15 * 128), F32), vmem((2, 256, 15 * 128), F32),
        vmem((4, 256, 128), F32),
        vmem((D // 2, S), U32), vmem((S // 2, D), U32), vmem((D // 2, S), U32),
        vmem((2, DH // 2, NQ), U32), vmem((2, S // 2, 128), U32), vmem((2, DH // 2, S), U32),
        vmem((2, 8 * DH, NQ), F32), vmem((2, NV * DH * 16, 128), F32),
        vmem((S, NQ), F32), vmem((S, NQ), F32),
        pltpu.SemaphoreType.DMA((7,)), pltpu.SemaphoreType.DMA(()),
    ]
    out = pl.pallas_call(
        _kernel,
        out_shape=jax.ShapeDtypeStruct((128, 2, 8, D), A_x.dtype),
        in_specs=[pl.BlockSpec(memory_space=pl.ANY)] * 5,
        out_specs=pl.BlockSpec(memory_space=pl.ANY),
        scratch_shapes=scratch,
        compiler_params=pltpu.CompilerParams(vmem_limit_bytes=120 * 1024 * 1024),
        name="interleaved_attention_layers",
    )(A_x.reshape(128, 2, 8, D), A_wqkv, A_wo, B_wqkv, B_wo)
    return out.reshape(A_x.shape)
```

```python
import math

import jax
import jax.numpy as jnp
import numpy as np
from jax import lax
import jax.experimental.pallas as pl
import jax.experimental.pallas.tpu as pltpu

S = 2048
D = 1024
DH = 32
WIN = 8
EPS = 1e-5
LOG2E = math.log2(math.e)
QSCALE = DH ** -0.5 * LOG2E
MASKED = -1e9 * LOG2E

NQ = 512
NT = NQ // 128
KC = 128
NC = S // KC
LAG = 3
T0 = 24
NE = 6
NV = 5

BF = jnp.bfloat16
F32 = jnp.float32
U32 = jnp.uint32
WAO, WBQ, WBK, WBV, WBO = range(5)


def _pack(x):
    return pltpu.bitcast(x.astype(BF), U32)


def _unpack(x):
    return pltpu.bitcast(x, BF)


def _halves(w):
    lo = lax.bitcast_convert_type(w << 16, F32)
    hi = lax.bitcast_convert_type(w & np.uint32(0xFFFF0000), F32)
    return lo, hi


def _ds(i, n):
    if isinstance(i, int):
        return pl.ds(i * n, n)
    return pl.ds(pl.multiple_of(i * n, n), n)


def _dot(a, b):
    return jnp.dot(a, b, preferred_element_type=F32)


def _after(x, token):
    if token is None:
        return x
    if x.shape != token.shape:
        token = jnp.tile(token, (x.shape[0] // 8, x.shape[1] // 128))
    return lax.select(token < -jnp.inf, jnp.zeros_like(x), x)


class _Hold:
    def __init__(self, token=None):
        self.token = token

    def __call__(self, x):
        return _after(x, self.token)

    def head(self, x):
        return x if self.token is None else jnp.concatenate([self(x[:8]), x[8:]], axis=0)


class _Pace:
    def __init__(self):
        self.now, self.queue, self.results = 0, [], []

    def spread(self, lo, hi, *jobs):
        hold = _Hold()
        total = sum(sum(costs) for _, _, costs in jobs)
        done = 0
        for fn, args, costs in jobs:
            gen = fn(hold, *args)
            for cost in costs:
                self.queue.append((lo + (hi - lo) * done // total, hold, gen))
                done += cost
        self.queue.sort(key=lambda piece: piece[0])

    def at(self, time):
        for start, y in reversed(self.results):
            if start <= time:
                row = (time - start) // 8 * 8
                return _Hold(y[row:row + 8, :128])
        return _Hold()

    def tick(self, y):
        self.results.append((self.now, y))
        self.now += y.shape[0]
        while self.queue and self.queue[0][0] < self.now:
            time, hold, gen = self.queue.pop(0)
            hold.token = self.at(time).token
            next(gen)
        return y

    def close(self):
        assert not self.queue


def _job(costs):
    def wrap(fn):
        return lambda *args: (fn, args, costs(*args) if callable(costs) else costs)
    return wrap


def _run(*jobs):
    for fn, args, _ in jobs:
        for _ in fn(_Hold(), *args):
            pass


def _kernel(x_hbm, aq_hbm, ao_hbm, bq_hbm, bo_hbm, out_hbm,
            x_raw, aq_raw, w_raw, tmp0, tmp1, ao_perm, aq_t, w_t,
            x_t, xn_t, o_t,
            qa, ka, va, v_first,
            q_all, k_all, v_all, q_blk, k_head, v_head, q_rep, k_rep, s_early, s0, s1,
            sem_in, sem_out):
    tmp, scores = (tmp0, tmp1), (s0, s1)

    def inputs(n):
        def x(h):
            return x_hbm.at[:, h], x_raw.at[h]

        def aq(col, width):
            return aq_hbm.at[:, pl.ds(col, width)], aq_raw.at[:, pl.ds(col, width)]

        def w(src, j):
            return src, w_raw.at[:, pl.ds(j * D, src.shape[1])]

        batch = ([x(0)], [aq(D, 256)], [aq(2 * D, 256), aq(0, 256)], [x(1)],
                 [aq(t * D + 256, 256) for t in range(3)],
                 [aq(t * D + 512, 512) for t in range(3)] + [w(ao_hbm, WAO)],
                 [w(bq_hbm, WBQ), w(bo_hbm, WBO)])[n]
        return [pltpu.make_async_copy(src, dst, sem_in.at[n]) for src, dst in batch]

    def start(n):
        for copy in inputs(n):
            copy.start()

    def wait(n):
        for copy in inputs(n):
            copy.wait()

    def out_copy(h, r):
        return pltpu.make_async_copy(x_raw.at[h, :, :, _ds(r, 256)], out_hbm.at[:, h, :, _ds(r, 256)], sem_out)

    @_job([1] * 5)
    def load_x(hold, h, ct):
        tmp0[_ds(ct, 512), :] = hold(_pack(x_raw[h, :, :, _ds(ct, 128)].reshape(S // 2, 128)))
        yield
        for c in range(4):
            lo, hi = _halves(hold.head(tmp0[pl.ds(ct * 512 + c, 128, stride=4), :]).T)
            x_t[4 * h + c, _ds(ct, 128), :] = lo
            x_t[8 + 4 * h + c, _ds(ct, 128), :] = hi
            yield

    @_job([1])
    def gather_out(hold, ct, c):
        lo = lax.bitcast_convert_type(x_t[c, _ds(ct, 128), :].astype(BF).astype(F32), U32)
        hi = lax.bitcast_convert_type(x_t[8 + c, _ds(ct, 128), :].astype(BF).astype(F32), U32)
        tmp[c // 4][pl.ds(ct * 512 + c % 4, 128, stride=4), :] = hold.head((lo >> 16) | hi).T
        yield

    @_job([1] * 8)
    def write_out(hold, ct, h):
        for r in range(8):
            w = hold(tmp[h][pl.ds(ct * 512 + r * 64, 64), :])
            x_raw[h, _ds(r, 16), :, _ds(ct, 128)] = _unpack(w).reshape(16, 8, 128)
            if r == 7 and ct % 2:
                out_copy(h, ct // 2).start()
            yield

    def head_major(hold, src, base, dp):
        lo, hi = _halves(hold(src[pl.ds(base + dp, 64, stride=16), :]))
        w = jnp.concatenate([lo.reshape(8, 8, 128), hi.reshape(8, 8, 128)], axis=1)
        return jnp.concatenate([w[n] for n in range(8)], axis=1)

    @_job([1] * 8)
    def transpose_aq(hold, g, n):
        for kt in range(8):
            w = _pack(aq_raw[_ds(kt, 128), _ds(4 * ((n + 1) % 3) + g, 256)])
            tmp1[pl.ds(n * D + kt * 128, 128), :] = _pack(_unpack(hold.head(w)).T)
            yield

    @_job([40] * 16)
    def permute_aq(hold, g, n):
        for dp in range(16):
            aq_t[_ds(16 * (3 * g + n) + dp, 8), :] = _pack(head_major(hold, tmp1, n * D, dp))
            yield

    @_job([60] * 4 + [40] * 16)
    def permute_ao(hold, g):
        for n in range(4):
            w = [_pack(w_raw[_ds(g, 256), _ds(8 * WAO + 2 * n + ct, 128)]) for ct in range(2)]
            tmp0[_ds(4 * g + n, 256), :] = hold(jnp.concatenate(w, axis=0))
            yield
        for dp in range(16):
            ao_perm[_ds(16 * g + dp, 8), :] = _pack(head_major(hold, tmp0, g * D, dp))
            yield

    @_job(lambda j, tiles: [1] * (4 * len(tiles)))
    def transpose_w(hold, j, tiles):
        for ct in tiles:
            for k in range(4):
                if j == WAO:
                    w = ao_perm[_ds(k, 128), _ds(ct, 128)]
                else:
                    w = _pack(w_raw[_ds(k, 256), _ds(8 * j + ct, 128)])
                w_t[_ds(8 * j + ct, 64), _ds(k, 256)] = _pack(_unpack(hold.head(w)).T)
                yield

    @_job([40] * 10 + [30] * 8)
    def layernorm(hold, tile):
        stat = []
        for k in range(2):
            for r in range(4):
                x = x_t[tile, _ds(r, 256), :].reshape(16, 16, 128)
                if k:
                    x = x - hold(stat[0])
                    x = x * x
                acc = hold(jnp.sum(x, axis=0) if r == 0 else acc + jnp.sum(x, axis=0))
                yield
            t = jnp.broadcast_to(jnp.sum(acc, axis=0, keepdims=True) * (1.0 / D), (16, 128))
            stat.append(hold(lax.rsqrt(t + EPS) if k else t))
            yield
        for r in range(8):
            x = (x_t[tile, _ds(r, 128), :].reshape(8, 16, 128) - hold(stat[0])) * stat[1]
            xn_t[_ds(r, 64), _ds(tile, 128)] = _pack(x.reshape(128, 128))
            yield

    def project(pace, w_ref, row, words, src, tile):
        lo, hi = [pace.tick(_dot(_unpack(w_ref[_ds(row, words), _ds(k, D // 2)]),
                                 _unpack(src[_ds(k, D // 4), _ds(tile, 128)]))) for k in range(2)]
        return lo + hi

    def out_proj(pace, j, tile):
        for r in range(4):
            x_t[tile, _ds(r, 256), :] += project(pace, w_t, 4 * j + r, 128, o_t, tile)
        pace.close()

    def a_qkv(pace, g, e, c, arrived):
        par = g % 2
        k = project(pace, aq_t, 3 * g, 128, xn_t, 8 * e + c)
        ka[par, :, _ds(7 + c, 128)] = k
        if arrived:
            wait(arrived)
            start(arrived + 1)
        if c:
            ka[par, :, _ds(c - 1, 128)] = pltpu.roll(k, 1, 1)
        v = project(pace, aq_t, 3 * g + 1, 128, xn_t, 8 * e + c)
        va[par, :, _ds(7 + c, 128)] = v
        if c:
            lane0 = lax.broadcasted_iota(jnp.int32, (256, 128), 1) == 0
            va[par, :, _ds(c - 1, 128)] = jnp.where(lane0, v_first[g], pltpu.roll(v, 1, 1))
        elif e == 0:
            v_first[g] = v
        qa[par, :, _ds(c, 128)] = project(pace, aq_t, 3 * g + 2, 128, xn_t, 8 * e + c)

    @_job([32] * 7 + [30] * 4 + [32] * 8)
    def a_attn(hold, g, e, c):
        par = g % 2
        win = pl.ds(c * 128, WIN * 128)
        for r in range(8):
            t = jnp.tile(qa[par, _ds(r, 32), _ds(c, 128)], (1, WIN)) * ka[par, _ds(r, 32), win]
            t = jnp.sum(t.reshape(4, 8, WIN * 128), axis=0)
            acc = hold(t if r == 0 else acc + t)
            yield
        lane0 = lax.broadcasted_iota(jnp.int32, (8, 128), 1) == 0
        logit = []
        for w in range(WIN):
            t = acc[:, w * 128:(w + 1) * 128] * QSCALE
            logit.append(jnp.where(lane0, MASKED, t) if c + w < 7 else t)
        m = logit[0]
        for t in logit[1:]:
            m = jnp.maximum(m, t)
        m = hold(m)
        yield
        p = [jnp.exp2(t - m) for t in logit]
        total = hold(sum(p[1:], p[0]))
        yield
        inv = hold(1.0 / total)
        yield
        p = [t * inv for t in p]
        for r in range(8):
            t = jnp.tile(jnp.concatenate([hold(p[0])] + p[1:], axis=1), (4, 1)) * va[par, _ds(r, 32), win]
            o = sum([t[:, w * 128:(w + 1) * 128] for w in range(1, WIN)], t[:, :128])
            o_t[_ds(8 * g + r, 16), _ds(8 * e + c, 128)] = _pack(o)
            yield

    def a_layer(first):
        for u in range(8):
            pace = _Pace()
            jobs = [a_attn((u - 1) % 4, (u - 1) // 4, c) for c in range(8)] if u else []
            if not first:
                if u == 0:
                    pace.spread(0, 2000, layernorm(15))
            elif u == 0:
                for lo, hi, tile in ((600, 1300, 1), (1536, 2400, 2), (2500, 3400, 3), (5300, 5950, 4),
                                     (6144, 7000, 5), (7100, 8000, 6), (8192, 9800, 7)):
                    pace.spread(lo, hi, layernorm(tile))
                pace.spread(3584, 5100, *[load_x(1, ct) for ct in range(8)])
                pace.spread(8192, 9700, *[transpose_aq(1, n) for n in range(3)])
                pace.spread(9900, 12200, *[permute_aq(1, n) for n in range(3)])
            elif u < 3:
                pace.spread(6656 if u == 1 else 0, 9000, *[transpose_aq(u + 1, n) for n in range(3)])
                jobs += [layernorm(t) for t in range(8, 12)] if u == 1 else [permute_ao(g) for g in range(4)]
                jobs += [permute_aq(u + 1, n) for n in range(3)]
            elif u == 3:
                wait(6)
                jobs += [layernorm(t) for t in range(12, 16)]
                pace.spread(0, 1700, transpose_w(WAO, range(8)))
            if jobs:
                pace.spread(0, 12000, *jobs)
            for c in range(8):
                a_qkv(pace, u % 4, u // 4, c, first and {(0, 2): 3, (0, 5): 4, (1, 4): 5}.get((u, c)))
            pace.close()
        for tile in range(16):
            pace = _Pace()
            pace.spread(0, 2000, *([layernorm(tile - 1)] if tile else []), *([a_attn(3, 1, tile)] if tile < 8 else []))
            if first and tile >= 4:
                pace.spread(0, 1800, transpose_w((WBK, WBQ, WBV)[tile // 4 - 1], (tile % 4 * 2, tile % 4 * 2 + 1)))
            out_proj(pace, WAO, tile)

    def b_qkv(pace, k_tiles, q_tiles, v_tiles):
        for tile in k_tiles:
            k_all[_ds(tile, 64), :] = _pack(project(pace, w_t, WBK, D // 2, xn_t, tile).astype(BF).T)
        for tile in q_tiles:
            q_all[:, _ds(tile, 128)] = _pack(project(pace, w_t, WBQ, D // 2, xn_t, tile) * QSCALE)
        for tile in v_tiles:
            v_all[:, _ds(tile, 128)] = _pack(project(pace, w_t, WBV, D // 2, xn_t, tile))
        pace.close()

    def stage_k(hold, head, par, c):
        k = hold.head(k_all[_ds(c, KC // 2), _ds(head // 4, 128)])
        k_head[par, _ds(c, KC // 2), :] = pltpu.roll(k, (128 - DH * (head % 4)) % 128, 1)

    def repeat_k(k, d0, slot, n):
        k = _unpack(k).astype(F32)
        k_rep[slot, _ds(n, 128), :] = jnp.concatenate(
            [jnp.broadcast_to(k[:, d:d + 1], (16, 128)) for d in range(d0, d0 + 8)], axis=0)

    def vector_scores(k_slot, q_slot, b, r, cols):
        k = jnp.tile(k_rep[k_slot, _ds(8 * b + r, 64), :], (1, cols.size // 128)).reshape(4, 2, 8, -1)
        return jnp.sum(k * q_rep[q_slot, _ds(r, 32), cols].reshape(4, 1, 8, -1), axis=0).reshape(16, -1)

    def stage_v(hold, head, par, r):
        v_head[par, :, _ds(r, 512)] = hold(v_all[_ds(head, DH // 2), _ds(r, 512)])

    def stage_q(hold, head, blk, r):
        if r % 4 == 0:
            q_blk[blk % 2, _ds(r // 4, 8), :] = q_all[_ds(2 * head + r // 4, 8), _ds(blk, NQ)]
        q = _unpack(hold(q_blk[blk % 2, _ds(r // 4, 8), :])).astype(F32)
        for d in range(4 * r, 4 * r + 4):
            q_rep[blk % 2, _ds(d, 8), :] = jnp.broadcast_to(q[d % 16:d % 16 + 1], (8, NQ))

    @_job([1] * (4 * NE))
    def early_keys(hold, g, h):
        for n in range(4 * NE):
            repeat_k(hold(k_all[_ds(n // 4, 8), _ds(g, 128)]), DH * h + n % 4 * 8, 2 + h % 2, n)
            yield

    @_job([1] * 8)
    def early_queries(hold, head, blk):
        for r in range(8):
            stage_q(hold, head, blk, r)
            yield

    @_job([1] * (16 * NE))
    def early_scores(hold, g, h, blk):
        for n in range(16 * NE):
            b, j, r = n // 16, n // 8 % 2, n % 8
            term = vector_scores(2 + h % 2, blk, b, r, _ds(j, 256))
            sv = hold(term if r == 0 else sv + term)
            if r == 7:
                s_early[_ds((4 * g + h) * NE + b, 16), _ds(2 * blk + j, 256)] = sv
            yield

    def early(pace, g, turns, length):
        for n in range(turns):
            lo, hi = length * n // turns, length * (n + 1) // turns
            pace.spread(lo, hi, early_scores(g, n // 2, n % 2))
            more = turns == 8 or n + 1 < turns
            pace.spread(lo + 40, hi - 40, early_queries(4 * g + (n + 1) // 2 if more else 0, (n + 1) % 2))
            if n % 2 == 0 and (turns == 8 or n + 2 < turns):
                pace.spread(lo + 40, 2 * hi - lo - 300, early_keys(g + n // 6, (n // 2 + 1) % 4))

    @_job([1] * (NC + 4 * NV))
    def stage_first(hold):
        for c in range(NC):
            stage_k(hold, 0, 0, c)
            yield
        for n in range(4 * NV):
            repeat_k(hold(k_head[0, _ds(NE + n // 4, 8), :]), n % 4 * 8, 0, n)
            yield

    @_job([1] * NT)
    def reduce_max(hold, m, row_max, u):
        out = []
        for j in range(NT):
            top = jnp.max(m[:, j * 128:(j + 1) * 128], axis=0, keepdims=True)
            out.append(hold(jnp.broadcast_to(top, (8, 128))))
            if j == NT - 1:
                row_max[u] = jnp.concatenate(out, axis=1)
            yield

    @_job([1] * (2 * NT))
    def normalise(hold, l, acc, head, blk):
        for j in range(NT):
            total = jnp.sum(l[:, j * 128:(j + 1) * 128], axis=0, keepdims=True)
            total = hold(jnp.broadcast_to(total, (8, 128)))
            yield
            o = acc[:, j * 128:(j + 1) * 128] * jnp.tile(hold(1.0 / total), (DH // 8, 1))
            o_t[_ds(head, DH // 2), _ds(blk * NT + j, 128)] = _pack(o)
            yield

    def b_steps(head0, t_lo, t_hi, state, end=math.inf):
        m_prev, m_run, l, acc = state
        row_max = {t_lo // NC - 1: m_prev}
        pace = _Pace()
        for t in range(t_lo, t_hi):
            u, c = divmod(t, NC)
            par, begin = u // 4 % 2, pace.now
            has_early = u % 4 < 2 and t + 4 * NC < end
            if t < end:
                blocks = [b for b in range(S // 16) if b >= NE + NV or (b < NE and not has_early)]
                blocks = blocks[len(blocks) * c // NC:len(blocks) * (c + 1) // NC]
                runs = [r for r in ([b for b in blocks if b < NE], [b for b in blocks if b >= NE]) if r]
                k = jnp.concatenate([k_head[par, pl.ds(8 * r[0], 8 * len(r)), :] for r in runs], axis=0)
                q = jnp.concatenate([_unpack(q_blk[u % 2]), jnp.zeros((128 - DH, NQ), BF)], axis=0)
                s = pace.tick(_dot(_unpack(k), q))
            elif t - end < 16:
                x_t[0, _ds(t - end, 64), :] += project(pace, w_t, 16 * WBO + t - end, 32, o_t, 0)
            up, cp = divmod(t - NC - LAG, NC)
            if up >= 0:
                p = []
                for j, lead in enumerate((310, 272, 234, 204)):
                    z = scores[up % 2][_ds(4 * cp + 3 - j, KC // 4), :].reshape(-1, 8, NQ)
                    e = jnp.exp2(z - pace.at(pace.now - lead)(row_max[up]))
                    l = jnp.sum(e, axis=0) if cp == 0 and j == 0 else l + jnp.sum(e, axis=0)
                    p.insert(0, e.reshape(KC // 4, NQ))
                pv = _dot(_unpack(v_head[up // 4 % 2, :, _ds(cp, KC)]), jnp.concatenate(p, axis=0).astype(BF))
                acc = pace.tick(pv) if cp == 0 else acc + pace.tick(pv)
                if cp == NC - 1:
                    job = normalise(l, acc, head0 + up // 4, up % 4)
                    if t == t_hi - 1:
                        _run(job)
                    else:
                        pace.spread(pace.now, pace.now + 400, job)
            if t >= end:
                continue
            for r in runs:
                row = 16 * blocks.index(r[0])
                scores[u % 2][pl.ds(16 * r[0], 16 * len(r)), :] = s[row:row + 16 * len(r)]
            top = jnp.max(s.reshape(-1, 8, NQ), axis=0)
            m_run = top if c == 0 else jnp.maximum(m_run, top)
            if has_early and NE * (c + 1) // NC > NE * c // NC:
                b = NE * c // NC
                done = pace.at(begin - 90)(s_early[_ds((head0 + u // 4) * NE + b, 16), _ds(u % 4, NQ)])
                scores[u % 2][_ds(b, 16), :] = done
                m_run = jnp.maximum(m_run, jnp.maximum(done[:8], done[8:]))
            for n in range(2 * NV):
                bj, r = divmod(2 * NV * c + n, 8)
                b, j = divmod(bj, NT)
                term = vector_scores(par, u % 2, b, r, _ds(j, 128))
                hold = pace.at(begin + (pace.now - begin) * (n + 1) // (2 * NV) - 101)
                sv = hold(term if r == 0 else sv + term)
                if r == 7:
                    scores[u % 2][_ds(NE + b, 16), _ds(j, 128)] = sv
                    m_run = [m_run[:, i * 128:(i + 1) * 128] for i in range(NT)]
                    m_run[j] = jnp.maximum(m_run[j], jnp.maximum(sv[:8], sv[8:]))
                    m_run = jnp.concatenate(m_run, axis=1)
            if c == NC - 1:
                pace.spread(pace.now + 30, pace.now + 160, reduce_max(m_run, row_max, u))
            if t + NC < end and 5 <= c < 13:
                stage_q(pace.at(begin - 60), head0 + (u + 1) // 4, (u + 1) % 4, c - 5)
            if u % 4 == 0 and c % 4 == 3:
                stage_v(pace.at(begin - 80), head0 + u // 4, par, c // 4)
            if t + 4 * NC < end:
                n = (t % (4 * NC) - T0 - 3) * 4 // 5
                if u % 4 == 0:
                    stage_k(pace.at(begin - 154), head0 + u // 4 + 1, 1 - par, c)
                elif 0 <= n < 4 * NV and n != (t % (4 * NC) - T0 - 4) * 4 // 5:
                    repeat_k(pace.at(begin - 154)(k_head[1 - par, _ds(NE + n // 4, 8), :]), n % 4 * 8, 1 - par, n)
        pace.close()
        return row_max.get(t_hi // NC - 1), m_run, l, acc

    def b_layer(first):
        pace = _Pace()
        pace.spread(0, 2000, layernorm(15))
        if first:
            pace.spread(4500, 11500, transpose_w(WBO, range(8)))
        pace.spread(12000, 18000, early_keys(0, 0), early_queries(0, 0))
        b_qkv(pace, [0], range(8), [])

        def body(g, _):
            pace = _Pace()
            early(pace, g, 8, 10200)
            b_qkv(pace, [2 * g + 1, 2 * g + 2], [8 + g], [2 * g, 2 * g + 1])

        lax.fori_loop(0, 7, body, None)
        pace = _Pace()
        early(pace, 7, 6, 8150)
        pace.spread(2300, 7800, stage_first())
        b_qkv(pace, [15], [15], [14, 15])
        heads = D // DH
        state = b_steps(0, 0, T0, (None,) * 4)
        state = lax.fori_loop(0, heads // 2 - 1, lambda i, st: b_steps(2 * i, T0, T0 + 8 * NC, st), state)
        b_steps(heads - 2, T0, 9 * NC + LAG, state, 8 * NC)

    for n in range(3):
        start(n)
    wait(0)
    _run(*[load_x(0, ct) for ct in range(8)], layernorm(0))
    wait(1)
    start(3)
    _run(transpose_aq(0, 0), permute_aq(0, 0))
    wait(2)
    _run(transpose_aq(0, 1), transpose_aq(0, 2), permute_aq(0, 1), permute_aq(0, 2))

    a_layer(True)
    b_layer(True)
    for tile in range(1, 16):
        pace = _Pace()
        pace.spread(0, 2000, layernorm(tile - 1))
        out_proj(pace, WBO, tile)
    a_layer(False)
    b_layer(False)

    for r in range(4):
        for c in range(8):
            pace = _Pace()
            r1, c1 = divmod(8 * r + c - 1, 8)
            if r1 >= 0:
                pace.spread(0, 300, gather_out(2 * r1, c1), gather_out(2 * r1 + 1, c1))
            r2, c2 = divmod(8 * r + c - 2, 8)
            if r2 >= 0 and c2 % 4 == 3:
                pace.spread(0, 1000, write_out(2 * r2, c2 // 4), write_out(2 * r2 + 1, c2 // 4))
            for tile in (c, 8 + c) if c else (8,):
                x_t[tile, _ds(r, 256), :] += project(pace, w_t, 4 * WBO + r, 128, o_t, tile)
            pace.close()
    _run(gather_out(6, 7), gather_out(7, 7), write_out(6, 1), write_out(7, 1))
    for n in range(8):
        out_copy(n // 4, n % 4).wait()


@jax.jit
def pallas_interleave_layers__sliding_local_dilated__softmax_full_mha__prompt_kernel(
    A_x: jax.Array,
    A_wqkv: jax.Array,
    A_wo: jax.Array,
    B_x: jax.Array,
    B_wqkv: jax.Array,
    B_wo: jax.Array,
):
    del B_x
    vmem = pltpu.VMEM
    scratch = [
        vmem((2, 128, 8, D), BF), vmem((D, 3 * D), BF), vmem((D, 5 * D), BF),
        vmem((4 * D + 32, 128), U32), vmem((4 * D + 32, 128), U32), vmem((D // 2, D), U32),
        vmem((3 * D // 2, D), U32), vmem((5 * D // 2, D), U32),
        vmem((16, D, 128), F32), vmem((D // 2, S), U32), vmem((D // 2, S), U32),
        vmem((2, 256, 8 * 128), F32), vmem((2, 256, 15 * 128), F32), vmem((2, 256, 15 * 128), F32),
        vmem((4, 256, 128), F32),
        vmem((D // 2, S), U32), vmem((S // 2, D), U32), vmem((D // 2, S), U32),
        vmem((2, DH // 2, NQ), U32), vmem((2, S // 2, 128), U32), vmem((2, DH // 2, S), U32),
        vmem((2, 8 * DH, NQ), F32), vmem((4, max(NE, NV) * DH * 16, 128), F32),
        vmem((D // DH * NE * 16, 2 * NQ), F32), vmem((S, NQ), F32), vmem((S, NQ), F32),
        pltpu.SemaphoreType.DMA((7,)), pltpu.SemaphoreType.DMA(()),
    ]
    out = pl.pallas_call(
        _kernel,
        out_shape=jax.ShapeDtypeStruct((128, 2, 8, D), A_x.dtype),
        in_specs=[pl.BlockSpec(memory_space=pl.ANY)] * 5,
        out_specs=pl.BlockSpec(memory_space=pl.ANY),
        scratch_shapes=scratch,
        compiler_params=pltpu.CompilerParams(vmem_limit_bytes=120 * 1024 * 1024),
        name="interleaved_attention_layers",
    )(A_x.reshape(128, 2, 8, D), A_wqkv, A_wo, B_wqkv, B_wo)
    return out.reshape(A_x.shape)
```

```python
import math

import jax
import jax.numpy as jnp
import numpy as np
from jax import lax
import jax.experimental.pallas as pl
import jax.experimental.pallas.tpu as pltpu

S = 2048
D = 1024
DH = 32
WIN = 8
EPS = 1e-5
LOG2E = math.log2(math.e)
QSCALE = DH ** -0.5 * LOG2E
MASKED = -1e9 * LOG2E

NQ = 256
KC = 256
NC = S // KC
NH = NC * S // NQ
LAG = 3
T0 = 14
NE = 6
NV = 6

BF = jnp.bfloat16
F32 = jnp.float32
U32 = jnp.uint32
WAO, WBQ, WBK, WBV, WBO = range(5)


def _pack(x):
    return pltpu.bitcast(x.astype(BF), U32)


def _unpack(x):
    return pltpu.bitcast(x, BF)


def _halves(w):
    lo = lax.bitcast_convert_type(w << 16, F32)
    hi = lax.bitcast_convert_type(w & np.uint32(0xFFFF0000), F32)
    return lo, hi


def _ds(i, n):
    if isinstance(i, int):
        return pl.ds(i * n, n)
    return pl.ds(pl.multiple_of(i * n, n), n)


def _dot(a, b):
    return lax.dot_general(a, b, (((1,), (0,)), ((), ())), preferred_element_type=F32)


def _after(x, token):
    if token is None:
        return x
    if x.shape != token.shape:
        token = jnp.tile(token, (x.shape[0] // 8, x.shape[1] // 128))
    return lax.select(token < -jnp.inf, jnp.zeros_like(x), x)


class _Hold:
    def __init__(self, token=None):
        self.token = token

    def __call__(self, x):
        return _after(x, self.token)

    def head(self, x):
        return x if self.token is None else jnp.concatenate([self(x[:8]), x[8:]], axis=0)


class _Pace:
    def __init__(self):
        self.now, self.queue, self.results = 0, [], []

    def spread(self, lo, hi, *jobs):
        hold = _Hold()
        total = sum(sum(costs) for _, _, costs in jobs)
        done = 0
        for fn, args, costs in jobs:
            gen = fn(hold, *args)
            for cost in costs:
                self.queue.append((lo + (hi - lo) * done // total, hold, gen))
                done += cost
        self.queue.sort(key=lambda piece: piece[0])

    def at(self, time):
        for start, y in reversed(self.results):
            if start <= time:
                row = (time - start) // 8 * 8
                return _Hold(y[row:row + 8, :128])
        return _Hold()

    def tick(self, y):
        self.results.append((self.now, y))
        self.now += y.shape[0]
        while self.queue and self.queue[0][0] < self.now:
            time, hold, gen = self.queue.pop(0)
            hold.token = self.at(time).token
            next(gen)
        return y

    def close(self):
        assert not self.queue


def _job(costs):
    def wrap(fn):
        return lambda *args: (fn, args, costs(*args) if callable(costs) else costs)
    return wrap


def _run(*jobs):
    for fn, args, _ in jobs:
        for _ in fn(_Hold(), *args):
            pass


def _kernel(x_hbm, aq_hbm, ao_hbm, bq_hbm, bo_hbm, out_hbm,
            x_raw, aq_raw, w_raw, tmp0, tmp1, ao_perm, aq_t, w_t,
            x_t, xn_t, o_t,
            qa, ka, va, v_first,
            q_all, k_all, v_all, q_blk, k_head, v_head, q_rep, k_rep, s_early, scores,
            sem_in, sem_out):
    tmp = (tmp0, tmp1)

    def inputs(n):
        def x(h):
            return x_hbm.at[:, h], x_raw.at[h]

        def aq(col, width):
            return aq_hbm.at[:, pl.ds(col, width)], aq_raw.at[:, pl.ds(col, width)]

        def w(src, j):
            return src, w_raw.at[:, pl.ds(j * D, src.shape[1])]

        batch = ([x(0)], [aq(D, 256)], [aq(2 * D, 256), aq(0, 256)], [x(1)],
                 [aq(t * D + 256, 256) for t in range(3)],
                 [aq(t * D + 512, 512) for t in range(3)] + [w(ao_hbm, WAO)],
                 [w(bq_hbm, WBQ), w(bo_hbm, WBO)])[n]
        return [pltpu.make_async_copy(src, dst, sem_in.at[n]) for src, dst in batch]

    def start(n):
        for copy in inputs(n):
            copy.start()

    def wait(n):
        for copy in inputs(n):
            copy.wait()

    def out_copy(h, r):
        return pltpu.make_async_copy(x_raw.at[h, :, :, _ds(r, 256)], out_hbm.at[:, h, :, _ds(r, 256)], sem_out)

    @_job([1] * 5)
    def load_x(hold, h, ct):
        tmp0[_ds(ct, 512), :] = hold(_pack(x_raw[h, :, :, _ds(ct, 128)].reshape(S // 2, 128)))
        yield
        for c in range(4):
            lo, hi = _halves(hold.head(tmp0[pl.ds(ct * 512 + c, 128, stride=4), :]).T)
            x_t[4 * h + c, _ds(ct, 128), :] = lo
            x_t[8 + 4 * h + c, _ds(ct, 128), :] = hi
            yield

    @_job([1])
    def gather_out(hold, ct, c):
        lo = lax.bitcast_convert_type(x_t[c, _ds(ct, 128), :].astype(BF).astype(F32), U32)
        hi = lax.bitcast_convert_type(x_t[8 + c, _ds(ct, 128), :].astype(BF).astype(F32), U32)
        tmp[c // 4][pl.ds(ct * 512 + c % 4, 128, stride=4), :] = hold.head((lo >> 16) | hi).T
        yield

    @_job([1] * 8)
    def write_out(hold, ct, h):
        for r in range(8):
            w = hold(tmp[h][pl.ds(ct * 512 + r * 64, 64), :])
            x_raw[h, _ds(r, 16), :, _ds(ct, 128)] = _unpack(w).reshape(16, 8, 128)
            if r == 7 and ct % 2:
                out_copy(h, ct // 2).start()
            yield

    def head_major(hold, src, base, dp):
        lo, hi = _halves(hold(src[pl.ds(base + dp, 64, stride=16), :]))
        w = jnp.concatenate([lo.reshape(8, 8, 128), hi.reshape(8, 8, 128)], axis=1)
        return jnp.concatenate([w[n] for n in range(8)], axis=1)

    @_job([1] * 8)
    def transpose_aq(hold, g, n):
        for kt in range(8):
            w = _pack(aq_raw[_ds(kt, 128), _ds(4 * ((n + 1) % 3) + g, 256)])
            tmp1[pl.ds(n * D + kt * 128, 128), :] = _pack(_unpack(hold.head(w)).T)
            yield

    @_job([40] * 16)
    def permute_aq(hold, g, n):
        for dp in range(16):
            aq_t[_ds(16 * (3 * g + n) + dp, 8), :] = _pack(head_major(hold, tmp1, n * D, dp))
            yield

    @_job([60] * 4 + [40] * 16)
    def permute_ao(hold, g):
        for n in range(4):
            w = [_pack(w_raw[_ds(g, 256), _ds(8 * WAO + 2 * n + ct, 128)]) for ct in range(2)]
            tmp0[_ds(4 * g + n, 256), :] = hold(jnp.concatenate(w, axis=0))
            yield
        for dp in range(16):
            ao_perm[_ds(16 * g + dp, 8), :] = _pack(head_major(hold, tmp0, g * D, dp))
            yield

    @_job(lambda j, tiles: [1] * (4 * len(tiles)))
    def transpose_w(hold, j, tiles):
        for ct in tiles:
            for k in range(4):
                if j == WAO:
                    w = ao_perm[_ds(k, 128), _ds(ct, 128)]
                else:
                    w = _pack(w_raw[_ds(k, 256), _ds(8 * j + ct, 128)])
                w_t[_ds(8 * j + ct, 64), _ds(k, 256)] = _pack(_unpack(hold.head(w)).T)
                yield

    @_job([40] * 10 + [30] * 8)
    def layernorm(hold, tile):
        stat = []
        for k in range(2):
            for r in range(4):
                x = x_t[tile, _ds(r, 256), :].reshape(16, 16, 128)
                if k:
                    x = x - hold(stat[0])
                    x = x * x
                acc = hold(jnp.sum(x, axis=0) if r == 0 else acc + jnp.sum(x, axis=0))
                yield
            t = jnp.broadcast_to(jnp.sum(acc, axis=0, keepdims=True) * (1.0 / D), (16, 128))
            stat.append(hold(lax.rsqrt(t + EPS) if k else t))
            yield
        for r in range(8):
            x = (x_t[tile, _ds(r, 128), :].reshape(8, 16, 128) - hold(stat[0])) * stat[1]
            xn_t[_ds(r, 64), _ds(tile, 128)] = _pack(x.reshape(128, 128))
            yield

    def project(pace, w_ref, row, words, src, tile):
        lo, hi = [pace.tick(_dot(_unpack(w_ref[_ds(row, words), _ds(k, D // 2)]),
                                 _unpack(src[_ds(k, D // 4), _ds(tile, 128)]))) for k in range(2)]
        return lo + hi

    def out_proj(pace, j, tile):
        for r in range(4):
            x_t[tile, _ds(r, 256), :] += project(pace, w_t, 4 * j + r, 128, o_t, tile)
        pace.close()

    def a_qkv(pace, g, e, c, arrived):
        par = g % 2
        k = project(pace, aq_t, 3 * g, 128, xn_t, 8 * e + c)
        ka[par, :, _ds(7 + c, 128)] = k
        if arrived:
            wait(arrived)
            start(arrived + 1)
        if c:
            ka[par, :, _ds(c - 1, 128)] = pltpu.roll(k, 1, 1)
        v = project(pace, aq_t, 3 * g + 1, 128, xn_t, 8 * e + c)
        va[par, :, _ds(7 + c, 128)] = v
        if c:
            lane0 = lax.broadcasted_iota(jnp.int32, (256, 128), 1) == 0
            va[par, :, _ds(c - 1, 128)] = jnp.where(lane0, v_first[g], pltpu.roll(v, 1, 1))
        elif e == 0:
            v_first[g] = v
        qa[par, :, _ds(c, 128)] = project(pace, aq_t, 3 * g + 2, 128, xn_t, 8 * e + c)

    @_job([32] * 7 + [30] * 4 + [32] * 8)
    def a_attn(hold, g, e, c):
        par = g % 2
        win = pl.ds(c * 128, WIN * 128)
        for r in range(8):
            t = jnp.tile(qa[par, _ds(r, 32), _ds(c, 128)], (1, WIN)) * ka[par, _ds(r, 32), win]
            t = jnp.sum(t.reshape(4, 8, WIN * 128), axis=0)
            acc = hold(t if r == 0 else acc + t)
            yield
        lane0 = lax.broadcasted_iota(jnp.int32, (8, 128), 1) == 0
        logit = []
        for w in range(WIN):
            t = acc[:, w * 128:(w + 1) * 128] * QSCALE
            logit.append(jnp.where(lane0, MASKED, t) if c + w < 7 else t)
        m = logit[0]
        for t in logit[1:]:
            m = jnp.maximum(m, t)
        m = hold(m)
        yield
        p = [jnp.exp2(t - m) for t in logit]
        total = hold(sum(p[1:], p[0]))
        yield
        inv = hold(1.0 / total)
        yield
        p = [t * inv for t in p]
        for r in range(8):
            t = jnp.tile(jnp.concatenate([hold(p[0])] + p[1:], axis=1), (4, 1)) * va[par, _ds(r, 32), win]
            o = sum([t[:, w * 128:(w + 1) * 128] for w in range(1, WIN)], t[:, :128])
            o_t[_ds(8 * g + r, 16), _ds(8 * e + c, 128)] = _pack(o)
            yield

    def a_layer(first):
        for u in range(8):
            pace = _Pace()
            jobs = [a_attn((u - 1) % 4, (u - 1) // 4, c) for c in range(8)] if u else []
            if not first:
                if u == 0:
                    pace.spread(0, 2000, layernorm(15))
            elif u == 0:
                for lo, hi, tile in ((600, 1300, 1), (1536, 2400, 2), (2500, 3400, 3), (5300, 5950, 4),
                                     (6144, 7000, 5), (7100, 8000, 6), (8192, 9800, 7)):
                    pace.spread(lo, hi, layernorm(tile))
                pace.spread(3584, 5100, *[load_x(1, ct) for ct in range(8)])
                pace.spread(8192, 9700, *[transpose_aq(1, n) for n in range(3)])
                pace.spread(9900, 12200, *[permute_aq(1, n) for n in range(3)])
            elif u < 3:
                pace.spread(6656 if u == 1 else 0, 9000, *[transpose_aq(u + 1, n) for n in range(3)])
                jobs += [layernorm(t) for t in range(8, 12)] if u == 1 else [permute_ao(g) for g in range(4)]
                jobs += [permute_aq(u + 1, n) for n in range(3)]
            elif u == 3:
                wait(6)
                jobs += [layernorm(t) for t in range(12, 16)]
                pace.spread(0, 1700, transpose_w(WAO, range(8)))
            if jobs:
                pace.spread(0, 12000, *jobs)
            for c in range(8):
                a_qkv(pace, u % 4, u // 4, c, first and {(0, 2): 3, (0, 5): 4, (1, 4): 5}.get((u, c)))
            pace.close()
        for tile in range(16):
            pace = _Pace()
            pace.spread(0, 2000, *([layernorm(tile - 1)] if tile else []), *([a_attn(3, 1, tile)] if tile < 8 else []))
            if first and tile >= 4:
                pace.spread(0, 1800, transpose_w((WBK, WBQ, WBV)[tile // 4 - 1], (tile % 4 * 2, tile % 4 * 2 + 1)))
            out_proj(pace, WAO, tile)

    def b_qkv(pace, k_tiles, q_tiles, v_tiles):
        for tile in k_tiles:
            k_all[_ds(tile, 64), :] = _pack(project(pace, w_t, WBK, D // 2, xn_t, tile).astype(BF).T)
        for tile in q_tiles:
            q_all[:, _ds(tile, 128)] = _pack(project(pace, w_t, WBQ, D // 2, xn_t, tile) * QSCALE)
        for tile in v_tiles:
            v_all[:, _ds(tile, 128)] = _pack(project(pace, w_t, WBV, D // 2, xn_t, tile))
        pace.close()

    def stage_k(hold, head, par, c):
        k = hold.head(k_all[_ds(c, 64), _ds(head // 4, 128)])
        k_head[par, _ds(c, 64), :] = pltpu.roll(k, (128 - DH * (head % 4)) % 128, 1)

    def repeat_k(k, d0, slot, n):
        k = _unpack(k).astype(F32)
        k_rep[slot, _ds(n, 128), :] = jnp.concatenate(
            [jnp.broadcast_to(k[:, d:d + 1], (16, 128)) for d in range(d0, d0 + 8)], axis=0)

    def vector_scores(slot, b, r, cols):
        k = jnp.tile(k_rep[slot, _ds(8 * b + r, 64), :], (1, cols.size // 128)).reshape(4, 2, 8, -1)
        return jnp.sum(k * q_rep[_ds(r, 32), cols].reshape(4, 1, 8, -1), axis=0).reshape(16, -1)

    def stage_v(hold, head, par, r):
        v_head[par, :, _ds(r, 512)] = hold(v_all[_ds(head, DH // 2), _ds(r, 512)])

    def stage_q(hold, head, tile, r):
        cols = _ds(tile % 8, 128)
        if r % 2 == 0:
            q_blk[_ds(r // 2, 8), cols] = q_all[_ds(2 * head + r // 2, 8), _ds(tile, 128)]
        q = _unpack(hold(q_blk[_ds(r // 2, 8), cols])).astype(F32)
        q_rep[_ds(r, 64), cols] = jnp.concatenate(
            [jnp.broadcast_to(q[d:d + 1], (8, 128)) for d in range(r % 2 * 8, r % 2 * 8 + 8)], axis=0)

    @_job([1] * (4 * NE))
    def early_keys(hold, g, h):
        for n in range(4 * NE):
            repeat_k(hold(k_all[_ds(n // 4, 8), _ds(g, 128)]), DH * h + n % 4 * 8, 2 + h % 2, n)
            yield

    @_job([1] * 16)
    def early_queries(hold, head, blk):
        for n in range(16):
            stage_q(hold, head, 4 * blk + n // 4, n % 4)
            yield

    @_job([1] * (16 * NE))
    def early_scores(hold, g, h, blk):
        for n in range(16 * NE):
            b, j, r = n // 16, n // 8 % 2, n % 8
            term = vector_scores(2 + h % 2, b, r, _ds(2 * blk + j, 256))
            sv = hold(term if r == 0 else sv + term)
            if r == 7:
                s_early[_ds((4 * g + h) * NE + b, 16), _ds(2 * blk + j, 256)] = sv
            yield

    def early(pace, g, turns, length):
        for n in range(turns):
            lo, hi = length * n // turns, length * (n + 1) // turns
            pace.spread(lo, hi, early_scores(g, n // 2, n % 2))
            more = turns == 8 or n + 1 < turns
            pace.spread(lo + 40, hi - 40, early_queries(4 * g + (n + 1) // 2 if more else 0, (n + 1) % 2))
            if n % 2 == 0 and (turns == 8 or n + 2 < turns):
                pace.spread(lo + 40, 2 * hi - lo - 300, early_keys(g + n // 6, (n // 2 + 1) % 4))

    @_job([1] * (16 + 4 * NV))
    def stage_first(hold):
        for c in range(16):
            stage_k(hold, 0, 0, c)
            yield
        for n in range(4 * NV):
            repeat_k(hold(k_head[0, _ds(NE + n // 4, 8), :]), n % 4 * 8, 0, n)
            yield

    @_job([1] * 2)
    def reduce_max(hold, m, row_max, u):
        lo = hold(jnp.broadcast_to(jnp.max(m[:, :128], axis=0, keepdims=True), (8, 128)))
        yield
        hi = hold(jnp.broadcast_to(jnp.max(m[:, 128:], axis=0, keepdims=True), (8, 128)))
        row_max[u] = jnp.concatenate([lo, hi], axis=1)
        yield

    @_job([1] * 4)
    def normalise(hold, l, acc, head, blk):
        for j in range(2):
            total = jnp.sum(l[:, j * 128:(j + 1) * 128], axis=0, keepdims=True)
            total = hold(jnp.broadcast_to(total, (8, 128)))
            yield
            o = acc[:, j * 128:(j + 1) * 128] * jnp.tile(hold(1.0 / total), (DH // 8, 1))
            o_t[_ds(head, DH // 2), _ds(2 * blk + j, 128)] = _pack(o)
            yield

    def b_steps(head0, t_lo, t_hi, state, end=math.inf):
        m_prev, m_run, l, acc = state
        row_max = {t_lo // NC - 1: m_prev}
        pace = _Pace()
        for t in range(t_lo, t_hi):
            u, c = divmod(t, NC)
            head, step = divmod(t, NH)
            par, blk, begin = head % 2, step // NC, pace.now
            has_early = step < NH // 2 and t + NH < end
            if t < end:
                blocks = [b for b in range(S // 16) if b >= NE + NV or (b < NE and not has_early)]
                blocks = blocks[len(blocks) // 2 * c // NC * 2:len(blocks) // 2 * (c + 1) // NC * 2]
                runs = [r for r in ([b for b in blocks if b < NE], [b for b in blocks if b >= NE]) if r]
                k = jnp.concatenate([k_head[par, pl.ds(8 * r[0], 8 * len(r)), :] for r in runs], axis=0)
                q = jnp.concatenate([_unpack(q_blk[:, _ds(blk % 4, NQ)]), jnp.zeros((128 - DH, NQ), BF)], axis=0)
                s_lo, s_hi = _dot(_unpack(k[:4 * len(blocks)]), q), _dot(_unpack(k[4 * len(blocks):]), q)
                s = jnp.concatenate([pace.tick(s_lo), s_hi], axis=0)
            elif t - end < 8:
                x_t[0, _ds(t - end, 128), :] += project(pace, w_t, 8 * WBO + t - end, 64, o_t, 0)
            up, cp = divmod(t - NC - LAG, NC)
            if up >= 0:
                p = []
                for j, lead in enumerate((302, 264, 226, 196)):
                    z = [scores[up % 2, pl.ds(cp * KC + i + 96 - 32 * j, 32), :] for i in (0, 128)]
                    e = jnp.exp2(jnp.concatenate(z).reshape(-1, 8, NQ) - pace.at(pace.now - lead)(row_max[up]))
                    l = jnp.sum(e, axis=0) if cp == 0 and j == 0 else l + jnp.sum(e, axis=0)
                    p.insert(0, e.reshape(2, 32, NQ))
                p = jnp.concatenate(p, axis=1).reshape(KC, NQ).astype(BF)
                pv = pace.tick(_dot(_unpack(v_head[up * NC // NH % 2, :, _ds(cp, KC)]), p))
                acc = pv if cp == 0 else acc + pv
                if cp == NC - 1:
                    job = normalise(l, acc, head0 + up * NC // NH, up % (NH // NC))
                    if t == t_hi - 1:
                        _run(job)
                    else:
                        pace.spread(pace.now, pace.now + 200, job)
            if t >= end:
                continue
            for r in runs:
                row = 16 * blocks.index(r[0])
                scores[u % 2, pl.ds(16 * r[0], 16 * len(r)), :] = s[row:row + 16 * len(r)]
            top = jnp.max(s.reshape(-1, 8, NQ), axis=0)
            m_run = top if c == 0 else jnp.maximum(m_run, top)
            for b in range(NE * c // NC, NE * (c + 1) // NC) if has_early else ():
                done = pace.at(begin - 120)(s_early[_ds((head0 + head) * NE + b, 16), _ds(blk, NQ)])
                scores[u % 2, _ds(b, 16), :] = done
                m_run = jnp.maximum(m_run, jnp.maximum(done[:8], done[8:]))
            for n in range(2 * NV):
                bj, r = divmod(2 * NV * c + n, 8)
                b, j = divmod(bj, 2)
                term = vector_scores(par, b, r, _ds((2 * blk + j) % 8, 128))
                hold = pace.at(begin + (pace.now - begin) * (n + 1) // (2 * NV) - 92)
                sv = hold(term if r == 0 else sv + term)
                if r == 7:
                    scores[u % 2, _ds(NE + b, 16), _ds(j, 128)] = sv
                    m_run = [m_run[:, :128], m_run[:, 128:]]
                    m_run[j] = jnp.maximum(m_run[j], jnp.maximum(sv[:8], sv[8:]))
                    m_run = jnp.concatenate(m_run, axis=1)
            if c == NC - 1:
                pace.spread(pace.now + 30, pace.now + 94, reduce_max(m_run, row_max, u))
            if t + NC < end:
                tile = (t + NC) // 4
                stage_q(pace.at(begin - 60), head0 + tile // 16, tile % 16, t % 4)
            if t < 4:
                stage_v(_Hold(), 0, 0, t)
            n = step - T0 - 2
            if t + NH < end and 0 <= n < 16:
                stage_k(pace.at(begin - 154), head0 + head + 1, 1 - par, n)
                if n % 4 == 0:
                    stage_v(pace.at(begin - 80), head0 + head + 1, 1 - par, n // 4)
            elif t + NH < end and 16 <= n < 16 + 4 * NV:
                k = pace.at(begin - 154)(k_head[1 - par, _ds(NE + (n - 16) // 4, 8), :])
                repeat_k(k, n % 4 * 8, 1 - par, n - 16)
        pace.close()
        return row_max[t_hi // NC - 1] if t_hi < end else None, m_run, l, acc

    def b_layer(first):
        pace = _Pace()
        pace.spread(0, 2000, layernorm(15))
        if first:
            pace.spread(4500, 11500, transpose_w(WBO, range(8)))
        pace.spread(12000, 18000, early_keys(0, 0), early_queries(0, 0))
        b_qkv(pace, [0], range(8), [])

        def body(g, _):
            pace = _Pace()
            early(pace, g, 8, 10200)
            b_qkv(pace, [2 * g + 1, 2 * g + 2], [8 + g], [2 * g, 2 * g + 1])

        lax.fori_loop(0, 7, body, None)
        pace = _Pace()
        early(pace, 7, 6, 8150)
        pace.spread(2300, 7800, stage_first())
        b_qkv(pace, [15], [15], [14, 15])
        heads = D // DH
        state = b_steps(0, 0, T0, (None,) * 4)
        state = lax.fori_loop(0, heads // 2 - 1, lambda i, st: b_steps(2 * i, T0, T0 + 2 * NH, st), state)
        b_steps(heads - 2, T0, 2 * NH + NC + LAG, state, 2 * NH)

    for n in range(3):
        start(n)
    wait(0)
    _run(*[load_x(0, ct) for ct in range(8)], layernorm(0))
    wait(1)
    start(3)
    _run(transpose_aq(0, 0), permute_aq(0, 0))
    wait(2)
    _run(transpose_aq(0, 1), transpose_aq(0, 2), permute_aq(0, 1), permute_aq(0, 2))

    a_layer(True)
    b_layer(True)
    for tile in range(1, 16):
        pace = _Pace()
        pace.spread(0, 2000, layernorm(tile - 1))
        out_proj(pace, WBO, tile)
    a_layer(False)
    b_layer(False)

    for r in range(4):
        for c in range(8):
            pace = _Pace()
            r1, c1 = divmod(8 * r + c - 1, 8)
            if r1 >= 0:
                pace.spread(0, 300, gather_out(2 * r1, c1), gather_out(2 * r1 + 1, c1))
            r2, c2 = divmod(8 * r + c - 2, 8)
            if r2 >= 0 and c2 % 4 == 3:
                pace.spread(0, 1000, write_out(2 * r2, c2 // 4), write_out(2 * r2 + 1, c2 // 4))
            for tile in (c, 8 + c) if c else (8,):
                x_t[tile, _ds(r, 256), :] += project(pace, w_t, 4 * WBO + r, 128, o_t, tile)
            pace.close()
    _run(gather_out(6, 7), gather_out(7, 7), write_out(6, 1), write_out(7, 1))
    for n in range(8):
        out_copy(n // 4, n % 4).wait()


@jax.jit
def pallas_interleave_layers__sliding_local_dilated__softmax_full_mha__prompt_kernel(
    A_x: jax.Array,
    A_wqkv: jax.Array,
    A_wo: jax.Array,
    B_x: jax.Array,
    B_wqkv: jax.Array,
    B_wo: jax.Array,
):
    del B_x
    vmem = pltpu.VMEM
    scratch = [
        vmem((2, 128, 8, D), BF), vmem((D, 3 * D), BF), vmem((D, 5 * D), BF),
        vmem((4 * D + 32, 128), U32), vmem((4 * D + 32, 128), U32), vmem((D // 2, D), U32),
        vmem((3 * D // 2, D), U32), vmem((5 * D // 2, D), U32),
        vmem((16, D, 128), F32), vmem((D // 2, S), U32), vmem((D // 2, S), U32),
        vmem((2, 256, 8 * 128), F32), vmem((2, 256, 15 * 128), F32), vmem((2, 256, 15 * 128), F32),
        vmem((4, 256, 128), F32),
        vmem((D // 2, S), U32), vmem((S // 2, D), U32), vmem((D // 2, S), U32),
        vmem((DH // 2, 1024), U32), vmem((2, S // 2, 128), U32), vmem((2, DH // 2, S), U32),
        vmem((8 * DH, 1024), F32), vmem((4, max(NE, NV) * DH * 16, 128), F32),
        vmem((D // DH * NE * 16, 1024), F32), vmem((2, S, NQ), F32),
        pltpu.SemaphoreType.DMA((7,)), pltpu.SemaphoreType.DMA(()),
    ]
    out = pl.pallas_call(
        _kernel,
        out_shape=jax.ShapeDtypeStruct((128, 2, 8, D), A_x.dtype),
        in_specs=[pl.BlockSpec(memory_space=pl.ANY)] * 5,
        out_specs=pl.BlockSpec(memory_space=pl.ANY),
        scratch_shapes=scratch,
        compiler_params=pltpu.CompilerParams(vmem_limit_bytes=120 * 1024 * 1024),
        name="interleaved_attention_layers",
    )(A_x.reshape(128, 2, 8, D), A_wqkv, A_wo, B_wqkv, B_wo)
    return out.reshape(A_x.shape)
```
